```python
import jax
import jax.numpy as jnp

def _softmax(x, axis=-1):
    return jax.nn.softmax(x, axis=axis)

def _gelu(x):
    return jax.nn.gelu(x, approximate=True)

def _silu(x):
    return jax.nn.silu(x)

def _sigmoid(x):
    return jax.nn.sigmoid(x)

def _layernorm(x, axis=-1, eps=1e-05):
    m = jnp.mean(x, axis=axis, keepdims=True)
    v = jnp.var(x, axis=axis, keepdims=True)
    return (x - m) / jnp.sqrt(v + eps)

def _scatter_add(tgt, idx, src, axis=0):
    return tgt.at[idx].add(src)

def _segment_sum(src, seg, n):
    return jax.ops.segment_sum(src, seg, n)

class _Rng:

    def __init__(self, key):
        self._k = key

    def _next(self):
        self._k, sub = jax.random.split(self._k)
        return sub

    def normal(self, shape):
        return jax.random.normal(self._next(), shape, dtype=jnp.bfloat16)

    def randint(self, lo, hi, shape):
        return jax.random.randint(self._next(), shape, lo, hi, dtype=jnp.int32)

    def uniform(self, shape, lo=0.0, hi=1.0):
        return jax.random.uniform(self._next(), shape, jnp.bfloat16, lo, hi)

    def permutation(self, n):
        return jax.random.permutation(self._next(), n)
kernel_name = 'interleave_layers__memory_aug_recurrent_mem_tr__linear_kernel_hedgehog__prompt'

def setup_inputs():
    _rng = _Rng(jax.random.key(int.from_bytes(__import__("os").urandom(4), "little")))
    _w = lambda a: (lambda t: t.astype(jnp.bfloat16) if jnp.issubdtype(t.dtype, jnp.floating) else t)(jnp.asarray(a))

    def _A_setup():
        B, S, Dm = (1, 2048, 640)
        H, Dh = (32, 192)
        M, seg = (8, 32)
        seg = min(seg, S)
        S = S // seg * seg
        return {'x': _w((lambda *s: _rng.normal(s) * 0.05)(B, S, Dm)), 'mem0': _w((lambda *s: _rng.normal(s) * 0.05)(B, M, Dm)), 'Wq': _w((lambda *s: _rng.normal(s) * 0.05)(Dm, H, Dh) * Dm ** (-0.5)), 'Wk': _w((lambda *s: _rng.normal(s) * 0.05)(Dm, H, Dh) * Dm ** (-0.5)), 'Wv': _w((lambda *s: _rng.normal(s) * 0.05)(Dm, H, Dh) * Dm ** (-0.5)), 'Wo': _w((lambda *s: _rng.normal(s) * 0.05)(H, Dh, Dm) * (H * Dh) ** (-0.5)), 'seg_len': seg}
    _A_in = _A_setup()

    def _B_setup():
        B, S, D, H = (1, 2048, 640, 32)
        Dh = D // H
        return {'x': _w((lambda *s: _rng.normal(s) * 0.05)(B, S, D)), 'wqkv': _w((lambda *s: _rng.normal(s) * 0.05)(D, 3 * D)), 'w_phi': _w((lambda *s: _rng.normal(s) * 0.05)(H, Dh, Dh) * Dh ** (-0.5)), 'wo': _w((lambda *s: _rng.normal(s) * 0.05)(D, D))}
    _B_in = _B_setup()
    return {'A_x': _A_in['x'], 'A_mem0': _A_in['mem0'], 'A_Wq': _A_in['Wq'], 'A_Wk': _A_in['Wk'], 'A_Wv': _A_in['Wv'], 'A_Wo': _A_in['Wo'], 'A_seg_len': _A_in['seg_len'], 'B_x': _B_in['x'], 'B_wqkv': _B_in['wqkv'], 'B_w_phi': _B_in['w_phi'], 'B_wo': _B_in['wo']}

def reference(A_x, A_mem0, A_Wq, A_Wk, A_Wv, A_Wo, A_seg_len, B_x, B_wqkv, B_w_phi, B_wo):

    def _A_ref(x, mem0, Wq, Wk, Wv, Wo, seg_len):
        B, S, Dm = x.shape
        H, Dh = (Wq.shape[1], Wq.shape[2])
        M = mem0.shape[1]
        scale = Dh ** (-0.5)
        n_seg = S // seg_len
        L = M + seg_len
        idx = jnp.arange(L)
        mask = (idx[:, None] < M) | (idx[:, None] >= idx[None, :])
        mem = mem0
        outs = []
        for s in range(n_seg):
            xs = x[:, s * seg_len:(s + 1) * seg_len, :].copy()
            h = jnp.concatenate([mem, xs], axis=1)
            q = jnp.einsum('btd,dhe->bhte', h, Wq)
            k = jnp.einsum('btd,dhe->bhte', h, Wk)
            v = jnp.einsum('btd,dhe->bhte', h, Wv)
            scores = jnp.einsum('bhqe,bhke->bhqk', q, k) * scale
            scores = jnp.where(mask[None, None], scores, -1000000000.0)
            p = _softmax(scores, axis=-1)
            o = jnp.einsum('bhqk,bhke->bhqe', p, v)
            o = jnp.einsum('bhte,hed->btd', o, Wo)
            mem = o[:, :M, :].copy()
            outs.append(o[:, M:, :])
        return jnp.concatenate(outs, axis=1)

    def _B_ref(x, wqkv, w_phi, wo):
        B, S, D = x.shape
        H = 32
        Dh = D // H
        qkv = (lambda x, *d: x.transpose(*d))((x @ wqkv).reshape(B, S, 3, H, Dh), 2, 0, 3, 1, 4)
        q, k, v = (qkv[0], qkv[1], qkv[2])
        pq = jnp.einsum('bhsd,hdf->bhsf', q, w_phi)
        pk = jnp.einsum('bhsd,hdf->bhsf', k, w_phi)
        phi_q = jnp.concatenate([_softmax(pq, axis=-1), _softmax(-pq, axis=-1)], axis=-1)
        phi_k = jnp.concatenate([_softmax(pk, axis=-1), _softmax(-pk, axis=-1)], axis=-1)
        kv = jnp.einsum('bhsf,bhsd->bhfd', phi_k, v)
        z = jnp.einsum('bhsf->bhf', phi_k)
        num = jnp.einsum('bhqf,bhfd->bhqd', phi_q, kv)
        den = jnp.einsum('bhqf,bhf->bhq', phi_q, z)[..., None] + 1e-06
        o = num / den
        return (lambda x, *d: x.transpose(*d))(o, 0, 2, 1, 3).reshape(B, S, D) @ wo
    x = A_x
    x = x + _A_ref(_layernorm(x, axis=-1), A_mem0, A_Wq, A_Wk, A_Wv, A_Wo, A_seg_len)
    x = x + _B_ref(_layernorm(x, axis=-1), B_wqkv, B_w_phi, B_wo)
    x = x + _A_ref(_layernorm(x, axis=-1), A_mem0, A_Wq, A_Wk, A_Wv, A_Wo, A_seg_len)
    x = x + _B_ref(_layernorm(x, axis=-1), B_wqkv, B_w_phi, B_wo)
    return x
```

```python
import functools
import math

import jax
import jax.numpy as jnp
from jax import lax
import jax.experimental.pallas as pl
import jax.experimental.pallas.tpu as pltpu

F32 = jnp.float32
BF16 = jnp.bfloat16
U32 = jnp.uint32
I32 = jnp.int32

LN_EPS = 1e-5
DEN_EPS = 1e-6
LOG2E = math.log2(math.e)


def _nn(a, b):
    return lax.dot_general(a, b, (((1,), (0,)), ((), ())), preferred_element_type=F32)


def _nt(a, b):
    return lax.dot_general(a, b, (((1,), (1,)), ((), ())), preferred_element_type=F32)


def _unpack(x):
    return pltpu.bitcast(x, BF16)


def _pack(x):
    return pltpu.bitcast(x, U32)


def _iota(shape, dim):
    return lax.broadcasted_iota(I32, shape, dim)


def _layernorm(x):
    inv_n = 1.0 / x.shape[-1]
    m = jnp.sum(x, axis=-1, keepdims=True) * inv_n
    d = x - m
    v = jnp.sum(d * d, axis=-1, keepdims=True) * inv_n
    return d * lax.rsqrt(v + LN_EPS)


def _pair_blockdiag(x, dh):
    rows, width = x.shape
    top, bot = [], []
    zero = jnp.zeros((rows, 128), F32)
    for c in range(0, width, 128):
        t = x[:, c:c + 128]
        if c + 128 <= dh:
            top.append(t)
            bot.append(zero)
        elif c >= dh:
            top.append(zero)
            bot.append(t)
        else:
            first = _iota((rows, 128), 1) < dh - c
            top.append(jnp.where(first, t, 0.0))
            bot.append(jnp.where(first, 0.0, t))
    return jnp.concatenate(
        [jnp.concatenate(top, axis=1), jnp.concatenate(bot, axis=1)], axis=0
    ).astype(BF16)


def _pair_softmax(s, n_mem, scale):
    rows = s.shape[0]
    row = _iota(s.shape, 0)
    col = _iota(s.shape, 1)
    is_a = col < rows
    key = jnp.where(is_a, col, col - rows)
    s = jnp.where((row < n_mem) | (row >= key), s * scale, -1000000000.0)
    ma = jnp.max(jnp.where(is_a, s, -jnp.inf), axis=1, keepdims=True)
    mb = jnp.max(jnp.where(is_a, -jnp.inf, s), axis=1, keepdims=True)
    e = jnp.exp(s - jnp.where(is_a, ma, mb))
    la = jnp.sum(jnp.where(is_a, e, 0.0), axis=1, keepdims=True)
    lb = jnp.sum(jnp.where(is_a, 0.0, e), axis=1, keepdims=True)
    return e / jnp.where(is_a, la, lb)


def _feature_map(p):
    parts = [p[i:i + 8] for i in range(0, p.shape[0], 8)]

    def allreduce(vals, op):
        r = functools.reduce(op, vals)
        r = op(r, pltpu.roll(r, 4, 0))
        return op(r, pltpu.roll(r, 2, 0))

    hi = allreduce(parts, jnp.maximum)
    lo = allreduce(parts, jnp.minimum)
    ep = [jnp.exp2(v - hi) for v in parts]
    en = [jnp.exp2(lo - v) for v in parts]
    rp = 1.0 / allreduce(ep, jnp.add)
    rn = 1.0 / allreduce(en, jnp.add)
    return jnp.concatenate([v * rp for v in ep] + [v * rn for v in en], axis=0).astype(BF16)


def _kernel(x_hbm, mem0_ref, wq_hbm, wk_hbm, wv_hbm, wo_hbm, bqkv_hbm, wphi_ref, bwo_hbm,
            out_hbm,
            stage, wo_stage, wqkv, wo, xio, bqkv_stage, bwo_stage, bw1, bwq, bwo,
            xres, xn_a, xn_b, o_scr, kv_acc, kv_mat,
            w_sem, b_sem, out_sem,
            *, seg, dh, n_layers, tb):
    n_pairs = wqkv.shape[0]
    pw = 2 * dh
    half = pw // 2
    seq, dm = xres.shape
    n_mem = mem0_ref.shape[0]
    n_seg = seq // seg
    scale = dh ** -0.5
    bdh, _, bh = wphi_ref.shape
    n_grp = bh // 2
    gw = 2 * bdh

    def weight_copies(p):
        rows = pl.ds(pl.multiple_of(p * pw, pw), pw)
        return [pltpu.make_async_copy(src.at[rows], stage.at[i, rows], w_sem.at[i, p])
                for i, src in enumerate((wq_hbm, wk_hbm, wv_hbm))] + [
            pltpu.make_async_copy(wo_hbm.at[rows], wo_stage.at[rows], w_sem.at[3, p])]

    x_copy = pltpu.make_async_copy(x_hbm, xio, b_sem.at[0])
    bqkv_copy = pltpu.make_async_copy(bqkv_hbm, bqkv_stage, b_sem.at[1])
    bwo_copy = pltpu.make_async_copy(bwo_hbm, bwo_stage, b_sem.at[2])
    x_copy.start()
    bqkv_copy.start()
    bwo_copy.start()
    ahead = 3
    for p in range(ahead):
        for c in weight_copies(p):
            c.start()

    x_copy.wait()

    def widen(i, carry):
        rows = pl.ds(pl.multiple_of(i * 256, 256), 256)
        xres[rows, :] = xio[rows, :].astype(F32)
        return carry

    lax.fori_loop(0, seq // 256, widen, 0)

    wphi = wphi_ref[...].astype(F32)
    wf = jnp.concatenate([wphi[d] for d in range(bdh)], axis=1)
    src = _iota((dm, dm), 0)
    dst = _iota((dm, dm), 1)
    to_natural = ((src % bh) * bdh + src // bh == dst).astype(BF16)
    wf = _nn(wf, to_natural)
    wf = jnp.concatenate([wf, jnp.zeros((128 - bdh, dm), F32)], axis=0).astype(BF16)
    pick = ((_iota((dm, 128), 0) % gw) // 2 == _iota((dm, 128), 1)).astype(BF16)
    head = (src // gw) * 2 + src % 2
    fold = jnp.where(head == dst // bdh, _nn(pick, wf), 0.0).astype(BF16)
    bqkv_copy.wait()
    bwq[...] = _nt(fold, bqkv_stage[:, :dm]) * LOG2E
    wpk = _nt(fold, bqkv_stage[:, dm:2 * dm]) * LOG2E
    wvt = bqkv_stage[:, 2 * dm:].astype(F32).T
    for g in range(n_grp):
        bw1[2 * g * gw:(2 * g + 1) * gw, :] = wpk[g * gw:(g + 1) * gw]
        bw1[(2 * g + 1) * gw:(2 * g + 2) * gw, :] = wvt[g * gw:(g + 1) * gw]
    bwo_copy.wait()
    bwo[...] = _pack(bwo_stage[...])

    def load_pair(p, carry):
        @pl.when(p + ahead < n_pairs)
        def _():
            for c in weight_copies(p + ahead):
                c.start()

        rows = pl.ds(pl.multiple_of(p * pw, pw), pw)
        copies = weight_copies(p)
        for i in range(3):
            copies[i].wait()
            wqkv[p, :, i * pw:(i + 1) * pw] = _pack(stage[i, rows, :].T)
        copies[3].wait()
        wo[pl.ds(pl.multiple_of(p * half, half), half), :] = _pack(wo_stage[rows, :])
        return carry

    lax.fori_loop(0, n_pairs, load_pair, 0)

    def seg_rows(s):
        return pl.ds(pl.multiple_of(s * seg, seg), seg)

    def rmt_step(s, mem):
        h = jnp.concatenate([mem, xn_a[...]], axis=0)
        xn_next = _layernorm(xres[seg_rows(jnp.minimum(s + 1, n_seg - 1)), :])
        prev = seg_rows(jnp.maximum(s - 1, 0))
        xn_b[prev, :] = _layernorm(xres[prev, :]).astype(BF16)

        lag = n_pairs // 2
        qkv, prob = {}, {}
        acc, done = None, 0

        def out_proj(acc, lo, hi):
            t = _nn(o_scr[:, lo * pw:hi * pw], _unpack(wo[lo * half:hi * half, :]))
            return t if acc is None else acc + t

        for p in range(n_pairs + 2):
            if p < n_pairs:
                qkv[p] = _nn(h, _unpack(wqkv[p]))
            left = n_pairs - 2 - done
            n = 0 if p < lag else 1 if p < n_pairs else (left + 1) // 2 if p == n_pairs else left
            if n:
                acc = out_proj(acc, done, done + n)
                done += n
            if 0 <= p - 1 < n_pairs:
                t = qkv[p - 1]
                scores = _nt(t[:, :pw], _pair_blockdiag(t[:, pw:2 * pw], dh))
                prob[p - 1] = _pair_softmax(scores, n_mem, scale)
            if 0 <= p - 2 < n_pairs:
                o_scr[:, (p - 2) * pw:(p - 1) * pw] = _nn(
                    prob[p - 2], _pair_blockdiag(qkv[p - 2][:, 2 * pw:], dh))
        acc = out_proj(acc, done, n_pairs)
        xn_a[...] = xn_next
        rows = seg_rows(s)
        xres[rows, :] = xres[rows, :] + acc[n_mem:]
        return acc[:n_mem]

    def rmt_layer():
        xn_a[...] = _layernorm(xres[0:seg, :])
        lax.fori_loop(0, n_seg, rmt_step, mem0_ref[...].astype(F32))
        last = slice(seq - seg, seq)
        xn_b[last, :] = _layernorm(xres[last, :]).astype(BF16)

    chunk = 4
    n_chunk = n_grp // chunk

    def blk_rows(i):
        return pl.ds(pl.multiple_of(i * tb, tb), tb)

    def kv_block(i, carry):
        xn = xn_b[blk_rows(i), :]
        ones = jnp.ones((8, tb), F32)
        proj = {}
        for c in range(n_chunk + 1):
            if c < n_chunk:
                proj[c] = _nt(bw1[2 * c * chunk * gw:2 * (c + 1) * chunk * gw, :], xn)
            if c >= 1:
                t = proj[c - 1]
                for j in range(chunk):
                    g = (c - 1) * chunk + j
                    phi = _feature_map(t[2 * j * gw:(2 * j + 1) * gw])
                    lhs = jnp.concatenate([t[(2 * j + 1) * gw:(2 * j + 2) * gw], ones], axis=0)
                    kv_acc[g] += _nt(lhs, phi)
        return carry

    def out_copy(i):
        return pltpu.make_async_copy(xio.at[blk_rows(i)], out_hbm.at[blk_rows(i)], out_sem.at[i])

    def out_block(i, layer):
        rows = blk_rows(i)
        xn = xn_b[rows, :]
        first8 = _iota((8, tb), 0) < 4
        proj, outs = {}, []
        for c in range(n_chunk + 1):
            if c < n_chunk:
                proj[c] = _nt(bwq[c * chunk * gw:(c + 1) * chunk * gw, :], xn)
            if c >= 1:
                t = proj[c - 1]
                for j in range(chunk):
                    g = (c - 1) * chunk + j
                    nd = _nn(kv_mat[g], _feature_map(t[j * gw:(j + 1) * gw]))
                    inv = 1.0 / (nd[gw:] + DEN_EPS)
                    swapped = pltpu.roll(inv, 4, 0)
                    inv_a = jnp.where(first8, inv, swapped)
                    inv_b = jnp.where(first8, swapped, inv)
                    outs.append(nd[:gw] * jnp.concatenate([inv_a, inv_a, inv, inv_b, inv_b], axis=0))
        o = jnp.concatenate(outs, axis=0).astype(BF16).T
        y = xres[rows, :] + _nn(o, _unpack(bwo[...]))
        xres[rows, :] = y
        xio[rows, :] = y.astype(BF16)

        @pl.when(layer == n_layers - 1)
        def _():
            out_copy(i).start()

        return layer

    def hedgehog_layer(layer):
        kv_acc[...] = jnp.zeros(kv_acc.shape, F32)
        lax.fori_loop(0, seq // tb, kv_block, 0)
        shape = kv_acc.shape[1:]
        r = _iota(shape, 0)
        row_head = jnp.where(r < gw, r // bdh, (r - gw) // 4)
        same_head = row_head == _iota(shape, 1) % 2
        for g in range(n_grp):
            kv_mat[g] = jnp.where(same_head, kv_acc[g], 0.0)
        lax.fori_loop(0, seq // tb, out_block, layer)

    def layer_pair(layer, carry):
        with jax.named_scope("rmt"):
            rmt_layer()
        with jax.named_scope("hedgehog"):
            hedgehog_layer(layer)
        return carry

    lax.fori_loop(0, n_layers, layer_pair, 0)
    for i in range(seq // tb):
        out_copy(i).wait()


@functools.partial(jax.jit, static_argnames=("A_seg_len",))
def pallas_interleave_layers__memory_aug_recurrent_mem_tr__linear_kernel_hedgehog__prompt_kernel(
    A_x: jax.Array,
    A_mem0: jax.Array,
    A_Wq: jax.Array,
    A_Wk: jax.Array,
    A_Wv: jax.Array,
    A_Wo: jax.Array,
    A_seg_len: int,
    B_x: jax.Array,
    B_wqkv: jax.Array,
    B_w_phi: jax.Array,
    B_wo: jax.Array,
):
    del B_x
    batch, seq, dm = A_x.shape
    _, heads, dh = A_Wq.shape
    n_mem = A_mem0.shape[1]
    bh, bdh, _ = B_w_phi.shape
    seg = int(A_seg_len)
    assert batch == 1 and bdh == 20 and bh * bdh == dm and heads % 2 == 0
    assert (2 * dh) % 128 == 0 and n_mem % 8 == 0 and seg % 16 == 0 and 2 * (n_mem + seg) <= 128
    n_pairs, pw, hd = heads // 2, 2 * dh, heads * dh
    tb = 512

    def feature_major(w):
        return jnp.transpose(w, (1, 2, 0)).reshape(hd, dm)

    hbm = pl.BlockSpec(memory_space=pl.ANY)
    vmem = pl.BlockSpec(memory_space=pltpu.VMEM)
    out = pl.pallas_call(
        functools.partial(_kernel, seg=seg, dh=dh, n_layers=2, tb=tb),
        out_shape=jax.ShapeDtypeStruct((seq, dm), A_x.dtype),
        in_specs=[hbm, vmem, hbm, hbm, hbm, hbm, hbm, vmem, hbm],
        out_specs=hbm,
        scratch_shapes=[
            pltpu.VMEM((3, hd, dm), BF16),
            pltpu.VMEM((hd, dm), BF16),
            pltpu.VMEM((n_pairs, dm // 2, 3 * pw), U32),
            pltpu.VMEM((hd // 2, dm), U32),
            pltpu.VMEM((seq, dm), BF16),
            pltpu.VMEM((dm, 3 * dm), BF16),
            pltpu.VMEM((dm, dm), BF16),
            pltpu.VMEM((2 * dm, dm), F32),
            pltpu.VMEM((dm, dm), F32),
            pltpu.VMEM((dm // 2, dm), U32),
            pltpu.VMEM((seq, dm), F32),
            pltpu.VMEM((seg, dm), F32),
            pltpu.VMEM((seq, dm), BF16),
            pltpu.VMEM((n_mem + seg, hd), F32),
            pltpu.VMEM((bh // 2, 2 * bdh + 8, 4 * bdh), F32),
            pltpu.VMEM((bh // 2, 2 * bdh + 8, 4 * bdh), F32),
            pltpu.SemaphoreType.DMA((4, n_pairs)),
            pltpu.SemaphoreType.DMA((3,)),
            pltpu.SemaphoreType.DMA((seq // tb,)),
        ],
        compiler_params=pltpu.CompilerParams(vmem_limit_bytes=112 * 1024 * 1024),
        name="rmt_hedgehog",
    )(
        A_x.reshape(seq, dm),
        A_mem0.reshape(n_mem, dm),
        feature_major(A_Wq),
        feature_major(A_Wk),
        feature_major(A_Wv),
        A_Wo.reshape(hd, dm),
        B_wqkv,
        jnp.transpose(B_w_phi, (1, 2, 0)),
        B_wo,
    )
    return out.reshape(batch, seq, dm)
```

```python
import functools
import math

import jax
import jax.numpy as jnp
from jax import lax
import jax.experimental.pallas as pl
import jax.experimental.pallas.tpu as pltpu

F32 = jnp.float32
BF16 = jnp.bfloat16
U32 = jnp.uint32
I32 = jnp.int32

LN_EPS = 1e-5
DEN_EPS = 1e-6
LOG2E = math.log2(math.e)
EARLY_ROWS = 8


def _nn(a, b):
    return lax.dot_general(a, b, (((1,), (0,)), ((), ())), preferred_element_type=F32)


def _nt(a, b):
    return lax.dot_general(a, b, (((1,), (1,)), ((), ())), preferred_element_type=F32)


def _unpack(x):
    return pltpu.bitcast(x, BF16)


def _pack(x):
    return pltpu.bitcast(x, U32)


def _iota(shape, dim):
    return lax.broadcasted_iota(I32, shape, dim)


def _layernorm(x):
    inv_n = 1.0 / x.shape[-1]
    m = jnp.sum(x, axis=-1, keepdims=True) * inv_n
    d = x - m
    v = jnp.sum(d * d, axis=-1, keepdims=True) * inv_n
    return d * lax.rsqrt(v + LN_EPS)


def _pair_blockdiag(x, dh):
    rows, width = x.shape
    top, bot = [], []
    zero = jnp.zeros((rows, 128), F32)
    for c in range(0, width, 128):
        t = x[:, c:c + 128]
        if c + 128 <= dh:
            top.append(t)
            bot.append(zero)
        elif c >= dh:
            top.append(zero)
            bot.append(t)
        else:
            first = _iota((rows, 128), 1) < dh - c
            top.append(jnp.where(first, t, 0.0))
            bot.append(jnp.where(first, 0.0, t))
    return jnp.concatenate(
        [jnp.concatenate(top, axis=1), jnp.concatenate(bot, axis=1)], axis=0
    ).astype(BF16)


def _pair_softmax(s, n_mem, scale):
    rows = s.shape[0]
    row = _iota(s.shape, 0)
    col = _iota(s.shape, 1)
    is_a = col < rows
    key = jnp.where(is_a, col, col - rows)
    s = jnp.where((row < n_mem) | (row >= key), s * scale, -1000000000.0)
    ma = jnp.max(jnp.where(is_a, s, -jnp.inf), axis=1, keepdims=True)
    mb = jnp.max(jnp.where(is_a, -jnp.inf, s), axis=1, keepdims=True)
    e = jnp.exp(s - jnp.where(is_a, ma, mb))
    la = jnp.sum(jnp.where(is_a, e, 0.0), axis=1, keepdims=True)
    lb = jnp.sum(jnp.where(is_a, 0.0, e), axis=1, keepdims=True)
    return e / jnp.where(is_a, la, lb)


def _feature_map(p):
    parts = [p[i:i + 8] for i in range(0, p.shape[0], 8)]

    def allreduce(vals, op):
        r = functools.reduce(op, vals)
        r = op(r, pltpu.roll(r, 4, 0))
        return op(r, pltpu.roll(r, 2, 0))

    hi = allreduce(parts, jnp.maximum)
    lo = allreduce(parts, jnp.minimum)
    ep = [jnp.exp2(v - hi) for v in parts]
    en = [jnp.exp2(lo - v) for v in parts]
    rp = 1.0 / allreduce(ep, jnp.add)
    rn = 1.0 / allreduce(en, jnp.add)
    return jnp.concatenate([v * rp for v in ep] + [v * rn for v in en], axis=0).astype(BF16)


def _kernel(x_hbm, mem0_ref, wq_hbm, wk_hbm, wv_hbm, wo_hbm, bqkv_hbm, wphi_ref, bwo_hbm,
            out_hbm,
            stage, wo_stage, wqkv, wo, xio, bqkv_stage, bwo_stage, bw1, bwq, bwo,
            xres, xn_a, xn_b, o_scr, kv_acc, kv_mat, early_xn, early_qkv,
            w_sem, b_sem, out_sem,
            *, seg, dh, n_layers, tb, unroll):
    n_pairs = wqkv.shape[0]
    pw = 2 * dh
    half = pw // 2
    seq, dm = xres.shape
    n_mem = mem0_ref.shape[0]
    n_seg = seq // seg
    scale = dh ** -0.5
    bdh, _, bh = wphi_ref.shape
    n_grp = bh // 2
    gw = 2 * bdh
    n_early = early_xn.shape[0] // EARLY_ROWS

    def pair_rows(p):
        return pl.ds(pl.multiple_of(p * pw, pw), pw)

    def qkv_copies(p):
        return [pltpu.make_async_copy(src.at[pair_rows(p)], stage.at[i, pair_rows(p)], w_sem.at[i, p])
                for i, src in enumerate((wq_hbm, wk_hbm, wv_hbm))]

    def wo_copy(p):
        return pltpu.make_async_copy(wo_hbm.at[pair_rows(p)], wo_stage.at[pair_rows(p)], w_sem.at[3, p])

    x_copy = pltpu.make_async_copy(x_hbm, xio, b_sem.at[0])
    bqkv_copy = pltpu.make_async_copy(bqkv_hbm, bqkv_stage, b_sem.at[1])
    bwo_copy = pltpu.make_async_copy(bwo_hbm, bwo_stage, b_sem.at[2])
    bqkv_copy.start()
    x_copy.start()
    ahead = 3
    for p in range(ahead):
        for c in qkv_copies(p):
            c.start()
        wo_copy(p).start()
    bwo_copy.start()

    wphi = wphi_ref[...].astype(F32)
    wf = jnp.concatenate([wphi[d] for d in range(bdh)], axis=1)
    src = _iota((dm, dm), 0)
    dst = _iota((dm, dm), 1)
    to_natural = ((src % bh) * bdh + src // bh == dst).astype(BF16)
    wf = _nn(wf, to_natural)
    wf = jnp.concatenate([wf, jnp.zeros((128 - bdh, dm), F32)], axis=0).astype(BF16)
    pick = ((_iota((dm, 128), 0) % gw) // 2 == _iota((dm, 128), 1)).astype(BF16)
    head = (src // gw) * 2 + src % 2
    fold = jnp.where(head == dst // bdh, _nn(pick, wf), 0.0).astype(BF16)
    bqkv_copy.wait()
    bwq[...] = _nt(fold, bqkv_stage[:, :dm]) * LOG2E
    wpk = _nt(fold, bqkv_stage[:, dm:2 * dm]) * LOG2E
    wvt = bqkv_stage[:, 2 * dm:].astype(F32).T
    for g in range(n_grp):
        bw1[2 * g * gw:(2 * g + 1) * gw, :] = wpk[g * gw:(g + 1) * gw]
        bw1[(2 * g + 1) * gw:(2 * g + 2) * gw, :] = wvt[g * gw:(g + 1) * gw]

    x_copy.wait()

    def widen(i, carry):
        rows = pl.ds(pl.multiple_of(i * 256, 256), 256)
        xres[rows, :] = xio[rows, :].astype(F32)
        return carry

    lax.fori_loop(0, seq // 256, widen, 0)
    early_xn[...] = _layernorm(jnp.concatenate(
        [xres[(s + 1) * seg - EARLY_ROWS:(s + 1) * seg, :] for s in range(n_early)], axis=0)).astype(BF16)

    def load_pair(p, carry):
        @pl.when(p + ahead < n_pairs)
        def _():
            for c in qkv_copies(p + ahead):
                c.start()
            wo_copy(p + ahead).start()

        for c in qkv_copies(p):
            c.wait()
        wo_copy(p).wait()
        for i in range(3):
            w = stage[i, pair_rows(p), :]
            early_qkv[p, :, i * pw:(i + 1) * pw] = _nt(early_xn[...], w)
            wqkv[p, :, i * pw:(i + 1) * pw] = _pack(w.T)
        wo[pl.ds(pl.multiple_of(p * half, half), half), :] = _pack(wo_stage[pair_rows(p), :])
        return carry

    with jax.named_scope("load"):
        lax.fori_loop(0, n_pairs, load_pair, 0)
    bwo_copy.wait()
    bwo[...] = _pack(bwo_stage[...])

    def seg_rows(s):
        return pl.ds(pl.multiple_of(s * seg, seg), seg)

    def rmt_step(s, mem, early):
        if early:
            h = jnp.concatenate([mem, xn_a[:seg - EARLY_ROWS, :]], axis=0).astype(BF16)
            early_rows = pl.ds(pl.multiple_of(s * EARLY_ROWS, EARLY_ROWS), EARLY_ROWS)
        else:
            h = jnp.concatenate([mem, xn_a[...]], axis=0)
        xn_next = _layernorm(xres[seg_rows(jnp.minimum(s + 1, n_seg - 1)), :])
        prev = seg_rows(jnp.maximum(s - 1, 0))
        xn_b[prev, :] = _layernorm(xres[prev, :]).astype(BF16)

        lag, tail = n_pairs // 2, 2
        qkv, prob = {}, {}
        acc, done = None, 0

        def out_proj(acc, lo, hi):
            t = _nn(o_scr[:, lo * pw:hi * pw], _unpack(wo[lo * half:hi * half, :]))
            return t if acc is None else acc + t

        for p in range(n_pairs + 2):
            if p < n_pairs:
                qkv[p] = _nn(h, _unpack(wqkv[p]))
                if early:
                    qkv[p] = jnp.concatenate([qkv[p], early_qkv[p, early_rows, :]], axis=0)
            left = n_pairs - tail - done
            n = 0 if p < lag else 1 if p < n_pairs else (left + 1) // 2 if p == n_pairs else left
            if n:
                acc = out_proj(acc, done, done + n)
                done += n
            if 0 <= p - 1 < n_pairs:
                t = qkv[p - 1]
                scores = _nt(t[:, :pw], _pair_blockdiag(t[:, pw:2 * pw], dh))
                prob[p - 1] = _pair_softmax(scores, n_mem, scale)
            if 0 <= p - 2 < n_pairs:
                o_scr[:, (p - 2) * pw:(p - 1) * pw] = _nn(
                    prob[p - 2], _pair_blockdiag(qkv[p - 2][:, 2 * pw:], dh))
        for p in range(done, n_pairs):
            acc = out_proj(acc, p, p + 1)
        xn_a[...] = xn_next
        rows = seg_rows(s)
        xres[rows, :] = xres[rows, :] + acc[n_mem:]
        return acc[:n_mem]

    def rmt_steps(lo, hi, mem, early):
        def body(i, mem):
            for u in range(unroll):
                mem = rmt_step(i * unroll + u, mem, early)
            return mem

        return lax.fori_loop(lo, hi, body, mem)

    def rmt_layer(layer):
        xn_a[...] = _layernorm(xres[0:seg, :])
        split = jnp.where(layer == 0, n_early // unroll, 0)
        mem = rmt_steps(0, split, mem0_ref[...].astype(F32), True)
        rmt_steps(split, n_seg // unroll, mem, False)
        last = slice(seq - seg, seq)
        xn_b[last, :] = _layernorm(xres[last, :]).astype(BF16)

    chunk = 4
    n_chunk = n_grp // chunk

    def blk_rows(i):
        return pl.ds(pl.multiple_of(i * tb, tb), tb)

    def kv_block(i, carry):
        xn = xn_b[blk_rows(i), :]
        ones = jnp.ones((8, tb), F32)
        proj = {}
        for c in range(n_chunk + 1):
            if c < n_chunk:
                proj[c] = _nt(bw1[2 * c * chunk * gw:2 * (c + 1) * chunk * gw, :], xn)
            if c >= 1:
                t = proj[c - 1]
                for j in range(chunk):
                    g = (c - 1) * chunk + j
                    phi = _feature_map(t[2 * j * gw:(2 * j + 1) * gw])
                    lhs = jnp.concatenate([t[(2 * j + 1) * gw:(2 * j + 2) * gw], ones], axis=0)
                    kv_acc[g] += _nt(lhs, phi)
        return carry

    def out_copy(i):
        return pltpu.make_async_copy(xio.at[blk_rows(i)], out_hbm.at[blk_rows(i)], out_sem.at[i])

    def out_block(i, layer):
        rows = blk_rows(i)
        xn = xn_b[rows, :]
        first8 = _iota((8, tb), 0) < 4
        proj, outs = {}, []
        for c in range(n_chunk + 1):
            if c < n_chunk:
                proj[c] = _nt(bwq[c * chunk * gw:(c + 1) * chunk * gw, :], xn)
            if c >= 1:
                t = proj[c - 1]
                for j in range(chunk):
                    g = (c - 1) * chunk + j
                    nd = _nn(kv_mat[g], _feature_map(t[j * gw:(j + 1) * gw]))
                    inv = 1.0 / (nd[gw:] + DEN_EPS)
                    swapped = pltpu.roll(inv, 4, 0)
                    inv_a = jnp.where(first8, inv, swapped)
                    inv_b = jnp.where(first8, swapped, inv)
                    outs.append(nd[:gw] * jnp.concatenate([inv_a, inv_a, inv, inv_b, inv_b], axis=0))
        o = jnp.concatenate(outs, axis=0).astype(BF16).T
        y = xres[rows, :] + _nn(o, _unpack(bwo[...]))
        xres[rows, :] = y
        xio[rows, :] = y.astype(BF16)

        @pl.when(layer == n_layers - 1)
        def _():
            out_copy(i).start()

        return layer

    def hedgehog_layer(layer):
        kv_acc[...] = jnp.zeros(kv_acc.shape, F32)
        lax.fori_loop(0, seq // tb, kv_block, 0)
        shape = kv_acc.shape[1:]
        r = _iota(shape, 0)
        row_head = jnp.where(r < gw, r // bdh, (r - gw) // 4)
        same_head = row_head == _iota(shape, 1) % 2
        for g in range(n_grp):
            kv_mat[g] = jnp.where(same_head, kv_acc[g], 0.0)
        lax.fori_loop(0, seq // tb, out_block, layer)

    def layer_pair(layer, carry):
        with jax.named_scope("rmt"):
            rmt_layer(layer)
        with jax.named_scope("hedgehog"):
            hedgehog_layer(layer)
        return carry

    lax.fori_loop(0, n_layers, layer_pair, 0)
    for i in range(seq // tb):
        out_copy(i).wait()


@functools.partial(jax.jit, static_argnames=("A_seg_len",))
def pallas_interleave_layers__memory_aug_recurrent_mem_tr__linear_kernel_hedgehog__prompt_kernel(
    A_x: jax.Array,
    A_mem0: jax.Array,
    A_Wq: jax.Array,
    A_Wk: jax.Array,
    A_Wv: jax.Array,
    A_Wo: jax.Array,
    A_seg_len: int,
    B_x: jax.Array,
    B_wqkv: jax.Array,
    B_w_phi: jax.Array,
    B_wo: jax.Array,
):
    del B_x
    batch, seq, dm = A_x.shape
    _, heads, dh = A_Wq.shape
    n_mem = A_mem0.shape[1]
    bh, bdh, _ = B_w_phi.shape
    seg = int(A_seg_len)
    assert batch == 1 and bdh == 20 and bh * bdh == dm and heads % 2 == 0
    assert (2 * dh) % 128 == 0 and n_mem % 8 == 0 and seg % 16 == 0 and 2 * (n_mem + seg) <= 128
    n_pairs, pw, hd = heads // 2, 2 * dh, heads * dh
    tb, unroll, n_early = 512, 1, 40

    def feature_major(w):
        return jnp.transpose(w, (1, 2, 0)).reshape(hd, dm)

    hbm = pl.BlockSpec(memory_space=pl.ANY)
    vmem = pl.BlockSpec(memory_space=pltpu.VMEM)
    out = pl.pallas_call(
        functools.partial(_kernel, seg=seg, dh=dh, n_layers=2, tb=tb, unroll=unroll),
        out_shape=jax.ShapeDtypeStruct((seq, dm), A_x.dtype),
        in_specs=[hbm, vmem, hbm, hbm, hbm, hbm, hbm, vmem, hbm],
        out_specs=hbm,
        scratch_shapes=[
            pltpu.VMEM((3, hd, dm), BF16),
            pltpu.VMEM((hd, dm), BF16),
            pltpu.VMEM((n_pairs, dm // 2, 3 * pw), U32),
            pltpu.VMEM((hd // 2, dm), U32),
            pltpu.VMEM((seq, dm), BF16),
            pltpu.VMEM((dm, 3 * dm), BF16),
            pltpu.VMEM((dm, dm), BF16),
            pltpu.VMEM((2 * dm, dm), F32),
            pltpu.VMEM((dm, dm), F32),
            pltpu.VMEM((dm // 2, dm), U32),
            pltpu.VMEM((seq, dm), F32),
            pltpu.VMEM((seg, dm), F32),
            pltpu.VMEM((seq, dm), BF16),
            pltpu.VMEM((n_mem + seg, hd), F32),
            pltpu.VMEM((bh // 2, 2 * bdh + 8, 4 * bdh), F32),
            pltpu.VMEM((bh // 2, 2 * bdh + 8, 4 * bdh), F32),
            pltpu.VMEM((n_early * EARLY_ROWS, dm), BF16),
            pltpu.VMEM((n_pairs, n_early * EARLY_ROWS, 3 * pw), F32),
            pltpu.SemaphoreType.DMA((4, n_pairs)),
            pltpu.SemaphoreType.DMA((3,)),
            pltpu.SemaphoreType.DMA((seq // tb,)),
        ],
        compiler_params=pltpu.CompilerParams(vmem_limit_bytes=120 * 1024 * 1024),
        name="rmt_hedgehog",
    )(
        A_x.reshape(seq, dm),
        A_mem0.reshape(n_mem, dm),
        feature_major(A_Wq),
        feature_major(A_Wk),
        feature_major(A_Wv),
        A_Wo.reshape(hd, dm),
        B_wqkv,
        jnp.transpose(B_w_phi, (1, 2, 0)),
        B_wo,
    )
    return out.reshape(batch, seq, dm)
```

```python
import functools
import math

import jax
import jax.numpy as jnp
from jax import lax
import jax.experimental.pallas as pl
import jax.experimental.pallas.tpu as pltpu

F32 = jnp.float32
BF16 = jnp.bfloat16
U32 = jnp.uint32
I32 = jnp.int32

LN_EPS = 1e-5
DEN_EPS = 1e-6
LOG2E = math.log2(math.e)
EARLY_ROWS = 8


def _nn(a, b):
    return lax.dot_general(a, b, (((1,), (0,)), ((), ())), preferred_element_type=F32)


def _nt(a, b):
    return lax.dot_general(a, b, (((1,), (1,)), ((), ())), preferred_element_type=F32)


def _unpack(x):
    return pltpu.bitcast(x, BF16)


def _pack(x):
    return pltpu.bitcast(x, U32)


def _iota(shape, dim):
    return lax.broadcasted_iota(I32, shape, dim)


def _layernorm(x):
    inv_n = 1.0 / x.shape[-1]
    m = jnp.sum(x, axis=-1, keepdims=True) * inv_n
    d = x - m
    v = jnp.sum(d * d, axis=-1, keepdims=True) * inv_n
    return d * lax.rsqrt(v + LN_EPS)


def _pair_blockdiag(x, dh):
    rows, width = x.shape
    top, bot = [], []
    zero = jnp.zeros((rows, 128), F32)
    for c in range(0, width, 128):
        t = x[:, c:c + 128]
        if c + 128 <= dh:
            top.append(t)
            bot.append(zero)
        elif c >= dh:
            top.append(zero)
            bot.append(t)
        else:
            first = _iota((rows, 128), 1) < dh - c
            top.append(jnp.where(first, t, 0.0))
            bot.append(jnp.where(first, 0.0, t))
    return jnp.concatenate(
        [jnp.concatenate(top, axis=1), jnp.concatenate(bot, axis=1)], axis=0
    ).astype(BF16)


def _pair_softmax(s, n_mem, scale):
    rows = s.shape[0]
    row = _iota(s.shape, 0)
    col = _iota(s.shape, 1)
    is_a = col < rows
    key = jnp.where(is_a, col, col - rows)
    s = jnp.where((row < n_mem) | (row >= key), s * scale, -1000000000.0)
    ma = jnp.max(jnp.where(is_a, s, -jnp.inf), axis=1, keepdims=True)
    mb = jnp.max(jnp.where(is_a, -jnp.inf, s), axis=1, keepdims=True)
    e = jnp.exp(s - jnp.where(is_a, ma, mb))
    la = jnp.sum(jnp.where(is_a, e, 0.0), axis=1, keepdims=True)
    lb = jnp.sum(jnp.where(is_a, 0.0, e), axis=1, keepdims=True)
    return e / jnp.where(is_a, la, lb)


def _feature_map(p):
    parts = [p[i:i + 8] for i in range(0, p.shape[0], 8)]

    def allreduce(vals, op):
        r = functools.reduce(op, vals)
        r = op(r, pltpu.roll(r, 4, 0))
        return op(r, pltpu.roll(r, 2, 0))

    hi = allreduce(parts, jnp.maximum)
    lo = allreduce(parts, jnp.minimum)
    ep = [jnp.exp2(v - hi) for v in parts]
    en = [jnp.exp2(lo - v) for v in parts]
    rp = 1.0 / allreduce(ep, jnp.add)
    rn = 1.0 / allreduce(en, jnp.add)
    return jnp.concatenate([v * rp for v in ep] + [v * rn for v in en], axis=0).astype(BF16)


def _kernel(x_hbm, mem0_ref, wq_hbm, wk_hbm, wv_hbm, wo_hbm, bqkv_hbm, wphi_ref, bwo_hbm,
            out_hbm,
            stage, wqkv, wo, x_stage, out_stage, bqkv_stage, bwo_stage, fold, bw1, bwq, bwo,
            xres, xn_a, xn_b, o_scr, kv_acc, kv_mat, early_x, early_xn, early_qkv,
            w_sem, b_sem, out_sem,
            *, seg, dh, n_layers, tb, unroll):
    n_pairs = wqkv.shape[0]
    pw = 2 * dh
    half = pw // 2
    seq, dm = xres.shape
    n_mem = mem0_ref.shape[0]
    n_seg = seq // seg
    scale = dh ** -0.5
    bdh, _, bh = wphi_ref.shape
    n_grp = bh // 2
    gw = 2 * bdh
    n_early = early_xn.shape[0] // EARLY_ROWS

    x_chunk = n_seg // n_pairs

    def pair_rows(p):
        return pl.ds(pl.multiple_of(p * pw, pw), pw)

    def pair_copies(p):
        rows = pair_rows(p)
        segs = pl.ds(p * x_chunk, x_chunk)
        return [pltpu.make_async_copy(src.at[rows], stage.at[i, rows], w_sem.at[i, p])
                for i, src in enumerate((wq_hbm, wk_hbm, wv_hbm, wo_hbm))] + [
            pltpu.make_async_copy(x_hbm.at[segs], x_stage.at[segs], w_sem.at[4, p])]

    early_copy = pltpu.make_async_copy(
        x_hbm.at[pl.ds(0, n_early), pl.ds(seg - EARLY_ROWS, EARLY_ROWS)], early_x, b_sem.at[0])
    bqkv_copy = pltpu.make_async_copy(bqkv_hbm, bqkv_stage, b_sem.at[1])
    bwo_copy = pltpu.make_async_copy(bwo_hbm, bwo_stage, b_sem.at[2])
    early_copy.start()
    for c in pair_copies(0):
        c.start()

    wphi = wphi_ref[...].astype(F32)
    wf = jnp.concatenate([wphi[d] for d in range(bdh)], axis=1)
    src = _iota((dm, 128), 0)
    natural = (src % bh) * bdh + src // bh
    first_grp = [c // gw for c in range(0, dm, 128)]
    r = _iota((4 * gw, 128), 0)
    lane = _iota((4 * gw, 128), 1)
    pick = ((r % gw) // 2 == lane).astype(BF16)
    head_start = ((r // gw) * 2 + r % 2) * bdh
    for j, g0 in enumerate(first_grp):
        wj = _nn(wf, (natural == _iota((dm, 128), 1) + j * 128).astype(BF16))
        wj = jnp.concatenate([wj, jnp.zeros((128 - bdh, 128), F32)], axis=0).astype(BF16)
        d = lane + (j * 128 - g0 * gw) - head_start
        fold[j] = jnp.where((d >= 0) & (d < bdh), _nn(pick, wj), 0.0).astype(BF16)

    early_copy.wait()
    for c in pair_copies(1):
        c.start()
    early_xn[...] = _layernorm(
        early_x[...].astype(F32).reshape(n_early * EARLY_ROWS, dm)).astype(BF16)

    def load_pair(p, carry):
        for c in pair_copies(p):
            c.wait()

        @pl.when(p + 2 < n_pairs)
        def _():
            for c in pair_copies(p + 2):
                c.start()

        pl.when(p == n_pairs // 2)(bqkv_copy.start)
        pl.when(p == n_pairs - 3)(bwo_copy.start)
        for i in range(3):
            w = stage[i, pair_rows(p), :]
            early_qkv[p, :, i * pw:(i + 1) * pw] = _nt(early_xn[...], w)
            wqkv[p, :, i * pw:(i + 1) * pw] = _pack(w.T)
        wo[pl.ds(pl.multiple_of(p * half, half), half), :] = _pack(stage[3, pair_rows(p), :])
        wide = x_stage[pl.ds(p * x_chunk, x_chunk)].astype(F32).reshape(x_chunk * seg, dm)
        xres[pl.ds(pl.multiple_of(p * x_chunk * seg, x_chunk * seg), x_chunk * seg), :] = wide
        return carry

    with jax.named_scope("load"):
        lax.fori_loop(0, n_pairs, load_pair, 0)

    def fold_phi(base):
        groups = [None] * n_grp
        for j, g0 in enumerate(first_grp):
            t = _nt(fold[j], bqkv_stage[:, base + j * 128:base + (j + 1) * 128]) * LOG2E
            for i in range(4):
                part = t[i * gw:(i + 1) * gw]
                groups[g0 + i] = part if groups[g0 + i] is None else groups[g0 + i] + part
        return groups

    bqkv_copy.wait()
    bwo_copy.wait()
    wvt = bqkv_stage[:, 2 * dm:].astype(F32).T
    for g, (wpq, wpk) in enumerate(zip(fold_phi(0), fold_phi(dm))):
        bwq[g * gw:(g + 1) * gw, :] = wpq
        bw1[2 * g * gw:(2 * g + 1) * gw, :] = wpk
        bw1[(2 * g + 1) * gw:(2 * g + 2) * gw, :] = wvt[g * gw:(g + 1) * gw]
    bwo[...] = _pack(bwo_stage[...])

    def seg_rows(s):
        return pl.ds(pl.multiple_of(s * seg, seg), seg)

    def rmt_step(s, mem, early):
        if early:
            h = jnp.concatenate([mem, xn_a[:seg - EARLY_ROWS, :]], axis=0).astype(BF16)
            early_rows = pl.ds(pl.multiple_of(s * EARLY_ROWS, EARLY_ROWS), EARLY_ROWS)
        else:
            h = jnp.concatenate([mem, xn_a[...]], axis=0)
        xn_next = _layernorm(xres[seg_rows(jnp.minimum(s + 1, n_seg - 1)), :])
        prev = seg_rows(jnp.maximum(s - 1, 0))
        xn_b[prev, :] = _layernorm(xres[prev, :]).astype(BF16)

        lag, tail = n_pairs // 2, 2
        qkv, prob = {}, {}
        acc, done = None, 0

        def out_proj(acc, lo, hi):
            t = _nn(o_scr[:, lo * pw:hi * pw], _unpack(wo[lo * half:hi * half, :]))
            return t if acc is None else acc + t

        for p in range(n_pairs + 2):
            if p < n_pairs:
                qkv[p] = _nn(h, _unpack(wqkv[p]))
                if early:
                    qkv[p] = jnp.concatenate([qkv[p], early_qkv[p, early_rows, :]], axis=0)
            left = n_pairs - tail - done
            n = 0 if p < lag else 1 if p < n_pairs else (left + 1) // 2 if p == n_pairs else left
            if n:
                acc = out_proj(acc, done, done + n)
                done += n
            if 0 <= p - 1 < n_pairs:
                t = qkv[p - 1]
                scores = _nt(t[:, :pw], _pair_blockdiag(t[:, pw:2 * pw], dh))
                prob[p - 1] = _pair_softmax(scores, n_mem, scale)
            if 0 <= p - 2 < n_pairs:
                o_scr[:, (p - 2) * pw:(p - 1) * pw] = _nn(
                    prob[p - 2], _pair_blockdiag(qkv[p - 2][:, 2 * pw:], dh))
        for p in range(done, n_pairs):
            acc = out_proj(acc, p, p + 1)
        xn_a[...] = xn_next
        rows = seg_rows(s)
        xres[rows, :] = xres[rows, :] + acc[n_mem:]
        return acc[:n_mem]

    def rmt_steps(lo, hi, mem, early):
        def body(i, mem):
            for u in range(unroll):
                mem = rmt_step(i * unroll + u, mem, early)
            return mem

        return lax.fori_loop(lo, hi, body, mem)

    def rmt_layer(layer):
        xn_a[...] = _layernorm(xres[0:seg, :])
        split = jnp.where(layer == 0, n_early // unroll, 0)
        mem = rmt_steps(0, split, mem0_ref[...].astype(F32), True)
        rmt_steps(split, n_seg // unroll, mem, False)
        last = slice(seq - seg, seq)
        xn_b[last, :] = _layernorm(xres[last, :]).astype(BF16)

    chunk = 4
    n_chunk = n_grp // chunk

    def blk_rows(i):
        return pl.ds(pl.multiple_of(i * tb, tb), tb)

    def kv_block(i, carry):
        xn = xn_b[blk_rows(i), :]
        ones = jnp.ones((8, tb), F32)
        proj = {}
        for c in range(n_chunk + 1):
            if c < n_chunk:
                proj[c] = _nt(bw1[2 * c * chunk * gw:2 * (c + 1) * chunk * gw, :], xn)
            if c >= 1:
                t = proj[c - 1]
                for j in range(chunk):
                    g = (c - 1) * chunk + j
                    phi = _feature_map(t[2 * j * gw:(2 * j + 1) * gw])
                    lhs = jnp.concatenate([t[(2 * j + 1) * gw:(2 * j + 2) * gw], ones], axis=0)
                    kv_acc[g] += _nt(lhs, phi)
        return carry

    def out_copy(i):
        return pltpu.make_async_copy(out_stage.at[blk_rows(i)], out_hbm.at[blk_rows(i)], out_sem.at[i])

    def out_block(i, layer):
        rows = blk_rows(i)
        xn = xn_b[rows, :]
        first8 = _iota((8, tb), 0) < 4
        proj, outs = {}, []
        for c in range(n_chunk + 1):
            if c < n_chunk:
                proj[c] = _nt(bwq[c * chunk * gw:(c + 1) * chunk * gw, :], xn)
            if c >= 1:
                t = proj[c - 1]
                for j in range(chunk):
                    g = (c - 1) * chunk + j
                    nd = _nn(kv_mat[g], _feature_map(t[j * gw:(j + 1) * gw]))
                    inv = 1.0 / (nd[gw:] + DEN_EPS)
                    swapped = pltpu.roll(inv, 4, 0)
                    inv_a = jnp.where(first8, inv, swapped)
                    inv_b = jnp.where(first8, swapped, inv)
                    outs.append(nd[:gw] * jnp.concatenate([inv_a, inv_a, inv, inv_b, inv_b], axis=0))
        o = jnp.concatenate(outs, axis=0).astype(BF16).T
        y = xres[rows, :] + _nn(o, _unpack(bwo[...]))
        xres[rows, :] = y
        out_stage[rows, :] = y.astype(BF16)

        @pl.when(layer == n_layers - 1)
        def _():
            out_copy(i).start()

        return layer

    def hedgehog_layer(layer):
        kv_acc[...] = jnp.zeros(kv_acc.shape, F32)
        lax.fori_loop(0, seq // tb, kv_block, 0)
        shape = kv_acc.shape[1:]
        r = _iota(shape, 0)
        row_head = jnp.where(r < gw, r // bdh, (r - gw) // 4)
        same_head = row_head == _iota(shape, 1) % 2
        for g in range(n_grp):
            kv_mat[g] = jnp.where(same_head, kv_acc[g], 0.0)
        lax.fori_loop(0, seq // tb, out_block, layer)

    def layer_pair(layer, carry):
        with jax.named_scope("rmt"):
            rmt_layer(layer)
        with jax.named_scope("hedgehog"):
            hedgehog_layer(layer)
        return carry

    lax.fori_loop(0, n_layers, layer_pair, 0)
    for i in range(seq // tb):
        out_copy(i).wait()


@functools.partial(jax.jit, static_argnames=("A_seg_len",))
def pallas_interleave_layers__memory_aug_recurrent_mem_tr__linear_kernel_hedgehog__prompt_kernel(
    A_x: jax.Array,
    A_mem0: jax.Array,
    A_Wq: jax.Array,
    A_Wk: jax.Array,
    A_Wv: jax.Array,
    A_Wo: jax.Array,
    A_seg_len: int,
    B_x: jax.Array,
    B_wqkv: jax.Array,
    B_w_phi: jax.Array,
    B_wo: jax.Array,
):
    del B_x
    batch, seq, dm = A_x.shape
    _, heads, dh = A_Wq.shape
    n_mem = A_mem0.shape[1]
    bh, bdh, _ = B_w_phi.shape
    seg = int(A_seg_len)
    assert batch == 1 and bdh == 20 and bh * bdh == dm and heads % 2 == 0
    assert (2 * dh) % 128 == 0 and n_mem % 8 == 0 and seg % 16 == 0 and 2 * (n_mem + seg) <= 128
    n_pairs, pw, hd = heads // 2, 2 * dh, heads * dh
    tb, unroll, n_early = 512, 1, 48

    def feature_major(w):
        return jnp.transpose(w, (1, 2, 0)).reshape(hd, dm)

    hbm = pl.BlockSpec(memory_space=pl.ANY)
    vmem = pl.BlockSpec(memory_space=pltpu.VMEM)
    out = pl.pallas_call(
        functools.partial(_kernel, seg=seg, dh=dh, n_layers=2, tb=tb, unroll=unroll),
        out_shape=jax.ShapeDtypeStruct((seq, dm), A_x.dtype),
        in_specs=[hbm, vmem, hbm, hbm, hbm, hbm, hbm, vmem, hbm],
        out_specs=hbm,
        scratch_shapes=[
            pltpu.VMEM((4, hd, dm), BF16),
            pltpu.VMEM((n_pairs, dm // 2, 3 * pw), U32),
            pltpu.VMEM((hd // 2, dm), U32),
            pltpu.VMEM((seq // seg, seg, dm), BF16),
            pltpu.VMEM((seq, dm), BF16),
            pltpu.VMEM((dm, 3 * dm), BF16),
            pltpu.VMEM((dm, dm), BF16),
            pltpu.VMEM((dm // 128, 8 * bdh, 128), BF16),
            pltpu.VMEM((2 * dm, dm), F32),
            pltpu.VMEM((dm, dm), F32),
            pltpu.VMEM((dm // 2, dm), U32),
            pltpu.VMEM((seq, dm), F32),
            pltpu.VMEM((seg, dm), F32),
            pltpu.VMEM((seq, dm), BF16),
            pltpu.VMEM((n_mem + seg, hd), F32),
            pltpu.VMEM((bh // 2, 2 * bdh + 8, 4 * bdh), F32),
            pltpu.VMEM((bh // 2, 2 * bdh + 8, 4 * bdh), F32),
            pltpu.VMEM((n_early, EARLY_ROWS, dm), BF16),
            pltpu.VMEM((n_early * EARLY_ROWS, dm), BF16),
            pltpu.VMEM((n_pairs, n_early * EARLY_ROWS, 3 * pw), F32),
            pltpu.SemaphoreType.DMA((5, n_pairs)),
            pltpu.SemaphoreType.DMA((3,)),
            pltpu.SemaphoreType.DMA((seq // tb,)),
        ],
        compiler_params=pltpu.CompilerParams(vmem_limit_bytes=120 * 1024 * 1024),
        name="rmt_hedgehog",
    )(
        A_x.reshape(seq // seg, seg, dm),
        A_mem0.reshape(n_mem, dm),
        feature_major(A_Wq),
        feature_major(A_Wk),
        feature_major(A_Wv),
        A_Wo.reshape(hd, dm),
        B_wqkv,
        jnp.transpose(B_w_phi, (1, 2, 0)),
        B_wo,
    )
    return out.reshape(batch, seq, dm)
```

```python
import functools
import math

import jax
import jax.numpy as jnp
from jax import lax
import jax.experimental.pallas as pl
import jax.experimental.pallas.tpu as pltpu

F32 = jnp.float32
BF16 = jnp.bfloat16
U32 = jnp.uint32
I32 = jnp.int32

LN_EPS = 1e-5
DEN_EPS = 1e-6
LOG2E = math.log2(math.e)
EARLY_ROWS = 8


def _nn(a, b):
    return lax.dot_general(a, b, (((1,), (0,)), ((), ())), preferred_element_type=F32)


def _nt(a, b):
    return lax.dot_general(a, b, (((1,), (1,)), ((), ())), preferred_element_type=F32)


def _unpack(x):
    return pltpu.bitcast(x, BF16)


def _pack(x):
    return pltpu.bitcast(x, U32)


def _iota(shape, dim):
    return lax.broadcasted_iota(I32, shape, dim)


def _layernorm(x):
    inv_n = 1.0 / x.shape[-1]
    m = jnp.sum(x, axis=-1, keepdims=True) * inv_n
    d = x - m
    v = jnp.sum(d * d, axis=-1, keepdims=True) * inv_n
    return d * lax.rsqrt(v + LN_EPS)


def _pair_blockdiag(x, dh):
    rows, width = x.shape
    top, bot = [], []
    zero = jnp.zeros((rows, 128), F32)
    for c in range(0, width, 128):
        t = x[:, c:c + 128]
        if c + 128 <= dh:
            top.append(t)
            bot.append(zero)
        elif c >= dh:
            top.append(zero)
            bot.append(t)
        else:
            first = _iota((rows, 128), 1) < dh - c
            top.append(jnp.where(first, t, 0.0))
            bot.append(jnp.where(first, 0.0, t))
    return jnp.concatenate(
        [jnp.concatenate(top, axis=1), jnp.concatenate(bot, axis=1)], axis=0
    ).astype(BF16)


def _pair_softmax(s, n_mem, scale):
    rows = s.shape[0]
    row = _iota(s.shape, 0)
    col = _iota(s.shape, 1)
    is_a = col < rows
    key = jnp.where(is_a, col, col - rows)
    s = jnp.where((row < n_mem) | (row >= key), s * scale, -1000000000.0)
    ma = jnp.max(jnp.where(is_a, s, -jnp.inf), axis=1, keepdims=True)
    mb = jnp.max(jnp.where(is_a, -jnp.inf, s), axis=1, keepdims=True)
    e = jnp.exp(s - jnp.where(is_a, ma, mb))
    la = jnp.sum(jnp.where(is_a, e, 0.0), axis=1, keepdims=True)
    lb = jnp.sum(jnp.where(is_a, 0.0, e), axis=1, keepdims=True)
    return e / jnp.where(is_a, la, lb)


def _feature_map(p):
    parts = [p[i:i + 8] for i in range(0, p.shape[0], 8)]

    def allreduce(vals, op):
        r = functools.reduce(op, vals)
        r = op(r, pltpu.roll(r, 4, 0))
        return op(r, pltpu.roll(r, 2, 0))

    hi = allreduce(parts, jnp.maximum)
    lo = allreduce(parts, jnp.minimum)
    ep = [jnp.exp2(v - hi) for v in parts]
    en = [jnp.exp2(lo - v) for v in parts]
    rp = 1.0 / allreduce(ep, jnp.add)
    rn = 1.0 / allreduce(en, jnp.add)
    return jnp.concatenate([v * rp for v in ep] + [v * rn for v in en], axis=0).astype(BF16)


def _kernel(x_hbm, mem0_ref, wq_hbm, wk_hbm, wv_hbm, wo_hbm, bqkv_hbm, wphi_ref, bwo_hbm,
            out_hbm,
            stage, wqkv, wo, x_stage, out_stage, bqkv_stage, bwo_stage, fold, bw1, bwq, bwo,
            xres, xn_a, xn_b, o_scr, kv_acc, kv_mat, early_x, early_xn, early_qkv,
            w_sem, b_sem, out_sem,
            *, seg, dh, n_layers, tb, unroll):
    n_pairs = wqkv.shape[0]
    pw = 2 * dh
    half = pw // 2
    seq, dm = xres.shape
    n_mem = mem0_ref.shape[0]
    n_seg = seq // seg
    scale = dh ** -0.5
    bdh, _, bh = wphi_ref.shape
    n_grp = bh // 2
    gw = 2 * bdh
    n_early = early_xn.shape[0] // EARLY_ROWS

    x_chunk = n_seg // n_pairs

    def pair_rows(p):
        return pl.ds(pl.multiple_of(p * pw, pw), pw)

    def pair_copies(p):
        rows = pair_rows(p)
        segs = pl.ds(p * x_chunk, x_chunk)
        return [pltpu.make_async_copy(src.at[rows], stage.at[i, rows], w_sem.at[i, p])
                for i, src in enumerate((wq_hbm, wk_hbm, wv_hbm, wo_hbm))] + [
            pltpu.make_async_copy(x_hbm.at[segs], x_stage.at[segs], w_sem.at[4, p])]

    early_copy = pltpu.make_async_copy(
        x_hbm.at[pl.ds(0, n_early), pl.ds(seg - EARLY_ROWS, EARLY_ROWS)], early_x, b_sem.at[0])
    bqkv_copy = pltpu.make_async_copy(bqkv_hbm, bqkv_stage, b_sem.at[1])
    bwo_copy = pltpu.make_async_copy(bwo_hbm, bwo_stage, b_sem.at[2])
    early_copy.start()
    for c in pair_copies(0):
        c.start()

    wphi = wphi_ref[...].astype(F32)
    wf = jnp.concatenate([wphi[d] for d in range(bdh)], axis=1)
    src = _iota((dm, 128), 0)
    natural = (src % bh) * bdh + src // bh
    first_grp = [c // gw for c in range(0, dm, 128)]
    r = _iota((4 * gw, 128), 0)
    lane = _iota((4 * gw, 128), 1)
    pick = ((r % gw) // 2 == lane).astype(BF16)
    head_start = ((r // gw) * 2 + r % 2) * bdh
    for j, g0 in enumerate(first_grp):
        wj = _nn(wf, (natural == _iota((dm, 128), 1) + j * 128).astype(BF16))
        wj = jnp.concatenate([wj, jnp.zeros((128 - bdh, 128), F32)], axis=0).astype(BF16)
        d = lane + (j * 128 - g0 * gw) - head_start
        fold[j] = jnp.where((d >= 0) & (d < bdh), _nn(pick, wj), 0.0).astype(BF16)

    early_copy.wait()
    for c in pair_copies(1):
        c.start()
    early_xn[...] = _layernorm(
        early_x[...].astype(F32).reshape(n_early * EARLY_ROWS, dm)).astype(BF16)

    def load_pair(p, carry):
        for c in pair_copies(p):
            c.wait()

        @pl.when(p + 2 < n_pairs)
        def _():
            for c in pair_copies(p + 2):
                c.start()

        pl.when(p == n_pairs // 2)(bqkv_copy.start)
        pl.when(p == n_pairs - 3)(bwo_copy.start)
        for i in range(3):
            w = stage[i, pair_rows(p), :]
            early_qkv[p, :, i * pw:(i + 1) * pw] = _nt(early_xn[...], w)
            wqkv[p, :, i * pw:(i + 1) * pw] = _pack(w.T)
        wo[pl.ds(pl.multiple_of(p * half, half), half), :] = _pack(stage[3, pair_rows(p), :])
        wide = x_stage[pl.ds(p * x_chunk, x_chunk)].astype(F32).reshape(x_chunk * seg, dm)
        xres[pl.ds(pl.multiple_of(p * x_chunk * seg, x_chunk * seg), x_chunk * seg), :] = wide
        return carry

    with jax.named_scope("load"):
        lax.fori_loop(0, n_pairs, load_pair, 0)

    def fold_phi(base):
        groups = [None] * n_grp
        for j, g0 in enumerate(first_grp):
            t = _nt(fold[j], bqkv_stage[:, base + j * 128:base + (j + 1) * 128]) * LOG2E
            for i in range(4):
                part = t[i * gw:(i + 1) * gw]
                groups[g0 + i] = part if groups[g0 + i] is None else groups[g0 + i] + part
        return groups

    bqkv_copy.wait()
    bwo_copy.wait()
    wvt = bqkv_stage[:, 2 * dm:].astype(F32).T
    for g, (wpq, wpk) in enumerate(zip(fold_phi(0), fold_phi(dm))):
        bwq[g * gw:(g + 1) * gw, :] = wpq
        bw1[2 * g * gw:(2 * g + 1) * gw, :] = wpk
        bw1[(2 * g + 1) * gw:(2 * g + 2) * gw, :] = wvt[g * gw:(g + 1) * gw]
    bwo[...] = _pack(bwo_stage[...])

    def seg_rows(s):
        return pl.ds(pl.multiple_of(s * seg, seg), seg)

    def rmt_step(s, mem, early):
        if early:
            h = jnp.concatenate([mem, xn_a[:seg - EARLY_ROWS, :]], axis=0).astype(BF16)
            early_rows = pl.ds(pl.multiple_of(s * EARLY_ROWS, EARLY_ROWS), EARLY_ROWS)
        else:
            h = jnp.concatenate([mem, xn_a[...]], axis=0)
        xn_next = _layernorm(xres[seg_rows(jnp.minimum(s + 1, n_seg - 1)), :])
        prev = seg_rows(jnp.maximum(s - 1, 0))
        xn_b[prev, :] = _layernorm(xres[prev, :]).astype(BF16)

        lag, tail, ks = n_pairs // 2, 2, 256
        qkv, prob = {}, {}
        acc, done = None, 0

        def out_proj(acc, lo, hi):
            t = _nn(o_scr[:, lo * pw:hi * pw], _unpack(wo[lo * half:hi * half, :]))
            return t if acc is None else acc + t

        for p in range(n_pairs + 2):
            if p == 0:
                start = _nn(h[:, :ks], _unpack(wqkv[p, :ks // 2, :]))
                qkv[p] = _nn(h[:, ks:], _unpack(wqkv[p, ks // 2:, :])) + start
            elif p < n_pairs:
                qkv[p] = _nn(h, _unpack(wqkv[p]))
            if p < n_pairs:
                if early:
                    qkv[p] = jnp.concatenate([qkv[p], early_qkv[p, early_rows, :]], axis=0)
            left = n_pairs - tail - done
            n = 0 if p < lag else 1 if p < n_pairs else (left + 1) // 2 if p == n_pairs else left
            if n:
                acc = out_proj(acc, done, done + n)
                done += n
            if 0 <= p - 1 < n_pairs:
                t = qkv[p - 1]
                scores = _nt(t[:, :pw], _pair_blockdiag(t[:, pw:2 * pw], dh))
                prob[p - 1] = _pair_softmax(scores, n_mem, scale)
            if 0 <= p - 2 < n_pairs:
                o_scr[:, (p - 2) * pw:(p - 1) * pw] = _nn(
                    prob[p - 2], _pair_blockdiag(qkv[p - 2][:, 2 * pw:], dh))
        acc = out_proj(acc, done, n_pairs - 1)
        o_last = o_scr[:, (n_pairs - 1) * pw:]
        acc = jnp.concatenate(
            [acc[:, cols] + _nn(o_last, _unpack(wo[(n_pairs - 1) * half:, cols]))
             for cols in (slice(0, ks), slice(ks, dm))], axis=1)
        xn_a[...] = xn_next
        rows = seg_rows(s)
        xres[rows, :] = xres[rows, :] + acc[n_mem:]
        return acc[:n_mem]

    def rmt_steps(lo, hi, mem, early):
        def body(i, mem):
            for u in range(unroll):
                mem = rmt_step(i * unroll + u, mem, early)
            return mem

        return lax.fori_loop(lo, hi, body, mem)

    def rmt_layer(layer):
        xn_a[...] = _layernorm(xres[0:seg, :])
        split = jnp.where(layer == 0, n_early // unroll, 0)
        mem = rmt_steps(0, split, mem0_ref[...].astype(F32), True)
        rmt_steps(split, n_seg // unroll, mem, False)
        last = slice(seq - seg, seq)
        xn_b[last, :] = _layernorm(xres[last, :]).astype(BF16)

    chunk = 4
    n_chunk = n_grp // chunk

    def blk_rows(i):
        return pl.ds(pl.multiple_of(i * tb, tb), tb)

    def kv_block(i, carry):
        xn = xn_b[blk_rows(i), :]
        ones = jnp.ones((8, tb), F32)
        proj = {}
        for c in range(n_chunk + 1):
            if c < n_chunk:
                proj[c] = _nt(bw1[2 * c * chunk * gw:2 * (c + 1) * chunk * gw, :], xn)
            if c >= 1:
                t = proj[c - 1]
                for j in range(chunk):
                    g = (c - 1) * chunk + j
                    phi = _feature_map(t[2 * j * gw:(2 * j + 1) * gw])
                    lhs = jnp.concatenate([t[(2 * j + 1) * gw:(2 * j + 2) * gw], ones], axis=0)
                    kv_acc[g] += _nt(lhs, phi)
        return carry

    def out_copy(i):
        return pltpu.make_async_copy(out_stage.at[blk_rows(i)], out_hbm.at[blk_rows(i)], out_sem.at[i])

    def out_block(i, layer):
        rows = blk_rows(i)
        xn = xn_b[rows, :]
        first8 = _iota((8, tb), 0) < 4
        proj, outs = {}, []
        for c in range(n_chunk + 1):
            if c < n_chunk:
                proj[c] = _nt(bwq[c * chunk * gw:(c + 1) * chunk * gw, :], xn)
            if c >= 1:
                t = proj[c - 1]
                for j in range(chunk):
                    g = (c - 1) * chunk + j
                    nd = _nn(kv_mat[g], _feature_map(t[j * gw:(j + 1) * gw]))
                    inv = 1.0 / (nd[gw:] + DEN_EPS)
                    swapped = pltpu.roll(inv, 4, 0)
                    inv_a = jnp.where(first8, inv, swapped)
                    inv_b = jnp.where(first8, swapped, inv)
                    outs.append(nd[:gw] * jnp.concatenate([inv_a, inv_a, inv, inv_b, inv_b], axis=0))
        o = jnp.concatenate(outs, axis=0).astype(BF16).T
        y = xres[rows, :] + _nn(o, _unpack(bwo[...]))
        xres[rows, :] = y
        out_stage[rows, :] = y.astype(BF16)

        @pl.when(layer == n_layers - 1)
        def _():
            out_copy(i).start()

        return layer

    def hedgehog_layer(layer):
        kv_acc[...] = jnp.zeros(kv_acc.shape, F32)
        lax.fori_loop(0, seq // tb, kv_block, 0)
        shape = kv_acc.shape[1:]
        r = _iota(shape, 0)
        row_head = jnp.where(r < gw, r // bdh, (r - gw) // 4)
        same_head = row_head == _iota(shape, 1) % 2
        for g in range(n_grp):
            kv_mat[g] = jnp.where(same_head, kv_acc[g], 0.0)
        lax.fori_loop(0, seq // tb, out_block, layer)

    def layer_pair(layer, carry):
        with jax.named_scope("rmt"):
            rmt_layer(layer)
        with jax.named_scope("hedgehog"):
            hedgehog_layer(layer)
        return carry

    lax.fori_loop(0, n_layers, layer_pair, 0)
    for i in range(seq // tb):
        out_copy(i).wait()


@functools.partial(jax.jit, static_argnames=("A_seg_len",))
def pallas_interleave_layers__memory_aug_recurrent_mem_tr__linear_kernel_hedgehog__prompt_kernel(
    A_x: jax.Array,
    A_mem0: jax.Array,
    A_Wq: jax.Array,
    A_Wk: jax.Array,
    A_Wv: jax.Array,
    A_Wo: jax.Array,
    A_seg_len: int,
    B_x: jax.Array,
    B_wqkv: jax.Array,
    B_w_phi: jax.Array,
    B_wo: jax.Array,
):
    del B_x
    batch, seq, dm = A_x.shape
    _, heads, dh = A_Wq.shape
    n_mem = A_mem0.shape[1]
    bh, bdh, _ = B_w_phi.shape
    seg = int(A_seg_len)
    assert batch == 1 and bdh == 20 and bh * bdh == dm and heads % 2 == 0
    assert (2 * dh) % 128 == 0 and n_mem % 8 == 0 and seg % 16 == 0 and 2 * (n_mem + seg) <= 128
    n_pairs, pw, hd = heads // 2, 2 * dh, heads * dh
    tb, unroll, n_early = 512, 2, 48

    def feature_major(w):
        return jnp.transpose(w, (1, 2, 0)).reshape(hd, dm)

    hbm = pl.BlockSpec(memory_space=pl.ANY)
    vmem = pl.BlockSpec(memory_space=pltpu.VMEM)
    out = pl.pallas_call(
        functools.partial(_kernel, seg=seg, dh=dh, n_layers=2, tb=tb, unroll=unroll),
        out_shape=jax.ShapeDtypeStruct((seq, dm), A_x.dtype),
        in_specs=[hbm, vmem, hbm, hbm, hbm, hbm, hbm, vmem, hbm],
        out_specs=hbm,
        scratch_shapes=[
            pltpu.VMEM((4, hd, dm), BF16),
            pltpu.VMEM((n_pairs, dm // 2, 3 * pw), U32),
            pltpu.VMEM((hd // 2, dm), U32),
            pltpu.VMEM((seq // seg, seg, dm), BF16),
            pltpu.VMEM((seq, dm), BF16),
            pltpu.VMEM((dm, 3 * dm), BF16),
            pltpu.VMEM((dm, dm), BF16),
            pltpu.VMEM((dm // 128, 8 * bdh, 128), BF16),
            pltpu.VMEM((2 * dm, dm), F32),
            pltpu.VMEM((dm, dm), F32),
            pltpu.VMEM((dm // 2, dm), U32),
            pltpu.VMEM((seq, dm), F32),
            pltpu.VMEM((seg, dm), F32),
            pltpu.VMEM((seq, dm), BF16),
            pltpu.VMEM((n_mem + seg, hd), F32),
            pltpu.VMEM((bh // 2, 2 * bdh + 8, 4 * bdh), F32),
            pltpu.VMEM((bh // 2, 2 * bdh + 8, 4 * bdh), F32),
            pltpu.VMEM((n_early, EARLY_ROWS, dm), BF16),
            pltpu.VMEM((n_early * EARLY_ROWS, dm), BF16),
            pltpu.VMEM((n_pairs, n_early * EARLY_ROWS, 3 * pw), F32),
            pltpu.SemaphoreType.DMA((5, n_pairs)),
            pltpu.SemaphoreType.DMA((3,)),
            pltpu.SemaphoreType.DMA((seq // tb,)),
        ],
        compiler_params=pltpu.CompilerParams(vmem_limit_bytes=120 * 1024 * 1024),
        name="rmt_hedgehog",
    )(
        A_x.reshape(seq // seg, seg, dm),
        A_mem0.reshape(n_mem, dm),
        feature_major(A_Wq),
        feature_major(A_Wk),
        feature_major(A_Wv),
        A_Wo.reshape(hd, dm),
        B_wqkv,
        jnp.transpose(B_w_phi, (1, 2, 0)),
        B_wo,
    )
    return out.reshape(batch, seq, dm)
```

```python
import functools
import math

import jax
import jax.numpy as jnp
from jax import lax
import jax.experimental.pallas as pl
import jax.experimental.pallas.tpu as pltpu

F32 = jnp.float32
BF16 = jnp.bfloat16
U32 = jnp.uint32
I32 = jnp.int32

LN_EPS = 1e-5
DEN_EPS = 1e-6
LOG2E = math.log2(math.e)
EARLY_ROWS = 8
OUT_PLAN = "000000001111111133"
OUT_PLAN_EARLY = "000000001111111133"


def _nn(a, b):
    return lax.dot_general(a, b, (((1,), (0,)), ((), ())), preferred_element_type=F32)


def _nt(a, b):
    return lax.dot_general(a, b, (((1,), (1,)), ((), ())), preferred_element_type=F32)


def _unpack(x):
    return pltpu.bitcast(x, BF16)


def _pack(x):
    return pltpu.bitcast(x, U32)


def _iota(shape, dim):
    return lax.broadcasted_iota(I32, shape, dim)


def _layernorm(x):
    inv_n = 1.0 / x.shape[-1]
    m = jnp.sum(x, axis=-1, keepdims=True) * inv_n
    d = x - m
    v = jnp.sum(d * d, axis=-1, keepdims=True) * inv_n
    return d * lax.rsqrt(v + LN_EPS)


def _pair_blockdiag(x, dh):
    rows, width = x.shape
    top, bot = [], []
    zero = jnp.zeros((rows, 128), F32)
    for c in range(0, width, 128):
        t = x[:, c:c + 128]
        if c + 128 <= dh:
            top.append(t)
            bot.append(zero)
        elif c >= dh:
            top.append(zero)
            bot.append(t)
        else:
            first = _iota((rows, 128), 1) < dh - c
            top.append(jnp.where(first, t, 0.0))
            bot.append(jnp.where(first, 0.0, t))
    return jnp.concatenate(
        [jnp.concatenate(top, axis=1), jnp.concatenate(bot, axis=1)], axis=0
    ).astype(BF16)


def _pair_softmax(s, n_mem, scale):
    rows = s.shape[0]
    row = _iota(s.shape, 0)
    col = _iota(s.shape, 1)
    is_a = col < rows
    key = jnp.where(is_a, col, col - rows)
    s = jnp.where((row < n_mem) | (row >= key), s * scale, -1000000000.0)
    ma = jnp.max(jnp.where(is_a, s, -jnp.inf), axis=1, keepdims=True)
    mb = jnp.max(jnp.where(is_a, -jnp.inf, s), axis=1, keepdims=True)
    e = jnp.exp(s - jnp.where(is_a, ma, mb))
    la = jnp.sum(jnp.where(is_a, e, 0.0), axis=1, keepdims=True)
    lb = jnp.sum(jnp.where(is_a, 0.0, e), axis=1, keepdims=True)
    return e / jnp.where(is_a, la, lb)


def _feature_map(p):
    parts = [p[i:i + 8] for i in range(0, p.shape[0], 8)]

    def allreduce(vals, op):
        r = functools.reduce(op, vals)
        r = op(r, pltpu.roll(r, 4, 0))
        return op(r, pltpu.roll(r, 2, 0))

    hi = allreduce(parts, jnp.maximum)
    lo = allreduce(parts, jnp.minimum)
    ep = [jnp.exp2(v - hi) for v in parts]
    en = [jnp.exp2(lo - v) for v in parts]
    rp = 1.0 / allreduce(ep, jnp.add)
    rn = 1.0 / allreduce(en, jnp.add)
    return jnp.concatenate([v * rp for v in ep] + [v * rn for v in en], axis=0).astype(BF16)


def _kernel(x_hbm, mem0_ref, wq_hbm, wk_hbm, wv_hbm, wo_hbm, bqkv_hbm, wphi_ref, bwo_hbm,
            out_hbm,
            stage, wqkv, wo, x_stage, out_stage, bqkv_stage, bwo_stage, fold, bw1, bwq, bwo,
            xres, xn_a, xn_b, o_scr, kv_acc, kv_mat, early_x, early_xn, early_qkv,
            w_sem, b_sem, out_sem,
            *, seg, dh, n_layers, tb, unroll):
    n_pairs = wqkv.shape[0]
    pw = 2 * dh
    half = pw // 2
    seq, dm = xres.shape
    n_mem = mem0_ref.shape[0]
    n_seg = seq // seg
    scale = dh ** -0.5
    bdh, _, bh = wphi_ref.shape
    n_grp = bh // 2
    gw = 2 * bdh
    n_early = early_xn.shape[0] // EARLY_ROWS

    x_chunk = n_seg // n_pairs

    def pair_rows(p):
        return pl.ds(pl.multiple_of(p * pw, pw), pw)

    def pair_copies(p):
        rows = pair_rows(p)
        segs = pl.ds(p * x_chunk, x_chunk)
        return [pltpu.make_async_copy(src.at[rows], stage.at[i, rows], w_sem.at[i, p])
                for i, src in enumerate((wq_hbm, wk_hbm, wv_hbm, wo_hbm))] + [
            pltpu.make_async_copy(x_hbm.at[segs], x_stage.at[segs], w_sem.at[4, p])]

    early_copy = pltpu.make_async_copy(
        x_hbm.at[pl.ds(0, n_early), pl.ds(seg - EARLY_ROWS, EARLY_ROWS)], early_x, b_sem.at[0])
    bqkv_copy = pltpu.make_async_copy(bqkv_hbm, bqkv_stage, b_sem.at[1])
    bwo_copy = pltpu.make_async_copy(bwo_hbm, bwo_stage, b_sem.at[2])
    early_copy.start()
    for c in pair_copies(0):
        c.start()

    wphi = wphi_ref[...].astype(F32)
    wf = jnp.concatenate([wphi[d] for d in range(bdh)], axis=1)
    src = _iota((dm, 128), 0)
    natural = (src % bh) * bdh + src // bh
    first_grp = [c // gw for c in range(0, dm, 128)]
    r = _iota((4 * gw, 128), 0)
    lane = _iota((4 * gw, 128), 1)
    pick = ((r % gw) // 2 == lane).astype(BF16)
    head_start = ((r // gw) * 2 + r % 2) * bdh
    for j, g0 in enumerate(first_grp):
        wj = _nn(wf, (natural == _iota((dm, 128), 1) + j * 128).astype(BF16))
        wj = jnp.concatenate([wj, jnp.zeros((128 - bdh, 128), F32)], axis=0).astype(BF16)
        d = lane + (j * 128 - g0 * gw) - head_start
        fold[j] = jnp.where((d >= 0) & (d < bdh), _nn(pick, wj), 0.0).astype(BF16)

    early_copy.wait()
    for c in pair_copies(1):
        c.start()
    early_xn[...] = _layernorm(
        early_x[...].astype(F32).reshape(n_early * EARLY_ROWS, dm)).astype(BF16)

    def load_pair(p, carry):
        for c in pair_copies(p):
            c.wait()

        @pl.when(p + 2 < n_pairs)
        def _():
            for c in pair_copies(p + 2):
                c.start()

        pl.when(p == n_pairs // 2)(bqkv_copy.start)
        pl.when(p == n_pairs - 3)(bwo_copy.start)
        for i in range(3):
            w = stage[i, pair_rows(p), :]
            early_qkv[p, :, i * pw:(i + 1) * pw] = _nt(early_xn[...], w)
            wqkv[p, :, i * pw:(i + 1) * pw] = _pack(w.T)
        wo[pl.ds(pl.multiple_of(p * half, half), half), :] = _pack(stage[3, pair_rows(p), :])
        wide = x_stage[pl.ds(p * x_chunk, x_chunk)].astype(F32).reshape(x_chunk * seg, dm)
        xres[pl.ds(pl.multiple_of(p * x_chunk * seg, x_chunk * seg), x_chunk * seg), :] = wide
        return carry

    with jax.named_scope("load"):
        lax.fori_loop(0, n_pairs, load_pair, 0)

    def fold_phi(base):
        groups = [None] * n_grp
        for j, g0 in enumerate(first_grp):
            t = _nt(fold[j], bqkv_stage[:, base + j * 128:base + (j + 1) * 128]) * LOG2E
            for i in range(4):
                part = t[i * gw:(i + 1) * gw]
                groups[g0 + i] = part if groups[g0 + i] is None else groups[g0 + i] + part
        return groups

    bqkv_copy.wait()
    bwo_copy.wait()
    wvt = bqkv_stage[:, 2 * dm:].astype(F32).T
    for g, (wpq, wpk) in enumerate(zip(fold_phi(0), fold_phi(dm))):
        bwq[g * gw:(g + 1) * gw, :] = wpq
        bw1[2 * g * gw:(2 * g + 1) * gw, :] = wpk
        bw1[(2 * g + 1) * gw:(2 * g + 2) * gw, :] = wvt[g * gw:(g + 1) * gw]
    bwo[...] = _pack(bwo_stage[...])

    def seg_rows(s):
        return pl.ds(pl.multiple_of(s * seg, seg), seg)

    def rmt_step(s, mem, early):
        if early:
            h = jnp.concatenate([mem, xn_a[:seg - EARLY_ROWS, :]], axis=0).astype(BF16)
            early_rows = pl.ds(pl.multiple_of(s * EARLY_ROWS, EARLY_ROWS), EARLY_ROWS)
        else:
            h = jnp.concatenate([mem, xn_a[...]], axis=0)
        xn_next = _layernorm(xres[seg_rows(jnp.minimum(s + 1, n_seg - 1)), :])
        prev = seg_rows(jnp.maximum(s - 1, 0))
        xn_b[prev, :] = _layernorm(xres[prev, :]).astype(BF16)

        plan = OUT_PLAN_EARLY if early else OUT_PLAN
        ks = 256
        qkv, prob = {}, {}
        acc, done = None, 0

        def out_proj(acc, lo, hi):
            t = _nn(o_scr[:, lo * pw:hi * pw], _unpack(wo[lo * half:hi * half, :]))
            return t if acc is None else t + acc

        for p in range(n_pairs + 2):
            if p == 0:
                start = _nn(h[:, :ks], _unpack(wqkv[p, :ks // 2, :]))
                qkv[p] = _nn(h[:, ks:], _unpack(wqkv[p, ks // 2:, :])) + start
            elif p < n_pairs:
                qkv[p] = _nn(h, _unpack(wqkv[p]))
            if p < n_pairs:
                if early:
                    qkv[p] = jnp.concatenate([qkv[p], early_qkv[p, early_rows, :]], axis=0)
            n = int(plan[p])
            if n:
                acc = out_proj(acc, done, done + n)
                done += n
            if 0 <= p - 1 < n_pairs:
                t = qkv[p - 1]
                scores = _nt(t[:, :pw], _pair_blockdiag(t[:, pw:2 * pw], dh))
                prob[p - 1] = _pair_softmax(scores, n_mem, scale)
            if 0 <= p - 2 < n_pairs:
                o_scr[:, (p - 2) * pw:(p - 1) * pw] = _nn(
                    prob[p - 2], _pair_blockdiag(qkv[p - 2][:, 2 * pw:], dh))
        acc = out_proj(acc, done, n_pairs - 1)
        o_last = o_scr[:, (n_pairs - 1) * pw:]
        acc = jnp.concatenate(
            [acc[:, cols] + _nn(o_last, _unpack(wo[(n_pairs - 1) * half:, cols]))
             for cols in (slice(0, ks), slice(ks, dm))], axis=1)
        xn_a[...] = xn_next
        rows = seg_rows(s)
        xres[rows, :] = xres[rows, :] + acc[n_mem:]
        return acc[:n_mem]

    def rmt_steps(lo, hi, mem, early):
        def body(i, mem):
            for u in range(unroll):
                mem = rmt_step(i * unroll + u, mem, early)
            return mem

        return lax.fori_loop(lo, hi, body, mem)

    def rmt_layer(layer):
        xn_a[...] = _layernorm(xres[0:seg, :])
        split = jnp.where(layer == 0, n_early // unroll, 0)
        mem = rmt_steps(0, split, mem0_ref[...].astype(F32), True)
        rmt_steps(split, n_seg // unroll, mem, False)
        last = slice(seq - seg, seq)
        xn_b[last, :] = _layernorm(xres[last, :]).astype(BF16)

    chunk = 4
    n_chunk = n_grp // chunk

    def blk_rows(i):
        return pl.ds(pl.multiple_of(i * tb, tb), tb)

    def kv_block(i, carry):
        xn = xn_b[blk_rows(i), :]
        ones = jnp.ones((8, tb), F32)
        proj = {}
        for c in range(n_chunk + 1):
            if c < n_chunk:
                proj[c] = _nt(bw1[2 * c * chunk * gw:2 * (c + 1) * chunk * gw, :], xn)
            if c >= 1:
                t = proj[c - 1]
                for j in range(chunk):
                    g = (c - 1) * chunk + j
                    phi = _feature_map(t[2 * j * gw:(2 * j + 1) * gw])
                    lhs = jnp.concatenate([t[(2 * j + 1) * gw:(2 * j + 2) * gw], ones], axis=0)
                    kv_acc[g] += _nt(lhs, phi)
        return carry

    def out_copy(i):
        return pltpu.make_async_copy(out_stage.at[blk_rows(i)], out_hbm.at[blk_rows(i)], out_sem.at[i])

    def out_block(i, layer):
        rows = blk_rows(i)
        xn = xn_b[rows, :]
        first8 = _iota((8, tb), 0) < 4
        proj, outs = {}, []

        def out_proj(y, lo, hi):
            o = jnp.concatenate(outs, axis=0)[lo:hi].astype(BF16).T
            return _nn(o, _unpack(bwo[lo // 2:hi // 2, :])) + y

        y = xres[rows, :]
        for c in range(n_chunk + 1):
            if c < n_chunk:
                proj[c] = _nt(bwq[c * chunk * gw:(c + 1) * chunk * gw, :], xn)
            else:
                y = out_proj(y, 0, 256)
            if c >= 1:
                t = proj[c - 1]
                for j in range(chunk):
                    g = (c - 1) * chunk + j
                    nd = _nn(kv_mat[g], _feature_map(t[j * gw:(j + 1) * gw]))
                    inv = 1.0 / (nd[gw:] + DEN_EPS)
                    swapped = pltpu.roll(inv, 4, 0)
                    inv_a = jnp.where(first8, inv, swapped)
                    inv_b = jnp.where(first8, swapped, inv)
                    outs.append(nd[:gw] * jnp.concatenate([inv_a, inv_a, inv, inv_b, inv_b], axis=0))
        y = out_proj(out_proj(y, 256, 384), 384, dm)
        xres[rows, :] = y
        out_stage[rows, :] = y.astype(BF16)

        @pl.when(layer == n_layers - 1)
        def _():
            out_copy(i).start()

        return layer

    def hedgehog_layer(layer):
        kv_acc[...] = jnp.zeros(kv_acc.shape, F32)
        lax.fori_loop(0, seq // tb, kv_block, 0)
        shape = kv_acc.shape[1:]
        r = _iota(shape, 0)
        row_head = jnp.where(r < gw, r // bdh, (r - gw) // 4)
        same_head = row_head == _iota(shape, 1) % 2
        for g in range(n_grp):
            kv_mat[g] = jnp.where(same_head, kv_acc[g], 0.0)
        lax.fori_loop(0, seq // tb, out_block, layer)

    def layer_pair(layer, carry):
        with jax.named_scope("rmt"):
            rmt_layer(layer)
        with jax.named_scope("hedgehog"):
            hedgehog_layer(layer)
        return carry

    lax.fori_loop(0, n_layers, layer_pair, 0)
    for i in range(seq // tb):
        out_copy(i).wait()


@functools.partial(jax.jit, static_argnames=("A_seg_len",))
def pallas_interleave_layers__memory_aug_recurrent_mem_tr__linear_kernel_hedgehog__prompt_kernel(
    A_x: jax.Array,
    A_mem0: jax.Array,
    A_Wq: jax.Array,
    A_Wk: jax.Array,
    A_Wv: jax.Array,
    A_Wo: jax.Array,
    A_seg_len: int,
    B_x: jax.Array,
    B_wqkv: jax.Array,
    B_w_phi: jax.Array,
    B_wo: jax.Array,
):
    del B_x
    batch, seq, dm = A_x.shape
    _, heads, dh = A_Wq.shape
    n_mem = A_mem0.shape[1]
    bh, bdh, _ = B_w_phi.shape
    seg = int(A_seg_len)
    assert batch == 1 and bdh == 20 and bh * bdh == dm and heads % 2 == 0
    assert (2 * dh) % 128 == 0 and n_mem % 8 == 0 and seg % 16 == 0 and 2 * (n_mem + seg) <= 128
    n_pairs, pw, hd = heads // 2, 2 * dh, heads * dh
    tb, unroll, n_early = 512, 2, 48

    def feature_major(w):
        return jnp.transpose(w, (1, 2, 0)).reshape(hd, dm)

    hbm = pl.BlockSpec(memory_space=pl.ANY)
    vmem = pl.BlockSpec(memory_space=pltpu.VMEM)
    out = pl.pallas_call(
        functools.partial(_kernel, seg=seg, dh=dh, n_layers=2, tb=tb, unroll=unroll),
        out_shape=jax.ShapeDtypeStruct((seq, dm), A_x.dtype),
        in_specs=[hbm, vmem, hbm, hbm, hbm, hbm, hbm, vmem, hbm],
        out_specs=hbm,
        scratch_shapes=[
            pltpu.VMEM((4, hd, dm), BF16),
            pltpu.VMEM((n_pairs, dm // 2, 3 * pw), U32),
            pltpu.VMEM((hd // 2, dm), U32),
            pltpu.VMEM((seq // seg, seg, dm), BF16),
            pltpu.VMEM((seq, dm), BF16),
            pltpu.VMEM((dm, 3 * dm), BF16),
            pltpu.VMEM((dm, dm), BF16),
            pltpu.VMEM((dm // 128, 8 * bdh, 128), BF16),
            pltpu.VMEM((2 * dm, dm), F32),
            pltpu.VMEM((dm, dm), F32),
            pltpu.VMEM((dm // 2, dm), U32),
            pltpu.VMEM((seq, dm), F32),
            pltpu.VMEM((seg, dm), F32),
            pltpu.VMEM((seq, dm), BF16),
            pltpu.VMEM((n_mem + seg, hd), F32),
            pltpu.VMEM((bh // 2, 2 * bdh + 8, 4 * bdh), F32),
            pltpu.VMEM((bh // 2, 2 * bdh + 8, 4 * bdh), F32),
            pltpu.VMEM((n_early, EARLY_ROWS, dm), BF16),
            pltpu.VMEM((n_early * EARLY_ROWS, dm), BF16),
            pltpu.VMEM((n_pairs, n_early * EARLY_ROWS, 3 * pw), F32),
            pltpu.SemaphoreType.DMA((5, n_pairs)),
            pltpu.SemaphoreType.DMA((3,)),
            pltpu.SemaphoreType.DMA((seq // tb,)),
        ],
        compiler_params=pltpu.CompilerParams(vmem_limit_bytes=120 * 1024 * 1024),
        name="rmt_hedgehog",
    )(
        A_x.reshape(seq // seg, seg, dm),
        A_mem0.reshape(n_mem, dm),
        feature_major(A_Wq),
        feature_major(A_Wk),
        feature_major(A_Wv),
        A_Wo.reshape(hd, dm),
        B_wqkv,
        jnp.transpose(B_w_phi, (1, 2, 0)),
        B_wo,
    )
    return out.reshape(batch, seq, dm)
```

```python
import functools
import math

import jax
import jax.numpy as jnp
from jax import lax
import jax.experimental.pallas as pl
import jax.experimental.pallas.tpu as pltpu

F32 = jnp.float32
BF16 = jnp.bfloat16
U32 = jnp.uint32
I32 = jnp.int32

LN_EPS = 1e-5
DEN_EPS = 1e-6
LOG2E = math.log2(math.e)
EARLY_ROWS = 8
OUT_PLAN = "0000000011111111222"
OUT_PLAN_EARLY = "0000000011111111222"
VPU_PAIRS = range(0, 15)
VPU_PAIRS_EARLY = range(0, 15)


def _nn(a, b):
    return lax.dot_general(a, b, (((1,), (0,)), ((), ())), preferred_element_type=F32)


def _nt(a, b):
    return lax.dot_general(a, b, (((1,), (1,)), ((), ())), preferred_element_type=F32)


def _unpack(x):
    return pltpu.bitcast(x, BF16)


def _pack(x):
    return pltpu.bitcast(x, U32)


def _iota(shape, dim):
    return lax.broadcasted_iota(I32, shape, dim)


def _layernorm(x):
    inv_n = 1.0 / x.shape[-1]
    m = jnp.sum(x, axis=-1, keepdims=True) * inv_n
    d = x - m
    v = jnp.sum(d * d, axis=-1, keepdims=True) * inv_n
    return d * lax.rsqrt(v + LN_EPS)


def _pair_blockdiag(x, dh):
    rows, width = x.shape
    top, bot = [], []
    zero = jnp.zeros((rows, 128), F32)
    for c in range(0, width, 128):
        t = x[:, c:c + 128]
        if c + 128 <= dh:
            top.append(t)
            bot.append(zero)
        elif c >= dh:
            top.append(zero)
            bot.append(t)
        else:
            first = _iota((rows, 128), 1) < dh - c
            top.append(jnp.where(first, t, 0.0))
            bot.append(jnp.where(first, 0.0, t))
    return jnp.concatenate(
        [jnp.concatenate(top, axis=1), jnp.concatenate(bot, axis=1)], axis=0
    ).astype(BF16)


def _pair_softmax(s, n_mem, scale):
    rows = s.shape[0]
    row = _iota(s.shape, 0)
    col = _iota(s.shape, 1)
    is_a = col < rows
    key = jnp.where(is_a, col, col - rows)
    s = jnp.where((row < n_mem) | (row >= key), s * scale, -1000000000.0)
    ma = jnp.max(jnp.where(is_a, s, -jnp.inf), axis=1, keepdims=True)
    mb = jnp.max(jnp.where(is_a, -jnp.inf, s), axis=1, keepdims=True)
    e = jnp.exp(s - jnp.where(is_a, ma, mb))
    la = jnp.sum(jnp.where(is_a, e, 0.0), axis=1, keepdims=True)
    lb = jnp.sum(jnp.where(is_a, 0.0, e), axis=1, keepdims=True)
    return e / jnp.where(is_a, la, lb)


def _feature_map(p):
    parts = [p[i:i + 8] for i in range(0, p.shape[0], 8)]

    def allreduce(vals, op):
        r = functools.reduce(op, vals)
        r = op(r, pltpu.roll(r, 4, 0))
        return op(r, pltpu.roll(r, 2, 0))

    hi = allreduce(parts, jnp.maximum)
    lo = allreduce(parts, jnp.minimum)
    ep = [jnp.exp2(v - hi) for v in parts]
    en = [jnp.exp2(lo - v) for v in parts]
    rp = 1.0 / allreduce(ep, jnp.add)
    rn = 1.0 / allreduce(en, jnp.add)
    return jnp.concatenate([v * rp for v in ep] + [v * rn for v in en], axis=0).astype(BF16)


def _kernel(x_hbm, mem0_ref, wq_hbm, wk_hbm, wv_hbm, wo_hbm, bqkv_hbm, wphi_ref, bwo_hbm,
            out_hbm,
            stage, wqkv, wo, x_stage, out_stage, bqkv_stage, bwo_stage, fold, bw1, bwq, bwo,
            xres, xn_a, xn_b, o_scr, v_scr, kv_acc, kv_mat, early_x, early_xn, early_qkv,
            w_sem, b_sem, out_sem,
            *, seg, dh, n_layers, tb, unroll):
    n_pairs = wqkv.shape[0]
    pw = 2 * dh
    half = pw // 2
    seq, dm = xres.shape
    n_mem = mem0_ref.shape[0]
    n_seg = seq // seg
    scale = dh ** -0.5
    bdh, _, bh = wphi_ref.shape
    n_grp = bh // 2
    gw = 2 * bdh
    n_early = early_xn.shape[0] // EARLY_ROWS

    x_chunk = n_seg // n_pairs

    def pair_rows(p):
        return pl.ds(pl.multiple_of(p * pw, pw), pw)

    def pair_copies(p):
        rows = pair_rows(p)
        segs = pl.ds(p * x_chunk, x_chunk)
        return [pltpu.make_async_copy(src.at[rows], stage.at[i, rows], w_sem.at[i, p])
                for i, src in enumerate((wq_hbm, wk_hbm, wv_hbm, wo_hbm))] + [
            pltpu.make_async_copy(x_hbm.at[segs], x_stage.at[segs], w_sem.at[4, p])]

    early_copy = pltpu.make_async_copy(
        x_hbm.at[pl.ds(0, n_early), pl.ds(seg - EARLY_ROWS, EARLY_ROWS)], early_x, b_sem.at[0])
    bqkv_copy = pltpu.make_async_copy(bqkv_hbm, bqkv_stage, b_sem.at[1])
    bwo_copy = pltpu.make_async_copy(bwo_hbm, bwo_stage, b_sem.at[2])
    early_copy.start()
    for c in pair_copies(0):
        c.start()

    wphi = wphi_ref[...].astype(F32)
    wf = jnp.concatenate([wphi[d] for d in range(bdh)], axis=1)
    src = _iota((dm, 128), 0)
    natural = (src % bh) * bdh + src // bh
    first_grp = [c // gw for c in range(0, dm, 128)]
    r = _iota((4 * gw, 128), 0)
    lane = _iota((4 * gw, 128), 1)
    pick = ((r % gw) // 2 == lane).astype(BF16)
    head_start = ((r // gw) * 2 + r % 2) * bdh
    for j, g0 in enumerate(first_grp):
        wj = _nn(wf, (natural == _iota((dm, 128), 1) + j * 128).astype(BF16))
        wj = jnp.concatenate([wj, jnp.zeros((128 - bdh, 128), F32)], axis=0).astype(BF16)
        d = lane + (j * 128 - g0 * gw) - head_start
        fold[j] = jnp.where((d >= 0) & (d < bdh), _nn(pick, wj), 0.0).astype(BF16)

    early_copy.wait()
    for c in pair_copies(1):
        c.start()
    early_xn[...] = _layernorm(
        early_x[...].astype(F32).reshape(n_early * EARLY_ROWS, dm)).astype(BF16)

    def load_pair(p, carry):
        for c in pair_copies(p):
            c.wait()

        @pl.when(p + 2 < n_pairs)
        def _():
            for c in pair_copies(p + 2):
                c.start()

        pl.when(p == n_pairs // 2)(bqkv_copy.start)
        pl.when(p == n_pairs - 3)(bwo_copy.start)
        for i in range(3):
            w = stage[i, pair_rows(p), :]
            early_qkv[p, :, i * pw:(i + 1) * pw] = _nt(early_xn[...], w)
            wqkv[p, :, i * pw:(i + 1) * pw] = _pack(w.T)
        wo[pl.ds(pl.multiple_of(p * half, half), half), :] = _pack(stage[3, pair_rows(p), :])
        wide = x_stage[pl.ds(p * x_chunk, x_chunk)].astype(F32).reshape(x_chunk * seg, dm)
        xres[pl.ds(pl.multiple_of(p * x_chunk * seg, x_chunk * seg), x_chunk * seg), :] = wide
        return carry

    with jax.named_scope("load"):
        lax.fori_loop(0, n_pairs, load_pair, 0)

    def fold_phi(base):
        groups = [None] * n_grp
        for j, g0 in enumerate(first_grp):
            t = _nt(fold[j], bqkv_stage[:, base + j * 128:base + (j + 1) * 128]) * LOG2E
            for i in range(4):
                part = t[i * gw:(i + 1) * gw]
                groups[g0 + i] = part if groups[g0 + i] is None else groups[g0 + i] + part
        return groups

    bqkv_copy.wait()
    bwo_copy.wait()
    wvt = bqkv_stage[:, 2 * dm:].astype(F32).T
    for g, (wpq, wpk) in enumerate(zip(fold_phi(0), fold_phi(dm))):
        bwq[g * gw:(g + 1) * gw, :] = wpq
        bw1[2 * g * gw:(2 * g + 1) * gw, :] = wpk
        bw1[(2 * g + 1) * gw:(2 * g + 2) * gw, :] = wvt[g * gw:(g + 1) * gw]
    bwo[...] = _pack(bwo_stage[...])

    def seg_rows(s):
        return pl.ds(pl.multiple_of(s * seg, seg), seg)

    def rmt_step(s, mem, early):
        if early:
            h = jnp.concatenate([mem, xn_a[:seg - EARLY_ROWS, :]], axis=0).astype(BF16)
            early_rows = pl.ds(pl.multiple_of(s * EARLY_ROWS, EARLY_ROWS), EARLY_ROWS)
        else:
            h = jnp.concatenate([mem, xn_a[...]], axis=0)
        xn_next = _layernorm(xres[seg_rows(jnp.minimum(s + 1, n_seg - 1)), :])
        prev = seg_rows(jnp.maximum(s - 1, 0))
        xn_b[prev, :] = _layernorm(xres[prev, :]).astype(BF16)
        pending = {1: xn_b[seg_rows(jnp.maximum(s, 1) - 1), :128][:16].astype(F32)[:8]}

        def weighted_values(p, prob, v):
            head = prob[:n_mem]
            if p in pending:
                head = jnp.where(s < 0, pending[p][:, :prob.shape[1]], head)
            if p not in (VPU_PAIRS_EARLY if early else VPU_PAIRS):
                return _nn(jnp.concatenate([head, prob[n_mem:]], axis=0), _pair_blockdiag(v, dh))
            seen = n_mem + 8
            o = _nn(jnp.concatenate([head, prob[seen:]], axis=0), _pair_blockdiag(v, dh))
            v_scr[p] = v[:seen]
            first = prob[n_mem:seen]
            lane = _iota(first.shape, 1)
            tiles = [None] * (pw // 128)
            for k in range(seen):
                wa, wb = (jnp.sum(jnp.where(lane == col, first, 0.0), axis=1, keepdims=True)
                          for col in (k, prob.shape[0] + k))
                for t in range(pw // 128):
                    c = t * 128
                    w = wa if c + 128 <= dh else wb if c >= dh else jnp.where(
                        _iota((8, 128), 1) < dh - c, wa, wb)
                    term = w * jnp.broadcast_to(v_scr[p, k:k + 1, c:c + 128], (8, 128))
                    tiles[t] = term if tiles[t] is None else tiles[t] + term
            pending[p + 1] = functools.reduce(jnp.add, tiles + ([pending[p + 1]] if p + 1 in pending else []))
            return jnp.concatenate([o[:n_mem], jnp.concatenate(tiles, axis=1), o[n_mem:]], axis=0)

        plan = OUT_PLAN_EARLY if early else OUT_PLAN
        ks = 256
        qkv, prob = {}, {}
        acc, done = None, 0

        def out_proj(acc, lo, hi):
            t = _nn(o_scr[:, lo * pw:hi * pw], _unpack(wo[lo * half:hi * half, :]))
            return t if acc is None else t + acc

        depth = len(plan) - n_pairs
        for p in range(n_pairs + depth):
            if p == 0:
                start = _nn(h[:, :ks], _unpack(wqkv[p, :ks // 2, :]))
                qkv[p] = _nn(h[:, ks:], _unpack(wqkv[p, ks // 2:, :])) + start
            elif p < n_pairs:
                qkv[p] = _nn(h, _unpack(wqkv[p]))
            if p < n_pairs:
                if early:
                    qkv[p] = jnp.concatenate([qkv[p], early_qkv[p, early_rows, :]], axis=0)
            n = int(plan[p])
            if n:
                acc = out_proj(acc, done, done + n)
                done += n
            if 0 <= p - 1 < n_pairs:
                t = qkv[p - 1]
                scores = _nt(t[:, :pw], _pair_blockdiag(t[:, pw:2 * pw], dh))
                prob[p - 1] = _pair_softmax(scores, n_mem, scale)
            r = p - depth
            if r >= 0:
                o_scr[:, r * pw:(r + 1) * pw] = weighted_values(r, prob[r], qkv[r][:, 2 * pw:])
        acc = out_proj(acc, done, n_pairs - 1)
        o_last = o_scr[:, (n_pairs - 1) * pw:]
        acc = jnp.concatenate(
            [acc[:, cols] + _nn(o_last, _unpack(wo[(n_pairs - 1) * half:, cols]))
             for cols in (slice(0, ks), slice(ks, dm))], axis=1)
        xn_a[...] = xn_next
        rows = seg_rows(s)
        xres[rows, :] = xres[rows, :] + acc[n_mem:]
        return acc[:n_mem]

    def rmt_steps(lo, hi, mem, early):
        def body(i, mem):
            for u in range(unroll):
                mem = rmt_step(i * unroll + u, mem, early)
            return mem

        return lax.fori_loop(lo, hi, body, mem)

    def rmt_layer(layer):
        xn_a[...] = _layernorm(xres[0:seg, :])
        split = jnp.where(layer == 0, n_early // unroll, 0)
        mem = rmt_steps(0, split, mem0_ref[...].astype(F32), True)
        rmt_steps(split, n_seg // unroll, mem, False)
        last = slice(seq - seg, seq)
        xn_b[last, :] = _layernorm(xres[last, :]).astype(BF16)

    chunk = 4
    n_chunk = n_grp // chunk

    def blk_rows(i):
        return pl.ds(pl.multiple_of(i * tb, tb), tb)

    def kv_block(i, carry):
        xn = xn_b[blk_rows(i), :]
        ones = jnp.ones((8, tb), F32)
        proj = {}
        for c in range(n_chunk + 1):
            if c < n_chunk:
                proj[c] = _nt(bw1[2 * c * chunk * gw:2 * (c + 1) * chunk * gw, :], xn)
            if c >= 1:
                t = proj[c - 1]
                for j in range(chunk):
                    g = (c - 1) * chunk + j
                    phi = _feature_map(t[2 * j * gw:(2 * j + 1) * gw])
                    lhs = jnp.concatenate([t[(2 * j + 1) * gw:(2 * j + 2) * gw], ones], axis=0)
                    kv_acc[g] += _nt(lhs, phi)
        return carry

    def out_copy(i):
        return pltpu.make_async_copy(out_stage.at[blk_rows(i)], out_hbm.at[blk_rows(i)], out_sem.at[i])

    def out_block(i, layer):
        rows = blk_rows(i)
        xn = xn_b[rows, :]
        first8 = _iota((8, tb), 0) < 4
        proj, outs = {}, []

        def out_proj(y, lo, hi):
            o = jnp.concatenate(outs, axis=0)[lo:hi].astype(BF16).T
            return _nn(o, _unpack(bwo[lo // 2:hi // 2, :])) + y

        y = xres[rows, :]
        for c in range(n_chunk + 1):
            if c < n_chunk:
                proj[c] = _nt(bwq[c * chunk * gw:(c + 1) * chunk * gw, :], xn)
            else:
                y = out_proj(y, 0, 256)
            if c >= 1:
                t = proj[c - 1]
                for j in range(chunk):
                    g = (c - 1) * chunk + j
                    nd = _nn(kv_mat[g], _feature_map(t[j * gw:(j + 1) * gw]))
                    inv = 1.0 / (nd[gw:] + DEN_EPS)
                    swapped = pltpu.roll(inv, 4, 0)
                    inv_a = jnp.where(first8, inv, swapped)
                    inv_b = jnp.where(first8, swapped, inv)
                    outs.append(nd[:gw] * jnp.concatenate([inv_a, inv_a, inv, inv_b, inv_b], axis=0))
        y = out_proj(out_proj(y, 256, 384), 384, dm)
        xres[rows, :] = y
        out_stage[rows, :] = y.astype(BF16)

        @pl.when(layer == n_layers - 1)
        def _():
            out_copy(i).start()

        return layer

    def hedgehog_layer(layer):
        kv_acc[...] = jnp.zeros(kv_acc.shape, F32)
        lax.fori_loop(0, seq // tb, kv_block, 0)
        shape = kv_acc.shape[1:]
        r = _iota(shape, 0)
        row_head = jnp.where(r < gw, r // bdh, (r - gw) // 4)
        same_head = row_head == _iota(shape, 1) % 2
        for g in range(n_grp):
            kv_mat[g] = jnp.where(same_head, kv_acc[g], 0.0)
        lax.fori_loop(0, seq // tb, out_block, layer)

    def layer_pair(layer, carry):
        with jax.named_scope("rmt"):
            rmt_layer(layer)
        with jax.named_scope("hedgehog"):
            hedgehog_layer(layer)
        return carry

    lax.fori_loop(0, n_layers, layer_pair, 0)
    for i in range(seq // tb):
        out_copy(i).wait()


@functools.partial(jax.jit, static_argnames=("A_seg_len",))
def pallas_interleave_layers__memory_aug_recurrent_mem_tr__linear_kernel_hedgehog__prompt_kernel(
    A_x: jax.Array,
    A_mem0: jax.Array,
    A_Wq: jax.Array,
    A_Wk: jax.Array,
    A_Wv: jax.Array,
    A_Wo: jax.Array,
    A_seg_len: int,
    B_x: jax.Array,
    B_wqkv: jax.Array,
    B_w_phi: jax.Array,
    B_wo: jax.Array,
):
    del B_x
    batch, seq, dm = A_x.shape
    _, heads, dh = A_Wq.shape
    n_mem = A_mem0.shape[1]
    bh, bdh, _ = B_w_phi.shape
    seg = int(A_seg_len)
    assert batch == 1 and bdh == 20 and bh * bdh == dm and heads % 2 == 0
    assert (2 * dh) % 128 == 0 and n_mem % 8 == 0 and seg % 16 == 0 and 2 * (n_mem + seg) <= 128
    n_pairs, pw, hd = heads // 2, 2 * dh, heads * dh
    tb, unroll, n_early = 512, 2, 48

    def feature_major(w):
        return jnp.transpose(w, (1, 2, 0)).reshape(hd, dm)

    hbm = pl.BlockSpec(memory_space=pl.ANY)
    vmem = pl.BlockSpec(memory_space=pltpu.VMEM)
    out = pl.pallas_call(
        functools.partial(_kernel, seg=seg, dh=dh, n_layers=2, tb=tb, unroll=unroll),
        out_shape=jax.ShapeDtypeStruct((seq, dm), A_x.dtype),
        in_specs=[hbm, vmem, hbm, hbm, hbm, hbm, hbm, vmem, hbm],
        out_specs=hbm,
        scratch_shapes=[
            pltpu.VMEM((4, hd, dm), BF16),
            pltpu.VMEM((n_pairs, dm // 2, 3 * pw), U32),
            pltpu.VMEM((hd // 2, dm), U32),
            pltpu.VMEM((seq // seg, seg, dm), BF16),
            pltpu.VMEM((seq, dm), BF16),
            pltpu.VMEM((dm, 3 * dm), BF16),
            pltpu.VMEM((dm, dm), BF16),
            pltpu.VMEM((dm // 128, 8 * bdh, 128), BF16),
            pltpu.VMEM((2 * dm, dm), F32),
            pltpu.VMEM((dm, dm), F32),
            pltpu.VMEM((dm // 2, dm), U32),
            pltpu.VMEM((seq, dm), F32),
            pltpu.VMEM((seg, dm), F32),
            pltpu.VMEM((seq, dm), BF16),
            pltpu.VMEM((n_mem + seg, hd), F32),
            pltpu.VMEM((n_pairs, n_mem + 8, pw), F32),
            pltpu.VMEM((bh // 2, 2 * bdh + 8, 4 * bdh), F32),
            pltpu.VMEM((bh // 2, 2 * bdh + 8, 4 * bdh), F32),
            pltpu.VMEM((n_early, EARLY_ROWS, dm), BF16),
            pltpu.VMEM((n_early * EARLY_ROWS, dm), BF16),
            pltpu.VMEM((n_pairs, n_early * EARLY_ROWS, 3 * pw), F32),
            pltpu.SemaphoreType.DMA((5, n_pairs)),
            pltpu.SemaphoreType.DMA((3,)),
            pltpu.SemaphoreType.DMA((seq // tb,)),
        ],
        compiler_params=pltpu.CompilerParams(vmem_limit_bytes=120 * 1024 * 1024),
        name="rmt_hedgehog",
    )(
        A_x.reshape(seq // seg, seg, dm),
        A_mem0.reshape(n_mem, dm),
        feature_major(A_Wq),
        feature_major(A_Wk),
        feature_major(A_Wv),
        A_Wo.reshape(hd, dm),
        B_wqkv,
        jnp.transpose(B_w_phi, (1, 2, 0)),
        B_wo,
    )
    return out.reshape(batch, seq, dm)
```

```python
import functools
import math

import jax
import jax.numpy as jnp
from jax import lax
import jax.experimental.pallas as pl
import jax.experimental.pallas.tpu as pltpu

F32 = jnp.float32
BF16 = jnp.bfloat16
U32 = jnp.uint32
I32 = jnp.int32

LN_EPS = 1e-5
DEN_EPS = 1e-6
LOG2E = math.log2(math.e)
EARLY_ROWS = 8
OUT_PLAN = "0000000011111111222"
OUT_PLAN_EARLY = "0000000011111111222"
VPU_PAIRS = range(0, 15)
VPU_PAIRS_EARLY = range(0, 15)


def _nn(a, b):
    return lax.dot_general(a, b, (((1,), (0,)), ((), ())), preferred_element_type=F32)


def _nt(a, b):
    return lax.dot_general(a, b, (((1,), (1,)), ((), ())), preferred_element_type=F32)


def _unpack(x):
    return pltpu.bitcast(x, BF16)


def _pack(x):
    return pltpu.bitcast(x, U32)


def _iota(shape, dim):
    return lax.broadcasted_iota(I32, shape, dim)


def _layernorm(x):
    inv_n = 1.0 / x.shape[-1]
    m = jnp.sum(x, axis=-1, keepdims=True) * inv_n
    d = x - m
    v = jnp.sum(d * d, axis=-1, keepdims=True) * inv_n
    return d * lax.rsqrt(v + LN_EPS)


def _pair_blockdiag(x, dh):
    rows, width = x.shape
    top, bot = [], []
    zero = jnp.zeros((rows, 128), F32)
    for c in range(0, width, 128):
        t = x[:, c:c + 128]
        if c + 128 <= dh:
            top.append(t)
            bot.append(zero)
        elif c >= dh:
            top.append(zero)
            bot.append(t)
        else:
            first = _iota((rows, 128), 1) < dh - c
            top.append(jnp.where(first, t, 0.0))
            bot.append(jnp.where(first, 0.0, t))
    return jnp.concatenate(
        [jnp.concatenate(top, axis=1), jnp.concatenate(bot, axis=1)], axis=0
    ).astype(BF16)


def _pair_softmax(s, n_mem, scale):
    rows = s.shape[0]
    row = _iota(s.shape, 0)
    col = _iota(s.shape, 1)
    is_a = col < rows
    key = jnp.where(is_a, col, col - rows)
    s = jnp.where((row < n_mem) | (row >= key), s * scale, -1000000000.0)
    ma = jnp.max(jnp.where(is_a, s, -jnp.inf), axis=1, keepdims=True)
    mb = jnp.max(jnp.where(is_a, -jnp.inf, s), axis=1, keepdims=True)
    e = jnp.exp(s - jnp.where(is_a, ma, mb))
    la = jnp.sum(jnp.where(is_a, e, 0.0), axis=1, keepdims=True)
    lb = jnp.sum(jnp.where(is_a, 0.0, e), axis=1, keepdims=True)
    return e / jnp.where(is_a, la, lb)


def _over_features(x, op):
    r = functools.reduce(op, [x[i:i + 8] for i in range(0, x.shape[0], 8)])
    r = op(r, pltpu.roll(r, 4, 0))
    return op(r, pltpu.roll(r, 2, 0))


def _feature_map(p):
    def tile(r):
        return jnp.concatenate([r] * (p.shape[0] // 8), axis=0)

    ep = jnp.exp2(p - tile(_over_features(p, jnp.maximum)))
    en = jnp.exp2(tile(_over_features(p, jnp.minimum)) - p)
    return jnp.concatenate([e * tile(1.0 / _over_features(e, jnp.add)) for e in (ep, en)], axis=0)


def _kernel(x_hbm, mem0_ref, wq_hbm, wk_hbm, wv_hbm, wo_hbm, bqkv_hbm, wphi_ref, bwo_hbm,
            out_hbm,
            stage, wqkv, wo, x_stage, out_stage, bqkv_stage, bwo_stage, fold, bw1, bwq, bwo,
            xres, xn_a, xn_b, o_scr, v_scr, kv_acc, z_acc, early_x, early_xn, early_qkv,
            w_sem, b_sem, out_sem,
            *, seg, dh, n_layers, tb, unroll):
    n_pairs = wqkv.shape[0]
    pw = 2 * dh
    half = pw // 2
    seq, dm = xres.shape
    n_mem = mem0_ref.shape[0]
    n_seg = seq // seg
    scale = dh ** -0.5
    bdh, _, bh = wphi_ref.shape
    n_grp = bh // 2
    gw = 2 * bdh
    n_early = early_xn.shape[0] // EARLY_ROWS

    x_chunk = n_seg // n_pairs

    def pair_rows(p):
        return pl.ds(pl.multiple_of(p * pw, pw), pw)

    def pair_copies(p):
        rows = pair_rows(p)
        segs = pl.ds(p * x_chunk, x_chunk)
        return [pltpu.make_async_copy(src.at[rows], stage.at[i, rows], w_sem.at[i, p])
                for i, src in enumerate((wq_hbm, wk_hbm, wv_hbm, wo_hbm))] + [
            pltpu.make_async_copy(x_hbm.at[segs], x_stage.at[segs], w_sem.at[4, p])]

    early_copy = pltpu.make_async_copy(
        x_hbm.at[pl.ds(0, n_early), pl.ds(seg - EARLY_ROWS, EARLY_ROWS)], early_x, b_sem.at[0])
    bqkv_copy = pltpu.make_async_copy(bqkv_hbm, bqkv_stage, b_sem.at[1])
    bwo_copy = pltpu.make_async_copy(bwo_hbm, bwo_stage, b_sem.at[2])
    early_copy.start()
    for c in pair_copies(0):
        c.start()

    wphi = wphi_ref[...].astype(F32)
    wf = jnp.concatenate([wphi[d] for d in range(bdh)], axis=1)
    src = _iota((dm, 128), 0)
    natural = (src % bh) * bdh + src // bh
    first_grp = [c // gw for c in range(0, dm, 128)]
    r = _iota((4 * gw, 128), 0)
    lane = _iota((4 * gw, 128), 1)
    pick = ((r % gw) // 2 == lane).astype(BF16)
    head_start = ((r // gw) * 2 + r % 2) * bdh
    for j, g0 in enumerate(first_grp):
        wj = _nn(wf, (natural == _iota((dm, 128), 1) + j * 128).astype(BF16))
        wj = jnp.concatenate([wj, jnp.zeros((128 - bdh, 128), F32)], axis=0).astype(BF16)
        d = lane + (j * 128 - g0 * gw) - head_start
        fold[j] = jnp.where((d >= 0) & (d < bdh), _nn(pick, wj), 0.0).astype(BF16)

    early_copy.wait()
    for c in pair_copies(1):
        c.start()
    early_xn[...] = _layernorm(
        early_x[...].astype(F32).reshape(n_early * EARLY_ROWS, dm)).astype(BF16)

    def load_pair(p, carry):
        for c in pair_copies(p):
            c.wait()

        @pl.when(p + 2 < n_pairs)
        def _():
            for c in pair_copies(p + 2):
                c.start()

        pl.when(p == n_pairs // 2)(bqkv_copy.start)
        pl.when(p == n_pairs - 3)(bwo_copy.start)
        for i in range(3):
            w = stage[i, pair_rows(p), :]
            early_qkv[p, :, i * pw:(i + 1) * pw] = _nt(early_xn[...], w)
            wqkv[p, :, i * pw:(i + 1) * pw] = _pack(w.T)
        wo[pl.ds(pl.multiple_of(p * half, half), half), :] = _pack(stage[3, pair_rows(p), :])
        wide = x_stage[pl.ds(p * x_chunk, x_chunk)].astype(F32).reshape(x_chunk * seg, dm)
        xres[pl.ds(pl.multiple_of(p * x_chunk * seg, x_chunk * seg), x_chunk * seg), :] = wide
        return carry

    with jax.named_scope("load"):
        lax.fori_loop(0, n_pairs, load_pair, 0)

    def fold_phi(base):
        groups = [None] * n_grp
        for j, g0 in enumerate(first_grp):
            t = _nt(fold[j], bqkv_stage[:, base + j * 128:base + (j + 1) * 128]) * LOG2E
            for i in range(4):
                part = t[i * gw:(i + 1) * gw]
                groups[g0 + i] = part if groups[g0 + i] is None else groups[g0 + i] + part
        return groups

    bqkv_copy.wait()
    bwo_copy.wait()
    wvt = bqkv_stage[:, 2 * dm:].astype(F32).T
    for g, (wpq, wpk) in enumerate(zip(fold_phi(0), fold_phi(dm))):
        bwq[g * gw:(g + 1) * gw, :] = wpq
        bw1[2 * g * gw:(2 * g + 1) * gw, :] = wpk
        bw1[(2 * g + 1) * gw:(2 * g + 2) * gw, :] = wvt[g * gw:(g + 1) * gw]
    bwo[...] = _pack(bwo_stage[...])

    def seg_rows(s):
        return pl.ds(pl.multiple_of(s * seg, seg), seg)

    def rmt_step(s, mem, early):
        if early:
            h = jnp.concatenate([mem, xn_a[:seg - EARLY_ROWS, :]], axis=0).astype(BF16)
            early_rows = pl.ds(pl.multiple_of(s * EARLY_ROWS, EARLY_ROWS), EARLY_ROWS)
        else:
            h = jnp.concatenate([mem, xn_a[...]], axis=0)
        xn_next = _layernorm(xres[seg_rows(jnp.minimum(s + 1, n_seg - 1)), :])
        prev = seg_rows(jnp.maximum(s - 1, 0))
        xn_b[prev, :] = _layernorm(xres[prev, :]).astype(BF16)
        pending = {1: xn_b[seg_rows(jnp.maximum(s, 1) - 1), :128][:16].astype(F32)[:8]}

        def weighted_values(p, prob, v):
            head = prob[:n_mem]
            if p in pending:
                head = jnp.where(s < 0, pending[p][:, :prob.shape[1]], head)
            if p not in (VPU_PAIRS_EARLY if early else VPU_PAIRS):
                return _nn(jnp.concatenate([head, prob[n_mem:]], axis=0), _pair_blockdiag(v, dh))
            seen = n_mem + 8
            o = _nn(jnp.concatenate([head, prob[seen:]], axis=0), _pair_blockdiag(v, dh))
            v_scr[p] = v[:seen]
            first = prob[n_mem:seen]
            first = jnp.concatenate([first, jnp.zeros((8, 128 - first.shape[1]), F32)], axis=1)
            lane = _iota(first.shape, 1)
            tiles = [None] * (pw // 128)
            for k in range(seen):
                wa, wb = (jnp.sum(jnp.where(lane == col, first, 0.0), axis=1, keepdims=True)
                          for col in (k, prob.shape[0] + k))
                for t in range(pw // 128):
                    c = t * 128
                    w = wa if c + 128 <= dh else wb if c >= dh else jnp.where(
                        _iota((8, 128), 1) < dh - c, wa, wb)
                    term = w * jnp.broadcast_to(v_scr[p, k:k + 1, c:c + 128], (8, 128))
                    tiles[t] = term if tiles[t] is None else tiles[t] + term
            pending[p + 1] = functools.reduce(jnp.add, tiles + ([pending[p + 1]] if p + 1 in pending else []))
            return jnp.concatenate([o[:n_mem], jnp.concatenate(tiles, axis=1), o[n_mem:]], axis=0)

        plan = OUT_PLAN_EARLY if early else OUT_PLAN
        ks = 256
        qkv, prob = {}, {}
        acc, done = None, 0

        def out_proj(acc, lo, hi):
            t = _nn(o_scr[:, lo * pw:hi * pw], _unpack(wo[lo * half:hi * half, :]))
            return t if acc is None else t + acc

        depth = len(plan) - n_pairs
        for p in range(n_pairs + depth):
            if p == 0:
                start = _nn(h[:, :ks], _unpack(wqkv[p, :ks // 2, :]))
                qkv[p] = _nn(h[:, ks:], _unpack(wqkv[p, ks // 2:, :])) + start
            elif p < n_pairs:
                qkv[p] = _nn(h, _unpack(wqkv[p]))
            if p < n_pairs:
                if early:
                    qkv[p] = jnp.concatenate([qkv[p], early_qkv[p, early_rows, :]], axis=0)
            n = int(plan[p])
            if n:
                acc = out_proj(acc, done, done + n)
                done += n
            if 0 <= p - 1 < n_pairs:
                t = qkv[p - 1]
                scores = _nt(t[:, :pw], _pair_blockdiag(t[:, pw:2 * pw], dh))
                prob[p - 1] = _pair_softmax(scores, n_mem, scale)
            r = p - depth
            if r >= 0:
                o_scr[:, r * pw:(r + 1) * pw] = weighted_values(r, prob[r], qkv[r][:, 2 * pw:])
        acc = out_proj(acc, done, n_pairs - 1)
        o_last = o_scr[:, (n_pairs - 1) * pw:]
        acc = jnp.concatenate(
            [acc[:, cols] + _nn(o_last, _unpack(wo[(n_pairs - 1) * half:, cols]))
             for cols in (slice(0, ks), slice(ks, dm))], axis=1)
        xn_a[...] = xn_next
        rows = seg_rows(s)
        xres[rows, :] = xres[rows, :] + acc[n_mem:]
        return acc[:n_mem]

    def rmt_steps(lo, hi, mem, early):
        def body(i, mem):
            for u in range(unroll):
                mem = rmt_step(i * unroll + u, mem, early)
            return mem

        return lax.fori_loop(lo, hi, body, mem)

    def rmt_layer(layer):
        xn_a[...] = _layernorm(xres[0:seg, :])
        split = jnp.where(layer == 0, n_early // unroll, 0)
        mem = rmt_steps(0, split, mem0_ref[...].astype(F32), True)
        rmt_steps(split, n_seg // unroll, mem, False)
        last = slice(seq - seg, seq)
        xn_b[last, :] = _layernorm(xres[last, :]).astype(BF16)

    chunk = 4
    n_chunk = n_grp // chunk

    def blk_rows(i):
        return pl.ds(pl.multiple_of(i * tb, tb), tb)

    def kv_block(i, carry):
        xn = xn_b[blk_rows(i), :]
        proj = {}
        for c in range(n_chunk + 1):
            if c < n_chunk:
                proj[c] = _nt(bw1[2 * c * chunk * gw:2 * (c + 1) * chunk * gw, :], xn)
            if c >= 1:
                t = proj[c - 1]
                for j in range(chunk):
                    g = (c - 1) * chunk + j
                    phi = _feature_map(t[2 * j * gw:(2 * j + 1) * gw])
                    kv_acc[g] += _nt(t[(2 * j + 1) * gw:(2 * j + 2) * gw], phi.astype(BF16))
                    z_acc[g] += functools.reduce(jnp.add, [phi[:, i:i + 128] for i in range(0, tb, 128)])
        return carry

    def out_copy(i):
        return pltpu.make_async_copy(out_stage.at[blk_rows(i)], out_hbm.at[blk_rows(i)], out_sem.at[i])

    def out_block(i, layer):
        rows = blk_rows(i)
        xn = xn_b[rows, :]
        sublane = _iota((8, tb), 0)
        proj, outs = {}, []

        def out_proj(y, lo, hi):
            o = jnp.concatenate(outs, axis=0)[lo:hi].astype(BF16).T
            return _nn(o, _unpack(bwo[lo // 2:hi // 2, :])) + y

        y = xres[rows, :]
        for c in range(n_chunk + 1):
            if c < n_chunk:
                proj[c] = _nt(bwq[c * chunk * gw:(c + 1) * chunk * gw, :], xn)
            else:
                y = out_proj(y, 0, 256)
            if c >= 1:
                t = proj[c - 1]
                for j in range(chunk):
                    g = (c - 1) * chunk + j
                    phi = _feature_map(t[j * gw:(j + 1) * gw])
                    z = jnp.concatenate([z_acc[g]] * (tb // 128), axis=1)
                    inv = 1.0 / (_over_features(phi * z, jnp.add) + DEN_EPS)
                    swapped = pltpu.roll(inv, 1, 0)
                    inv_a = jnp.where(sublane % 2 == 0, inv, swapped)
                    inv_b = jnp.where(sublane % 2 == 0, swapped, inv)
                    inv_ab = jnp.where(sublane < bdh % 8, inv_a, inv_b)
                    outs.append(_nn(kv_acc[g], phi.astype(BF16))
                                * jnp.concatenate([inv_a, inv_a, inv_ab, inv_b, inv_b], axis=0))
        y = out_proj(out_proj(y, 256, 384), 384, dm)
        xres[rows, :] = y
        out_stage[rows, :] = y.astype(BF16)

        @pl.when(layer == n_layers - 1)
        def _():
            out_copy(i).start()

        return layer

    def hedgehog_layer(layer):
        kv_acc[...] = jnp.zeros(kv_acc.shape, F32)
        z_acc[...] = jnp.zeros(z_acc.shape, F32)
        lax.fori_loop(0, seq // tb, kv_block, 0)
        shape = kv_acc.shape[1:]
        same_head = _iota(shape, 0) // bdh == _iota(shape, 1) % 2
        for g in range(n_grp):
            kv_acc[g] = jnp.where(same_head, kv_acc[g], 0.0)
            z_acc[g] = jnp.broadcast_to(jnp.sum(z_acc[g], axis=1, keepdims=True), z_acc.shape[1:])
        lax.fori_loop(0, seq // tb, out_block, layer)

    def layer_pair(layer, carry):
        with jax.named_scope("rmt"):
            rmt_layer(layer)
        with jax.named_scope("hedgehog"):
            hedgehog_layer(layer)
        return carry

    lax.fori_loop(0, n_layers, layer_pair, 0)
    for i in range(seq // tb):
        out_copy(i).wait()


@functools.partial(jax.jit, static_argnames=("A_seg_len",))
def pallas_interleave_layers__memory_aug_recurrent_mem_tr__linear_kernel_hedgehog__prompt_kernel(
    A_x: jax.Array,
    A_mem0: jax.Array,
    A_Wq: jax.Array,
    A_Wk: jax.Array,
    A_Wv: jax.Array,
    A_Wo: jax.Array,
    A_seg_len: int,
    B_x: jax.Array,
    B_wqkv: jax.Array,
    B_w_phi: jax.Array,
    B_wo: jax.Array,
):
    del B_x
    batch, seq, dm = A_x.shape
    _, heads, dh = A_Wq.shape
    n_mem = A_mem0.shape[1]
    bh, bdh, _ = B_w_phi.shape
    seg = int(A_seg_len)
    assert batch == 1 and bdh == 20 and bh * bdh == dm and heads % 2 == 0
    assert (2 * dh) % 128 == 0 and n_mem % 8 == 0 and seg % 16 == 0 and 2 * (n_mem + seg) <= 128
    n_pairs, pw, hd = heads // 2, 2 * dh, heads * dh
    tb, unroll, n_early = 512, 2, 48

    def feature_major(w):
        return jnp.transpose(w, (1, 2, 0)).reshape(hd, dm)

    hbm = pl.BlockSpec(memory_space=pl.ANY)
    vmem = pl.BlockSpec(memory_space=pltpu.VMEM)
    out = pl.pallas_call(
        functools.partial(_kernel, seg=seg, dh=dh, n_layers=2, tb=tb, unroll=unroll),
        out_shape=jax.ShapeDtypeStruct((seq, dm), A_x.dtype),
        in_specs=[hbm, vmem, hbm, hbm, hbm, hbm, hbm, vmem, hbm],
        out_specs=hbm,
        scratch_shapes=[
            pltpu.VMEM((4, hd, dm), BF16),
            pltpu.VMEM((n_pairs, dm // 2, 3 * pw), U32),
            pltpu.VMEM((hd // 2, dm), U32),
            pltpu.VMEM((seq // seg, seg, dm), BF16),
            pltpu.VMEM((seq, dm), BF16),
            pltpu.VMEM((dm, 3 * dm), BF16),
            pltpu.VMEM((dm, dm), BF16),
            pltpu.VMEM((dm // 128, 8 * bdh, 128), BF16),
            pltpu.VMEM((2 * dm, dm), F32),
            pltpu.VMEM((dm, dm), F32),
            pltpu.VMEM((dm // 2, dm), U32),
            pltpu.VMEM((seq, dm), F32),
            pltpu.VMEM((seg, dm), F32),
            pltpu.VMEM((seq, dm), BF16),
            pltpu.VMEM((n_mem + seg, hd), F32),
            pltpu.VMEM((n_pairs, n_mem + 8, pw), F32),
            pltpu.VMEM((bh // 2, 2 * bdh, 4 * bdh), F32),
            pltpu.VMEM((bh // 2, 4 * bdh, 128), F32),
            pltpu.VMEM((n_early, EARLY_ROWS, dm), BF16),
            pltpu.VMEM((n_early * EARLY_ROWS, dm), BF16),
            pltpu.VMEM((n_pairs, n_early * EARLY_ROWS, 3 * pw), F32),
            pltpu.SemaphoreType.DMA((5, n_pairs)),
            pltpu.SemaphoreType.DMA((3,)),
            pltpu.SemaphoreType.DMA((seq // tb,)),
        ],
        compiler_params=pltpu.CompilerParams(vmem_limit_bytes=120 * 1024 * 1024),
        name="rmt_hedgehog",
    )(
        A_x.reshape(seq // seg, seg, dm),
        A_mem0.reshape(n_mem, dm),
        feature_major(A_Wq),
        feature_major(A_Wk),
        feature_major(A_Wv),
        A_Wo.reshape(hd, dm),
        B_wqkv,
        jnp.transpose(B_w_phi, (1, 2, 0)),
        B_wo,
    )
    return out.reshape(batch, seq, dm)
```

```python
import functools
import math

import jax
import jax.numpy as jnp
from jax import lax
import jax.experimental.pallas as pl
import jax.experimental.pallas.tpu as pltpu

F32 = jnp.float32
BF16 = jnp.bfloat16
U32 = jnp.uint32
I32 = jnp.int32

LN_EPS = 1e-5
DEN_EPS = 1e-6
LOG2E = math.log2(math.e)
EARLY_ROWS = 8
OUT_PLAN = "0000000011111111222"
OUT_PLAN_EARLY = "0000000011111111222"
VPU_PAIRS = range(0, 15)
VPU_PAIRS_EARLY = range(0, 15)


def _nn(a, b):
    return lax.dot_general(a, b, (((1,), (0,)), ((), ())), preferred_element_type=F32)


def _nt(a, b):
    return lax.dot_general(a, b, (((1,), (1,)), ((), ())), preferred_element_type=F32)


def _unpack(x):
    return pltpu.bitcast(x, BF16)


def _pack(x):
    return pltpu.bitcast(x, U32)


def _iota(shape, dim):
    return lax.broadcasted_iota(I32, shape, dim)


def _recip(x):
    r = pltpu.reciprocal(x, approx=True)
    return r * (2.0 - x * r)


def _layernorm(x):
    inv_n = 1.0 / x.shape[-1]
    m = jnp.sum(x, axis=-1, keepdims=True) * inv_n
    d = x - m
    v = jnp.sum(d * d, axis=-1, keepdims=True) * inv_n
    return d * lax.rsqrt(v + LN_EPS)


def _pair_blockdiag(x, dh):
    rows, width = x.shape
    top, bot = [], []
    zero = jnp.zeros((rows, 128), F32)
    for c in range(0, width, 128):
        t = x[:, c:c + 128]
        if c + 128 <= dh:
            top.append(t)
            bot.append(zero)
        elif c >= dh:
            top.append(zero)
            bot.append(t)
        else:
            first = _iota((rows, 128), 1) < dh - c
            top.append(jnp.where(first, t, 0.0))
            bot.append(jnp.where(first, 0.0, t))
    return jnp.concatenate(
        [jnp.concatenate(top, axis=1), jnp.concatenate(bot, axis=1)], axis=0
    ).astype(BF16)


def _pair_softmax(s, n_mem, scale):
    rows = s.shape[0]
    row = _iota(s.shape, 0)
    col = _iota(s.shape, 1)
    is_a = col < rows
    key = jnp.where(is_a, col, col - rows)
    s = jnp.where((row < n_mem) | (row >= key), s * scale, -1000000000.0)
    ma = jnp.max(jnp.where(is_a, s, -jnp.inf), axis=1, keepdims=True)
    mb = jnp.max(jnp.where(is_a, -jnp.inf, s), axis=1, keepdims=True)
    e = jnp.exp(s - jnp.where(is_a, ma, mb))
    la = jnp.sum(jnp.where(is_a, e, 0.0), axis=1, keepdims=True)
    lb = jnp.sum(jnp.where(is_a, 0.0, e), axis=1, keepdims=True)
    return e / jnp.where(is_a, la, lb)


def _over_features(x, op):
    r = functools.reduce(op, [x[i:i + 8] for i in range(0, x.shape[0], 8)])
    r = op(r, pltpu.roll(r, 4, 0))
    return op(r, pltpu.roll(r, 2, 0))


def _feature_map(p):
    def tile(r):
        return jnp.concatenate([r] * (p.shape[0] // 8), axis=0)

    ep = jnp.exp2(p - tile(_over_features(p, jnp.maximum)))
    en = jnp.exp2(tile(_over_features(p, jnp.minimum)) - p)
    return jnp.concatenate([e * tile(_recip(_over_features(e, jnp.add))) for e in (ep, en)], axis=0)


def _kernel(x_hbm, mem0_ref, wq_hbm, wk_hbm, wv_hbm, wo_hbm, bqkv_hbm, wphi_ref, bwo_hbm,
            out_hbm,
            stage, wqkv, wo, x_stage, out_stage, bqkv_stage, bwo_stage, fold, bw1, bwq, bwo,
            xres, xn_a, xn_b, o_scr, v_scr, kv_acc, z_acc, early_x, early_xn, early_qkv,
            w_sem, b_sem, out_sem,
            *, seg, dh, n_layers, tb, unroll):
    n_pairs = wqkv.shape[0]
    pw = 2 * dh
    half = pw // 2
    seq, dm = xres.shape
    n_mem = mem0_ref.shape[0]
    n_seg = seq // seg
    scale = dh ** -0.5
    bdh, _, bh = wphi_ref.shape
    n_grp = bh // 2
    gw = 2 * bdh
    n_early = early_xn.shape[0] // EARLY_ROWS

    x_chunk = n_seg // n_pairs

    def pair_rows(p):
        return pl.ds(pl.multiple_of(p * pw, pw), pw)

    def pair_copies(p):
        rows = pair_rows(p)
        segs = pl.ds(p * x_chunk, x_chunk)
        return [pltpu.make_async_copy(src.at[rows], stage.at[i, rows], w_sem.at[i, p])
                for i, src in enumerate((wq_hbm, wk_hbm, wv_hbm, wo_hbm))] + [
            pltpu.make_async_copy(x_hbm.at[segs], x_stage.at[segs], w_sem.at[4, p])]

    early_copy = pltpu.make_async_copy(
        x_hbm.at[pl.ds(0, n_early), pl.ds(seg - EARLY_ROWS, EARLY_ROWS)], early_x, b_sem.at[0])
    bqkv_copy = pltpu.make_async_copy(bqkv_hbm, bqkv_stage, b_sem.at[1])
    bwo_copy = pltpu.make_async_copy(bwo_hbm, bwo_stage, b_sem.at[2])
    early_copy.start()
    for c in pair_copies(0):
        c.start()

    wphi = wphi_ref[...].astype(F32)
    wf = jnp.concatenate([wphi[d] for d in range(bdh)], axis=1)
    src = _iota((dm, 128), 0)
    natural = (src % bh) * bdh + src // bh
    first_grp = [c // gw for c in range(0, dm, 128)]
    r = _iota((4 * gw, 128), 0)
    lane = _iota((4 * gw, 128), 1)
    pick = ((r % gw) // 2 == lane).astype(BF16)
    head_start = ((r // gw) * 2 + r % 2) * bdh
    for j, g0 in enumerate(first_grp):
        wj = _nn(wf, (natural == _iota((dm, 128), 1) + j * 128).astype(BF16))
        wj = jnp.concatenate([wj, jnp.zeros((128 - bdh, 128), F32)], axis=0).astype(BF16)
        d = lane + (j * 128 - g0 * gw) - head_start
        fold[j] = jnp.where((d >= 0) & (d < bdh), _nn(pick, wj), 0.0).astype(BF16)

    early_copy.wait()
    for c in pair_copies(1):
        c.start()
    early_xn[...] = _layernorm(
        early_x[...].astype(F32).reshape(n_early * EARLY_ROWS, dm)).astype(BF16)

    def load_pair(p, carry):
        for c in pair_copies(p):
            c.wait()

        def prefetch():
            @pl.when(p + 2 < n_pairs)
            def _():
                for c in pair_copies(p + 2):
                    c.start()

            pl.when(p == n_pairs // 2)(bqkv_copy.start)
            pl.when(p == n_pairs - 3)(bwo_copy.start)

        for i in range(3):
            w = stage[i, pair_rows(p), :]
            early_qkv[p, :, i * pw:(i + 1) * pw] = _nt(early_xn[...], w)
            wqkv[p, :, i * pw:(i + 1) * pw] = _pack(w.T)
            if i == 0:
                prefetch()
        wo[pl.ds(pl.multiple_of(p * half, half), half), :] = _pack(stage[3, pair_rows(p), :])
        wide = x_stage[pl.ds(p * x_chunk, x_chunk)].astype(F32).reshape(x_chunk * seg, dm)
        xres[pl.ds(pl.multiple_of(p * x_chunk * seg, x_chunk * seg), x_chunk * seg), :] = wide
        return carry

    with jax.named_scope("load"):
        lax.fori_loop(0, n_pairs, load_pair, 0)

    def fold_phi(base):
        groups = [None] * n_grp
        for j, g0 in enumerate(first_grp):
            t = _nt(fold[j], bqkv_stage[:, base + j * 128:base + (j + 1) * 128]) * LOG2E
            for i in range(4):
                part = t[i * gw:(i + 1) * gw]
                groups[g0 + i] = part if groups[g0 + i] is None else groups[g0 + i] + part
        return groups

    bqkv_copy.wait()
    bwo_copy.wait()
    wvt = bqkv_stage[:, 2 * dm:].astype(F32).T
    for g, (wpq, wpk) in enumerate(zip(fold_phi(0), fold_phi(dm))):
        bwq[g * gw:(g + 1) * gw, :] = wpq
        bw1[2 * g * gw:(2 * g + 1) * gw, :] = wpk
        bw1[(2 * g + 1) * gw:(2 * g + 2) * gw, :] = wvt[g * gw:(g + 1) * gw]
    bwo[...] = _pack(bwo_stage[...])

    def seg_rows(s):
        return pl.ds(pl.multiple_of(s * seg, seg), seg)

    def rmt_step(s, mem, early):
        if early:
            h = jnp.concatenate([mem, xn_a[:seg - EARLY_ROWS, :]], axis=0).astype(BF16)
            early_rows = pl.ds(pl.multiple_of(s * EARLY_ROWS, EARLY_ROWS), EARLY_ROWS)
        else:
            h = jnp.concatenate([mem, xn_a[...]], axis=0)
        xn_next = _layernorm(xres[seg_rows(jnp.minimum(s + 1, n_seg - 1)), :])
        prev = seg_rows(jnp.maximum(s - 1, 0))
        xn_b[prev, :] = _layernorm(xres[prev, :]).astype(BF16)
        pending = {1: xn_b[seg_rows(jnp.maximum(s, 1) - 1), :128][:16].astype(F32)[:8]}

        def weighted_values(p, prob, v):
            head = prob[:n_mem]
            if p in pending:
                head = jnp.where(s < 0, pending[p][:, :prob.shape[1]], head)
            if p not in (VPU_PAIRS_EARLY if early else VPU_PAIRS):
                return _nn(jnp.concatenate([head, prob[n_mem:]], axis=0), _pair_blockdiag(v, dh))
            seen = n_mem + 8
            o = _nn(jnp.concatenate([head, prob[seen:]], axis=0), _pair_blockdiag(v, dh))
            v_scr[p] = v[:seen]
            first = prob[n_mem:seen]
            first = jnp.concatenate([first, jnp.zeros((8, 128 - first.shape[1]), F32)], axis=1)
            lane = _iota(first.shape, 1)
            tiles = [None] * (pw // 128)
            for k in range(seen):
                wa, wb = (jnp.sum(jnp.where(lane == col, first, 0.0), axis=1, keepdims=True)
                          for col in (k, prob.shape[0] + k))
                for t in range(pw // 128):
                    c = t * 128
                    w = wa if c + 128 <= dh else wb if c >= dh else jnp.where(
                        _iota((8, 128), 1) < dh - c, wa, wb)
                    term = w * jnp.broadcast_to(v_scr[p, k:k + 1, c:c + 128], (8, 128))
                    tiles[t] = term if tiles[t] is None else tiles[t] + term
            pending[p + 1] = functools.reduce(jnp.add, tiles + ([pending[p + 1]] if p + 1 in pending else []))
            return jnp.concatenate([o[:n_mem], jnp.concatenate(tiles, axis=1), o[n_mem:]], axis=0)

        plan = OUT_PLAN_EARLY if early else OUT_PLAN
        ks = 256
        qkv, prob = {}, {}
        acc, done = None, 0

        def out_proj(acc, lo, hi):
            t = _nn(o_scr[:, lo * pw:hi * pw], _unpack(wo[lo * half:hi * half, :]))
            return t if acc is None else t + acc

        depth = len(plan) - n_pairs
        for p in range(n_pairs + depth):
            if p == 0:
                start = _nn(h[:, :ks], _unpack(wqkv[p, :ks // 2, :]))
                qkv[p] = _nn(h[:, ks:], _unpack(wqkv[p, ks // 2:, :])) + start
            elif p < n_pairs:
                qkv[p] = _nn(h, _unpack(wqkv[p]))
            if p < n_pairs:
                if early:
                    qkv[p] = jnp.concatenate([qkv[p], early_qkv[p, early_rows, :]], axis=0)
            n = int(plan[p])
            if n:
                acc = out_proj(acc, done, done + n)
                done += n
            if 0 <= p - 1 < n_pairs:
                t = qkv[p - 1]
                scores = _nt(t[:, :pw], _pair_blockdiag(t[:, pw:2 * pw], dh))
                prob[p - 1] = _pair_softmax(scores, n_mem, scale)
            r = p - depth
            if r >= 0:
                o_scr[:, r * pw:(r + 1) * pw] = weighted_values(r, prob[r], qkv[r][:, 2 * pw:])
        acc = out_proj(acc, done, n_pairs - 1)
        o_last = o_scr[:, (n_pairs - 1) * pw:]
        acc = jnp.concatenate(
            [acc[:, cols] + _nn(o_last, _unpack(wo[(n_pairs - 1) * half:, cols]))
             for cols in (slice(0, ks), slice(ks, dm))], axis=1)
        xn_a[...] = xn_next
        rows = seg_rows(s)
        xres[rows, :] = xres[rows, :] + acc[n_mem:]
        return acc[:n_mem]

    def rmt_steps(lo, hi, mem, early):
        def body(i, mem):
            for u in range(unroll):
                mem = rmt_step(i * unroll + u, mem, early)
            return mem

        return lax.fori_loop(lo, hi, body, mem)

    def rmt_layer(layer):
        xn_a[...] = _layernorm(xres[0:seg, :])
        split = jnp.where(layer == 0, n_early // unroll, 0)
        mem = rmt_steps(0, split, mem0_ref[...].astype(F32), True)
        rmt_steps(split, n_seg // unroll, mem, False)
        last = slice(seq - seg, seq)
        xn_b[last, :] = _layernorm(xres[last, :]).astype(BF16)

    chunk = 4
    n_chunk = n_grp // chunk

    def blk_rows(i):
        return pl.ds(pl.multiple_of(i * tb, tb), tb)

    def kv_block(i, carry):
        xn = xn_b[blk_rows(i), :]
        proj = {}
        for c in range(n_chunk + 1):
            if c < n_chunk:
                proj[c] = _nt(bw1[2 * c * chunk * gw:2 * (c + 1) * chunk * gw, :], xn)
            if c >= 1:
                t = proj[c - 1]
                for j in range(chunk):
                    g = (c - 1) * chunk + j
                    phi = _feature_map(t[2 * j * gw:(2 * j + 1) * gw])
                    kv_acc[g] += _nt(t[(2 * j + 1) * gw:(2 * j + 2) * gw], phi.astype(BF16))
                    z_acc[g] += functools.reduce(jnp.add, [phi[:, i:i + 128] for i in range(0, tb, 128)])
        return carry

    def out_copy(i):
        return pltpu.make_async_copy(out_stage.at[blk_rows(i)], out_hbm.at[blk_rows(i)], out_sem.at[i])

    def out_block(i, layer):
        rows = blk_rows(i)
        xn = xn_b[rows, :]
        sublane = _iota((8, tb), 0)
        proj, outs = {}, []

        def out_proj(y, lo, hi):
            o = jnp.concatenate(outs, axis=0)[lo:hi].astype(BF16).T
            return _nn(o, _unpack(bwo[lo // 2:hi // 2, :])) + y

        y = xres[rows, :]
        for c in range(n_chunk + 1):
            if c < n_chunk:
                proj[c] = _nt(bwq[c * chunk * gw:(c + 1) * chunk * gw, :], xn)
            else:
                y = out_proj(y, 0, 256)
            if c >= 1:
                for j in range(chunk):
                    g = (c - 1) * chunk + j
                    phi = _feature_map(proj[c - 1][j * gw:(j + 1) * gw])
                    z = jnp.concatenate([z_acc[g]] * (tb // 128), axis=1)
                    inv = _recip(_over_features(phi * z, jnp.add) + DEN_EPS)
                    swapped = pltpu.roll(inv, 1, 0)
                    inv_a = jnp.where(sublane % 2 == 0, inv, swapped)
                    inv_b = jnp.where(sublane % 2 == 0, swapped, inv)
                    inv_ab = jnp.where(sublane < bdh % 8, inv_a, inv_b)
                    outs.append(_nn(kv_acc[g], phi.astype(BF16))
                                * jnp.concatenate([inv_a, inv_a, inv_ab, inv_b, inv_b], axis=0))
        y = out_proj(out_proj(y, 256, 384), 384, dm)
        xres[rows, :] = y
        out_stage[rows, :] = y.astype(BF16)

        @pl.when(layer == n_layers - 1)
        def _():
            out_copy(i).start()

        return layer

    def hedgehog_layer(layer):
        kv_acc[...] = jnp.zeros(kv_acc.shape, F32)
        z_acc[...] = jnp.zeros(z_acc.shape, F32)
        lax.fori_loop(0, seq // tb, kv_block, 0)
        shape = kv_acc.shape[1:]
        same_head = _iota(shape, 0) // bdh == _iota(shape, 1) % 2
        for g in range(n_grp):
            kv_acc[g] = jnp.where(same_head, kv_acc[g], 0.0)
            z_acc[g] = jnp.broadcast_to(jnp.sum(z_acc[g], axis=1, keepdims=True), z_acc.shape[1:])
        lax.fori_loop(0, seq // tb, out_block, layer)

    def layer_pair(layer, carry):
        with jax.named_scope("rmt"):
            rmt_layer(layer)
        with jax.named_scope("hedgehog"):
            hedgehog_layer(layer)
        return carry

    lax.fori_loop(0, n_layers, layer_pair, 0)
    for i in range(seq // tb):
        out_copy(i).wait()


@functools.partial(jax.jit, static_argnames=("A_seg_len",))
def pallas_interleave_layers__memory_aug_recurrent_mem_tr__linear_kernel_hedgehog__prompt_kernel(
    A_x: jax.Array,
    A_mem0: jax.Array,
    A_Wq: jax.Array,
    A_Wk: jax.Array,
    A_Wv: jax.Array,
    A_Wo: jax.Array,
    A_seg_len: int,
    B_x: jax.Array,
    B_wqkv: jax.Array,
    B_w_phi: jax.Array,
    B_wo: jax.Array,
):
    del B_x
    batch, seq, dm = A_x.shape
    _, heads, dh = A_Wq.shape
    n_mem = A_mem0.shape[1]
    bh, bdh, _ = B_w_phi.shape
    seg = int(A_seg_len)
    assert batch == 1 and bdh == 20 and bh * bdh == dm and heads % 2 == 0
    assert (2 * dh) % 128 == 0 and n_mem % 8 == 0 and seg % 16 == 0 and 2 * (n_mem + seg) <= 128
    n_pairs, pw, hd = heads // 2, 2 * dh, heads * dh
    tb, unroll, n_early = 512, 2, 48

    def feature_major(w):
        return jnp.transpose(w, (1, 2, 0)).reshape(hd, dm)

    hbm = pl.BlockSpec(memory_space=pl.ANY)
    vmem = pl.BlockSpec(memory_space=pltpu.VMEM)
    out = pl.pallas_call(
        functools.partial(_kernel, seg=seg, dh=dh, n_layers=2, tb=tb, unroll=unroll),
        out_shape=jax.ShapeDtypeStruct((seq, dm), A_x.dtype),
        in_specs=[hbm, vmem, hbm, hbm, hbm, hbm, hbm, vmem, hbm],
        out_specs=hbm,
        scratch_shapes=[
            pltpu.VMEM((4, hd, dm), BF16),
            pltpu.VMEM((n_pairs, dm // 2, 3 * pw), U32),
            pltpu.VMEM((hd // 2, dm), U32),
            pltpu.VMEM((seq // seg, seg, dm), BF16),
            pltpu.VMEM((seq, dm), BF16),
            pltpu.VMEM((dm, 3 * dm), BF16),
            pltpu.VMEM((dm, dm), BF16),
            pltpu.VMEM((dm // 128, 8 * bdh, 128), BF16),
            pltpu.VMEM((2 * dm, dm), F32),
            pltpu.VMEM((dm, dm), F32),
            pltpu.VMEM((dm // 2, dm), U32),
            pltpu.VMEM((seq, dm), F32),
            pltpu.VMEM((seg, dm), F32),
            pltpu.VMEM((seq, dm), BF16),
            pltpu.VMEM((n_mem + seg, hd), F32),
            pltpu.VMEM((n_pairs, n_mem + 8, pw), F32),
            pltpu.VMEM((bh // 2, 2 * bdh, 4 * bdh), F32),
            pltpu.VMEM((bh // 2, 4 * bdh, 128), F32),
            pltpu.VMEM((n_early, EARLY_ROWS, dm), BF16),
            pltpu.VMEM((n_early * EARLY_ROWS, dm), BF16),
            pltpu.VMEM((n_pairs, n_early * EARLY_ROWS, 3 * pw), F32),
            pltpu.SemaphoreType.DMA((5, n_pairs)),
            pltpu.SemaphoreType.DMA((3,)),
            pltpu.SemaphoreType.DMA((seq // tb,)),
        ],
        compiler_params=pltpu.CompilerParams(vmem_limit_bytes=120 * 1024 * 1024),
        name="rmt_hedgehog",
    )(
        A_x.reshape(seq // seg, seg, dm),
        A_mem0.reshape(n_mem, dm),
        feature_major(A_Wq),
        feature_major(A_Wk),
        feature_major(A_Wv),
        A_Wo.reshape(hd, dm),
        B_wqkv,
        jnp.transpose(B_w_phi, (1, 2, 0)),
        B_wo,
    )
    return out.reshape(batch, seq, dm)
```

```python
import functools
import math

import jax
import jax.numpy as jnp
from jax import lax
import jax.experimental.pallas as pl
import jax.experimental.pallas.tpu as pltpu

F32 = jnp.float32
BF16 = jnp.bfloat16
U32 = jnp.uint32
I32 = jnp.int32

LN_EPS = 1e-5
DEN_EPS = 1e-6
LOG2E = math.log2(math.e)
EARLY_ROWS = 8
OUT_PLAN = "0000000001111111222"
OUT_PLAN_EARLY = "0000000001111111222"
VPU_PAIRS = range(0, 15)
VPU_PAIRS_EARLY = range(0, 15)


def _nn(a, b):
    return lax.dot_general(a, b, (((1,), (0,)), ((), ())), preferred_element_type=F32)


def _nt(a, b):
    return lax.dot_general(a, b, (((1,), (1,)), ((), ())), preferred_element_type=F32)


def _unpack(x):
    return pltpu.bitcast(x, BF16)


def _pack(x):
    return pltpu.bitcast(x, U32)


def _iota(shape, dim):
    return lax.broadcasted_iota(I32, shape, dim)


def _recip(x):
    r = pltpu.reciprocal(x, approx=True)
    return r * (2.0 - x * r)


def _layernorm(x):
    inv_n = 1.0 / x.shape[-1]
    m = jnp.sum(x, axis=-1, keepdims=True) * inv_n
    d = x - m
    v = jnp.sum(d * d, axis=-1, keepdims=True) * inv_n
    return d * lax.rsqrt(v + LN_EPS)


def _pair_blockdiag(x, dh):
    rows, width = x.shape
    top, bot = [], []
    zero = jnp.zeros((rows, 128), F32)
    for c in range(0, width, 128):
        t = x[:, c:c + 128]
        if c + 128 <= dh:
            top.append(t)
            bot.append(zero)
        elif c >= dh:
            top.append(zero)
            bot.append(t)
        else:
            first = _iota((rows, 128), 1) < dh - c
            top.append(jnp.where(first, t, 0.0))
            bot.append(jnp.where(first, 0.0, t))
    return jnp.concatenate(
        [jnp.concatenate(top, axis=1), jnp.concatenate(bot, axis=1)], axis=0
    ).astype(BF16)


def _pair_softmax(s, n_mem, scale):
    rows = s.shape[0]
    row = _iota(s.shape, 0)
    col = _iota(s.shape, 1)
    is_a = col < rows
    key = jnp.where(is_a, col, col - rows)
    s = jnp.where((row < n_mem) | (row >= key), s * scale, -1000000000.0)
    ma = jnp.max(jnp.where(is_a, s, -jnp.inf), axis=1, keepdims=True)
    mb = jnp.max(jnp.where(is_a, -jnp.inf, s), axis=1, keepdims=True)
    e = jnp.exp(s - jnp.where(is_a, ma, mb))
    la = jnp.sum(jnp.where(is_a, e, 0.0), axis=1, keepdims=True)
    lb = jnp.sum(jnp.where(is_a, 0.0, e), axis=1, keepdims=True)
    return e / jnp.where(is_a, la, lb)


def _over_features(x, op):
    r = functools.reduce(op, [x[i:i + 8] for i in range(0, x.shape[0], 8)])
    r = op(r, pltpu.roll(r, 4, 0))
    return op(r, pltpu.roll(r, 2, 0))


def _feature_map(p):
    def tile(r):
        return jnp.concatenate([r] * (p.shape[0] // 8), axis=0)

    ep = jnp.exp2(p - tile(_over_features(p, jnp.maximum)))
    en = jnp.exp2(tile(_over_features(p, jnp.minimum)) - p)
    return jnp.concatenate([e * tile(_recip(_over_features(e, jnp.add))) for e in (ep, en)], axis=0)


def _kernel(x_hbm, mem0_ref, wq_hbm, wk_hbm, wv_hbm, wo_hbm, bqkv_hbm, wphi_ref, bwo_hbm,
            out_hbm,
            stage, wqkv, wo, x_stage, out_stage, bqkv_stage, bwo_stage, fold, bw1, bwq, bwo,
            xres, xn_a, xn_b, o_scr, v_scr, kv_acc, z_acc, early_x, early_xn, early_qkv,
            w_sem, b_sem, out_sem,
            *, seg, dh, n_layers, tb, unroll):
    n_pairs = wqkv.shape[0]
    pw = 2 * dh
    half = pw // 2
    seq, dm = xres.shape
    n_mem = mem0_ref.shape[0]
    n_seg = seq // seg
    scale = dh ** -0.5
    bdh, _, bh = wphi_ref.shape
    n_grp = bh // 2
    gw = 2 * bdh
    n_early = early_xn.shape[0] // EARLY_ROWS

    x_chunk = n_seg // n_pairs

    def pair_rows(p):
        return pl.ds(pl.multiple_of(p * pw, pw), pw)

    def pair_copies(p):
        rows = pair_rows(p)
        segs = pl.ds(p * x_chunk, x_chunk)
        return [pltpu.make_async_copy(src.at[rows], stage.at[i, rows], w_sem.at[i, p])
                for i, src in enumerate((wq_hbm, wk_hbm, wv_hbm, wo_hbm))] + [
            pltpu.make_async_copy(x_hbm.at[segs], x_stage.at[segs], w_sem.at[4, p])]

    early_copy = pltpu.make_async_copy(
        x_hbm.at[pl.ds(0, n_early), pl.ds(seg - EARLY_ROWS, EARLY_ROWS)], early_x, b_sem.at[0])
    bqkv_copy = pltpu.make_async_copy(bqkv_hbm, bqkv_stage, b_sem.at[1])
    bwo_copy = pltpu.make_async_copy(bwo_hbm, bwo_stage, b_sem.at[2])
    early_copy.start()
    for c in pair_copies(0):
        c.start()

    wphi = wphi_ref[...].astype(F32)
    wf = jnp.concatenate([wphi[d] for d in range(bdh)], axis=1)
    src = _iota((dm, 128), 0)
    natural = (src % bh) * bdh + src // bh
    first_grp = [c // gw for c in range(0, dm, 128)]
    r = _iota((4 * gw, 128), 0)
    lane = _iota((4 * gw, 128), 1)
    pick = ((r % gw) // 2 == lane).astype(BF16)
    head_start = ((r // gw) * 2 + r % 2) * bdh
    for j, g0 in enumerate(first_grp):
        wj = _nn(wf, (natural == _iota((dm, 128), 1) + j * 128).astype(BF16))
        wj = jnp.concatenate([wj, jnp.zeros((128 - bdh, 128), F32)], axis=0).astype(BF16)
        d = lane + (j * 128 - g0 * gw) - head_start
        fold[j] = jnp.where((d >= 0) & (d < bdh), _nn(pick, wj), 0.0).astype(BF16)

    early_copy.wait()
    for c in pair_copies(1):
        c.start()
    early_xn[...] = _layernorm(
        early_x[...].astype(F32).reshape(n_early * EARLY_ROWS, dm)).astype(BF16)

    def load_pair(p, carry):
        for c in pair_copies(p):
            c.wait()

        def prefetch():
            @pl.when(p + 2 < n_pairs)
            def _():
                for c in pair_copies(p + 2):
                    c.start()

            pl.when(p == n_pairs // 2)(bqkv_copy.start)
            pl.when(p == n_pairs - 3)(bwo_copy.start)

        for i in range(3):
            w = stage[i, pair_rows(p), :]
            early_qkv[p, :, i * pw:(i + 1) * pw] = _nt(early_xn[...], w)
            wqkv[p, :, i * pw:(i + 1) * pw] = _pack(w.T)
            if i == 0:
                prefetch()
        wo[pl.ds(pl.multiple_of(p * half, half), half), :] = _pack(stage[3, pair_rows(p), :])
        wide = x_stage[pl.ds(p * x_chunk, x_chunk)].astype(F32).reshape(x_chunk * seg, dm)
        xres[pl.ds(pl.multiple_of(p * x_chunk * seg, x_chunk * seg), x_chunk * seg), :] = wide
        return carry

    with jax.named_scope("load"):
        lax.fori_loop(0, n_pairs, load_pair, 0)

    def fold_phi(base):
        groups = [None] * n_grp
        for j, g0 in enumerate(first_grp):
            t = _nt(fold[j], bqkv_stage[:, base + j * 128:base + (j + 1) * 128]) * LOG2E
            for i in range(4):
                part = t[i * gw:(i + 1) * gw]
                groups[g0 + i] = part if groups[g0 + i] is None else groups[g0 + i] + part
        return groups

    bqkv_copy.wait()
    bwo_copy.wait()
    wvt = bqkv_stage[:, 2 * dm:].astype(F32).T
    for g, (wpq, wpk) in enumerate(zip(fold_phi(0), fold_phi(dm))):
        bwq[g * gw:(g + 1) * gw, :] = wpq
        bw1[2 * g * gw:(2 * g + 1) * gw, :] = wpk
        bw1[(2 * g + 1) * gw:(2 * g + 2) * gw, :] = wvt[g * gw:(g + 1) * gw]
    bwo[...] = _pack(bwo_stage[...])

    def seg_rows(s):
        return pl.ds(pl.multiple_of(s * seg, seg), seg)

    def rmt_step(s, mem, early):
        if early:
            h = jnp.concatenate([mem, xn_a[:seg - EARLY_ROWS, :]], axis=0).astype(BF16)
            early_rows = pl.ds(pl.multiple_of(s * EARLY_ROWS, EARLY_ROWS), EARLY_ROWS)
        else:
            h = jnp.concatenate([mem, xn_a[...]], axis=0)
        xn_next = _layernorm(xres[seg_rows(jnp.minimum(s + 1, n_seg - 1)), :])
        prev = seg_rows(jnp.maximum(s - 1, 0))
        xn_b[prev, :] = _layernorm(xres[prev, :]).astype(BF16)
        pending = {1: xn_b[seg_rows(jnp.maximum(s, 1) - 1), :128][:16].astype(F32)[:8]}

        def weighted_values(p, prob, v):
            head = prob[:n_mem]
            if p in pending:
                head = jnp.where(s < 0, pending[p][:, :prob.shape[1]], head)
            if p not in (VPU_PAIRS_EARLY if early else VPU_PAIRS):
                return _nn(jnp.concatenate([head, prob[n_mem:]], axis=0), _pair_blockdiag(v, dh))
            seen = n_mem + 8
            o = _nn(jnp.concatenate([head, prob[seen:]], axis=0), _pair_blockdiag(v, dh))
            v_scr[p] = v[:seen]
            first = prob[n_mem:seen]
            first = jnp.concatenate([first, jnp.zeros((8, 128 - first.shape[1]), F32)], axis=1)
            lane = _iota(first.shape, 1)
            tiles = [None] * (pw // 128)
            for k in range(seen):
                wa, wb = (jnp.sum(jnp.where(lane == col, first, 0.0), axis=1, keepdims=True)
                          for col in (k, prob.shape[0] + k))
                for t in range(pw // 128):
                    c = t * 128
                    w = wa if c + 128 <= dh else wb if c >= dh else jnp.where(
                        _iota((8, 128), 1) < dh - c, wa, wb)
                    term = w * jnp.broadcast_to(v_scr[p, k:k + 1, c:c + 128], (8, 128))
                    tiles[t] = term if tiles[t] is None else tiles[t] + term
            pending[p + 1] = functools.reduce(jnp.add, tiles + ([pending[p + 1]] if p + 1 in pending else []))
            return jnp.concatenate([o[:n_mem], jnp.concatenate(tiles, axis=1), o[n_mem:]], axis=0)

        plan = OUT_PLAN_EARLY if early else OUT_PLAN
        ks = 256
        qkv, prob = {}, {}
        acc, done = None, 0

        def out_proj(acc, lo, hi):
            t = _nn(o_scr[:, lo * pw:hi * pw], _unpack(wo[lo * half:hi * half, :]))
            return t if acc is None else t + acc

        depth = len(plan) - n_pairs
        for p in range(n_pairs + depth):
            if p == 0:
                start = _nn(h[:, :ks], _unpack(wqkv[p, :ks // 2, :]))
                qkv[p] = _nn(h[:, ks:], _unpack(wqkv[p, ks // 2:, :])) + start
            elif p < n_pairs:
                qkv[p] = _nn(h, _unpack(wqkv[p]))
            if p < n_pairs:
                if early:
                    qkv[p] = jnp.concatenate([qkv[p], early_qkv[p, early_rows, :]], axis=0)
            n = int(plan[p])
            if n:
                acc = out_proj(acc, done, done + n)
                done += n
            if 0 <= p - 1 < n_pairs:
                t = qkv[p - 1]
                scores = _nt(t[:, :pw], _pair_blockdiag(t[:, pw:2 * pw], dh))
                prob[p - 1] = _pair_softmax(scores, n_mem, scale)
            r = p - depth
            if r >= 0:
                o_scr[:, r * pw:(r + 1) * pw] = weighted_values(r, prob[r], qkv[r][:, 2 * pw:])
        last = n_pairs - 2
        acc = out_proj(acc, done, last)
        acc = jnp.concatenate(
            [_nn(o_scr[:, last * pw:], _unpack(wo[last * half:, cols])) + acc[:, cols]
             for cols in (slice(0, ks), slice(ks, dm))], axis=1)
        xn_a[...] = xn_next
        rows = seg_rows(s)
        xres[rows, :] = xres[rows, :] + acc[n_mem:]
        return acc[:n_mem]

    def rmt_steps(lo, hi, mem, early):
        def body(i, mem):
            for u in range(unroll):
                mem = rmt_step(i * unroll + u, mem, early)
            return mem

        return lax.fori_loop(lo, hi, body, mem)

    def rmt_layer(layer):
        xn_a[...] = _layernorm(xres[0:seg, :])
        split = jnp.where(layer == 0, n_early // unroll, 0)
        mem = rmt_steps(0, split, mem0_ref[...].astype(F32), True)
        rmt_steps(split, n_seg // unroll, mem, False)
        last = slice(seq - seg, seq)
        xn_b[last, :] = _layernorm(xres[last, :]).astype(BF16)

    chunk = 4
    n_chunk = n_grp // chunk

    def blk_rows(i):
        return pl.ds(pl.multiple_of(i * tb, tb), tb)

    def kv_block(i, carry):
        xn = xn_b[blk_rows(i), :]
        proj = {}
        for c in range(n_chunk + 1):
            if c < n_chunk:
                proj[c] = _nt(bw1[2 * c * chunk * gw:2 * (c + 1) * chunk * gw, :], xn)
            if c >= 1:
                t = proj[c - 1]
                for j in range(chunk):
                    g = (c - 1) * chunk + j
                    phi = _feature_map(t[2 * j * gw:(2 * j + 1) * gw])
                    kv_acc[g] += _nt(t[(2 * j + 1) * gw:(2 * j + 2) * gw], phi.astype(BF16))
                    z_acc[g] += functools.reduce(jnp.add, [phi[:, i:i + 128] for i in range(0, tb, 128)])
        return carry

    def out_copy(i):
        return pltpu.make_async_copy(out_stage.at[blk_rows(i)], out_hbm.at[blk_rows(i)], out_sem.at[i])

    def out_block(i, layer):
        rows = blk_rows(i)
        xn = xn_b[rows, :]
        sublane = _iota((8, tb), 0)
        proj, outs = {}, []

        def out_proj(y, lo, hi):
            o = jnp.concatenate(outs, axis=0)[lo:hi].astype(BF16).T
            return _nn(o, _unpack(bwo[lo // 2:hi // 2, :])) + y

        y = xres[rows, :]
        for c in range(n_chunk + 1):
            if c < n_chunk:
                proj[c] = _nt(bwq[c * chunk * gw:(c + 1) * chunk * gw, :], xn)
            else:
                y = out_proj(y, 0, 256)
            if c >= 1:
                for j in range(chunk):
                    g = (c - 1) * chunk + j
                    phi = _feature_map(proj[c - 1][j * gw:(j + 1) * gw])
                    z = jnp.concatenate([z_acc[g]] * (tb // 128), axis=1)
                    inv = _recip(_over_features(phi * z, jnp.add) + DEN_EPS)
                    swapped = pltpu.roll(inv, 1, 0)
                    inv_a = jnp.where(sublane % 2 == 0, inv, swapped)
                    inv_b = jnp.where(sublane % 2 == 0, swapped, inv)
                    inv_ab = jnp.where(sublane < bdh % 8, inv_a, inv_b)
                    outs.append(_nn(kv_acc[g], phi.astype(BF16))
                                * jnp.concatenate([inv_a, inv_a, inv_ab, inv_b, inv_b], axis=0))
        y = out_proj(out_proj(y, 256, 384), 384, dm)
        xres[rows, :] = y
        out_stage[rows, :] = y.astype(BF16)

        @pl.when(layer == n_layers - 1)
        def _():
            out_copy(i).start()

        return layer

    def hedgehog_layer(layer):
        kv_acc[...] = jnp.zeros(kv_acc.shape, F32)
        z_acc[...] = jnp.zeros(z_acc.shape, F32)
        lax.fori_loop(0, seq // tb, kv_block, 0)
        shape = kv_acc.shape[1:]
        same_head = _iota(shape, 0) // bdh == _iota(shape, 1) % 2
        for g in range(n_grp):
            kv_acc[g] = jnp.where(same_head, kv_acc[g], 0.0)
            z_acc[g] = jnp.broadcast_to(jnp.sum(z_acc[g], axis=1, keepdims=True), z_acc.shape[1:])
        lax.fori_loop(0, seq // tb, out_block, layer)

    def layer_pair(layer, carry):
        with jax.named_scope("rmt"):
            rmt_layer(layer)
        with jax.named_scope("hedgehog"):
            hedgehog_layer(layer)
        return carry

    lax.fori_loop(0, n_layers, layer_pair, 0)
    for i in range(seq // tb):
        out_copy(i).wait()


@functools.partial(jax.jit, static_argnames=("A_seg_len",))
def pallas_interleave_layers__memory_aug_recurrent_mem_tr__linear_kernel_hedgehog__prompt_kernel(
    A_x: jax.Array,
    A_mem0: jax.Array,
    A_Wq: jax.Array,
    A_Wk: jax.Array,
    A_Wv: jax.Array,
    A_Wo: jax.Array,
    A_seg_len: int,
    B_x: jax.Array,
    B_wqkv: jax.Array,
    B_w_phi: jax.Array,
    B_wo: jax.Array,
):
    del B_x
    batch, seq, dm = A_x.shape
    _, heads, dh = A_Wq.shape
    n_mem = A_mem0.shape[1]
    bh, bdh, _ = B_w_phi.shape
    seg = int(A_seg_len)
    assert batch == 1 and bdh == 20 and bh * bdh == dm and heads % 2 == 0
    assert (2 * dh) % 128 == 0 and n_mem % 8 == 0 and seg % 16 == 0 and 2 * (n_mem + seg) <= 128
    n_pairs, pw, hd = heads // 2, 2 * dh, heads * dh
    tb, unroll, n_early = 512, 2, 48

    def feature_major(w):
        return jnp.transpose(w, (1, 2, 0)).reshape(hd, dm)

    hbm = pl.BlockSpec(memory_space=pl.ANY)
    vmem = pl.BlockSpec(memory_space=pltpu.VMEM)
    out = pl.pallas_call(
        functools.partial(_kernel, seg=seg, dh=dh, n_layers=2, tb=tb, unroll=unroll),
        out_shape=jax.ShapeDtypeStruct((seq, dm), A_x.dtype),
        in_specs=[hbm, vmem, hbm, hbm, hbm, hbm, hbm, vmem, hbm],
        out_specs=hbm,
        scratch_shapes=[
            pltpu.VMEM((4, hd, dm), BF16),
            pltpu.VMEM((n_pairs, dm // 2, 3 * pw), U32),
            pltpu.VMEM((hd // 2, dm), U32),
            pltpu.VMEM((seq // seg, seg, dm), BF16),
            pltpu.VMEM((seq, dm), BF16),
            pltpu.VMEM((dm, 3 * dm), BF16),
            pltpu.VMEM((dm, dm), BF16),
            pltpu.VMEM((dm // 128, 8 * bdh, 128), BF16),
            pltpu.VMEM((2 * dm, dm), F32),
            pltpu.VMEM((dm, dm), F32),
            pltpu.VMEM((dm // 2, dm), U32),
            pltpu.VMEM((seq, dm), F32),
            pltpu.VMEM((seg, dm), F32),
            pltpu.VMEM((seq, dm), BF16),
            pltpu.VMEM((n_mem + seg, hd), F32),
            pltpu.VMEM((n_pairs, n_mem + 8, pw), F32),
            pltpu.VMEM((bh // 2, 2 * bdh, 4 * bdh), F32),
            pltpu.VMEM((bh // 2, 4 * bdh, 128), F32),
            pltpu.VMEM((n_early, EARLY_ROWS, dm), BF16),
            pltpu.VMEM((n_early * EARLY_ROWS, dm), BF16),
            pltpu.VMEM((n_pairs, n_early * EARLY_ROWS, 3 * pw), F32),
            pltpu.SemaphoreType.DMA((5, n_pairs)),
            pltpu.SemaphoreType.DMA((3,)),
            pltpu.SemaphoreType.DMA((seq // tb,)),
        ],
        compiler_params=pltpu.CompilerParams(vmem_limit_bytes=120 * 1024 * 1024),
        name="rmt_hedgehog",
    )(
        A_x.reshape(seq // seg, seg, dm),
        A_mem0.reshape(n_mem, dm),
        feature_major(A_Wq),
        feature_major(A_Wk),
        feature_major(A_Wv),
        A_Wo.reshape(hd, dm),
        B_wqkv,
        jnp.transpose(B_w_phi, (1, 2, 0)),
        B_wo,
    )
    return out.reshape(batch, seq, dm)
```

```python
import functools
import math

import jax
import jax.numpy as jnp
from jax import lax
import jax.experimental.pallas as pl
import jax.experimental.pallas.tpu as pltpu

F32 = jnp.float32
BF16 = jnp.bfloat16
U32 = jnp.uint32
I32 = jnp.int32

LN_EPS = 1e-5
DEN_EPS = 1e-6
LOG2E = math.log2(math.e)
EARLY_ROWS = 8
OUT_PLAN = "0000000001111111222"
OUT_PLAN_EARLY = "0000000001111111222"
VPU_PAIRS = range(0, 15)
VPU_PAIRS_EARLY = range(0, 15)


def _nn(a, b):
    return lax.dot_general(a, b, (((1,), (0,)), ((), ())), preferred_element_type=F32)


def _nt(a, b):
    return lax.dot_general(a, b, (((1,), (1,)), ((), ())), preferred_element_type=F32)


def _unpack(x):
    return pltpu.bitcast(x, BF16)


def _pack(x):
    return pltpu.bitcast(x, U32)


def _iota(shape, dim):
    return lax.broadcasted_iota(I32, shape, dim)


def _recip(x):
    r = pltpu.reciprocal(x, approx=True)
    return r * (2.0 - x * r)


def _layernorm(x):
    inv_n = 1.0 / x.shape[-1]
    m = jnp.sum(x, axis=-1, keepdims=True) * inv_n
    d = x - m
    v = jnp.sum(d * d, axis=-1, keepdims=True) * inv_n
    return d * lax.rsqrt(v + LN_EPS)


def _pair_blockdiag(x, dh):
    rows, width = x.shape
    top, bot = [], []
    zero = jnp.zeros((rows, 128), F32)
    for c in range(0, width, 128):
        t = x[:, c:c + 128]
        if c + 128 <= dh:
            top.append(t)
            bot.append(zero)
        elif c >= dh:
            top.append(zero)
            bot.append(t)
        else:
            first = _iota((rows, 128), 1) < dh - c
            top.append(jnp.where(first, t, 0.0))
            bot.append(jnp.where(first, 0.0, t))
    return jnp.concatenate(
        [jnp.concatenate(top, axis=1), jnp.concatenate(bot, axis=1)], axis=0
    ).astype(BF16)


def _pair_softmax(s, n_mem, scale):
    rows = s.shape[0]
    row = _iota(s.shape, 0)
    col = _iota(s.shape, 1)
    is_a = col < rows
    key = jnp.where(is_a, col, col - rows)
    s = jnp.where((row < n_mem) | (row >= key), s * scale, -1000000000.0)
    ma = jnp.max(jnp.where(is_a, s, -jnp.inf), axis=1, keepdims=True)
    mb = jnp.max(jnp.where(is_a, -jnp.inf, s), axis=1, keepdims=True)
    e = jnp.exp(s - jnp.where(is_a, ma, mb))
    la = jnp.sum(jnp.where(is_a, e, 0.0), axis=1, keepdims=True)
    lb = jnp.sum(jnp.where(is_a, 0.0, e), axis=1, keepdims=True)
    return e / jnp.where(is_a, la, lb)


def _over_features(x, op):
    r = functools.reduce(op, [x[i:i + 8] for i in range(0, x.shape[0], 8)])
    r = op(r, pltpu.roll(r, 4, 0))
    return op(r, pltpu.roll(r, 2, 0))


def _feature_map(p):
    def tile(r):
        return jnp.concatenate([r] * (p.shape[0] // 8), axis=0)

    ep = jnp.exp2(p - tile(_over_features(p, jnp.maximum)))
    en = jnp.exp2(tile(_over_features(p, jnp.minimum)) - p)
    return jnp.concatenate([e * tile(_recip(_over_features(e, jnp.add))) for e in (ep, en)], axis=0)


def _kernel(x_hbm, mem0_ref, wq_hbm, wk_hbm, wv_hbm, wo_hbm, bqkv_hbm, wphi_ref, bwo_hbm,
            out_hbm,
            stage, wqkv, wo, x_stage, out_stage, bqkv_stage, bwo_stage, fold, bw1, bwq, bwo,
            xres, xn_a, xn_b, o_scr, v_scr, kv_acc, z_acc, early_x, early_xn, early_qkv,
            w_sem, b_sem, out_sem,
            *, seg, dh, n_layers, tb, unroll):
    n_pairs = wqkv.shape[0]
    pw = 2 * dh
    half = pw // 2
    seq, dm = xres.shape
    n_mem = mem0_ref.shape[0]
    n_seg = seq // seg
    scale = dh ** -0.5
    bdh, _, bh = wphi_ref.shape
    n_grp = bh // 2
    gw = 2 * bdh
    n_early = early_xn.shape[0] // EARLY_ROWS

    x_chunk = n_seg // n_pairs

    def pair_rows(p):
        return pl.ds(pl.multiple_of(p * pw, pw), pw)

    def pair_copies(p):
        rows = pair_rows(p)
        segs = pl.ds(p * x_chunk, x_chunk)
        return [pltpu.make_async_copy(src.at[rows], stage.at[i, rows], w_sem.at[i, p])
                for i, src in enumerate((wq_hbm, wk_hbm, wv_hbm, wo_hbm))] + [
            pltpu.make_async_copy(x_hbm.at[segs], x_stage.at[segs], w_sem.at[4, p])]

    early_copy = pltpu.make_async_copy(
        x_hbm.at[pl.ds(0, n_early), pl.ds(seg - EARLY_ROWS, EARLY_ROWS)], early_x, b_sem.at[0])
    bqkv_copy = pltpu.make_async_copy(bqkv_hbm, bqkv_stage, b_sem.at[1])
    bwo_copy = pltpu.make_async_copy(bwo_hbm, bwo_stage, b_sem.at[2])
    early_copy.start()

    wphi = wphi_ref[...].astype(F32)
    wf = jnp.concatenate([wphi[d] for d in range(bdh)], axis=1)
    src = _iota((dm, 128), 0)
    natural = (src % bh) * bdh + src // bh
    first_grp = [c // gw for c in range(0, dm, 128)]
    r = _iota((4 * gw, 128), 0)
    lane = _iota((4 * gw, 128), 1)
    pick = ((r % gw) // 2 == lane).astype(BF16)
    head_start = ((r // gw) * 2 + r % 2) * bdh
    for j, g0 in enumerate(first_grp):
        wj = _nn(wf, (natural == _iota((dm, 128), 1) + j * 128).astype(BF16))
        wj = jnp.concatenate([wj, jnp.zeros((128 - bdh, 128), F32)], axis=0).astype(BF16)
        d = lane + (j * 128 - g0 * gw) - head_start
        fold[j] = jnp.where((d >= 0) & (d < bdh), _nn(pick, wj), 0.0).astype(BF16)

    for c in pair_copies(0):
        c.start()
    early_copy.wait()
    early_xn[...] = _layernorm(
        early_x[...].astype(F32).reshape(n_early * EARLY_ROWS, dm)).astype(BF16)

    for c in pair_copies(1):
        c.start()

    def load_pair(p, carry):
        for c in pair_copies(p):
            c.wait()

        def prefetch():
            for c in pair_copies(p + 2):
                c.start()

        for i in range(3):
            w = stage[i, pair_rows(p), :]
            early_qkv[p, :, i * pw:(i + 1) * pw] = _nt(early_xn[...], w)
            wqkv[p, :, i * pw:(i + 1) * pw] = _pack(w.T)
            if i == 0:
                pl.when(p + 2 < n_pairs)(prefetch)
        wo[pl.ds(pl.multiple_of(p * half, half), half), :] = _pack(stage[3, pair_rows(p), :])
        wide = x_stage[pl.ds(p * x_chunk, x_chunk)].astype(F32).reshape(x_chunk * seg, dm)
        xres[pl.ds(pl.multiple_of(p * x_chunk * seg, x_chunk * seg), x_chunk * seg), :] = wide
        return carry

    with jax.named_scope("load"):
        lax.fori_loop(0, n_pairs, load_pair, 0)
    bqkv_copy.start()
    bwo_copy.start()

    def fold_phi(base):
        groups = [None] * n_grp
        for j, g0 in enumerate(first_grp):
            t = _nt(fold[j], bqkv_stage[:, base + j * 128:base + (j + 1) * 128]) * LOG2E
            for i in range(4):
                part = t[i * gw:(i + 1) * gw]
                groups[g0 + i] = part if groups[g0 + i] is None else groups[g0 + i] + part
        return groups

    def hedgehog_weights():
        bqkv_copy.wait()
        bwo_copy.wait()
        wvt = bqkv_stage[:, 2 * dm:].astype(F32).T
        for g, (wpq, wpk) in enumerate(zip(fold_phi(0), fold_phi(dm))):
            bwq[g * gw:(g + 1) * gw, :] = wpq
            bw1[2 * g * gw:(2 * g + 1) * gw, :] = wpk
            bw1[(2 * g + 1) * gw:(2 * g + 2) * gw, :] = wvt[g * gw:(g + 1) * gw]
        bwo[...] = _pack(bwo_stage[...])

    def seg_rows(s):
        return pl.ds(pl.multiple_of(s * seg, seg), seg)

    def rmt_step(s, mem, early):
        if early:
            h = jnp.concatenate([mem, xn_a[:seg - EARLY_ROWS, :]], axis=0).astype(BF16)
            early_rows = pl.ds(pl.multiple_of(s * EARLY_ROWS, EARLY_ROWS), EARLY_ROWS)
        else:
            h = jnp.concatenate([mem, xn_a[...]], axis=0)
        xn_next = _layernorm(xres[seg_rows(jnp.minimum(s + 1, n_seg - 1)), :])
        prev = seg_rows(jnp.maximum(s - 1, 0))
        xn_b[prev, :] = _layernorm(xres[prev, :]).astype(BF16)
        pending = {1: xn_b[seg_rows(jnp.maximum(s, 1) - 1), :128][:16].astype(F32)[:8]}

        def weighted_values(p, prob, v):
            head = prob[:n_mem]
            if p in pending:
                head = jnp.where(s < 0, pending[p][:, :prob.shape[1]], head)
            if p not in (VPU_PAIRS_EARLY if early else VPU_PAIRS):
                return _nn(jnp.concatenate([head, prob[n_mem:]], axis=0), _pair_blockdiag(v, dh))
            seen = n_mem + 8
            o = _nn(jnp.concatenate([head, prob[seen:]], axis=0), _pair_blockdiag(v, dh))
            v_scr[p] = v[:seen]
            first = prob[n_mem:seen]
            first = jnp.concatenate([first, jnp.zeros((8, 128 - first.shape[1]), F32)], axis=1)
            lane = _iota(first.shape, 1)
            tiles = [None] * (pw // 128)
            for k in range(seen):
                wa, wb = (jnp.sum(jnp.where(lane == col, first, 0.0), axis=1, keepdims=True)
                          for col in (k, prob.shape[0] + k))
                for t in range(pw // 128):
                    c = t * 128
                    w = wa if c + 128 <= dh else wb if c >= dh else jnp.where(
                        _iota((8, 128), 1) < dh - c, wa, wb)
                    term = w * jnp.broadcast_to(v_scr[p, k:k + 1, c:c + 128], (8, 128))
                    tiles[t] = term if tiles[t] is None else tiles[t] + term
            pending[p + 1] = functools.reduce(jnp.add, tiles + ([pending[p + 1]] if p + 1 in pending else []))
            return jnp.concatenate([o[:n_mem], jnp.concatenate(tiles, axis=1), o[n_mem:]], axis=0)

        plan = OUT_PLAN_EARLY if early else OUT_PLAN
        ks = 256
        qkv, prob = {}, {}
        acc, done = None, 0

        def out_proj(acc, lo, hi):
            t = _nn(o_scr[:, lo * pw:hi * pw], _unpack(wo[lo * half:hi * half, :]))
            return t if acc is None else t + acc

        depth = len(plan) - n_pairs
        for p in range(n_pairs + depth):
            if p == 0:
                start = _nn(h[:, :ks], _unpack(wqkv[p, :ks // 2, :]))
                qkv[p] = _nn(h[:, ks:], _unpack(wqkv[p, ks // 2:, :])) + start
            elif p < n_pairs:
                qkv[p] = _nn(h, _unpack(wqkv[p]))
            if p < n_pairs:
                if early:
                    qkv[p] = jnp.concatenate([qkv[p], early_qkv[p, early_rows, :]], axis=0)
            n = int(plan[p])
            if n:
                acc = out_proj(acc, done, done + n)
                done += n
            if 0 <= p - 1 < n_pairs:
                t = qkv[p - 1]
                scores = _nt(t[:, :pw], _pair_blockdiag(t[:, pw:2 * pw], dh))
                prob[p - 1] = _pair_softmax(scores, n_mem, scale)
            r = p - depth
            if r >= 0:
                o_scr[:, r * pw:(r + 1) * pw] = weighted_values(r, prob[r], qkv[r][:, 2 * pw:])
        last = n_pairs - 2
        acc = out_proj(acc, done, last)
        acc = jnp.concatenate(
            [_nn(o_scr[:, last * pw:], _unpack(wo[last * half:, cols])) + acc[:, cols]
             for cols in (slice(0, ks), slice(ks, dm))], axis=1)
        xn_a[...] = xn_next
        rows = seg_rows(s)
        xres[rows, :] = xres[rows, :] + acc[n_mem:]
        return acc[:n_mem]

    def rmt_steps(lo, hi, mem, early):
        def body(i, mem):
            for u in range(unroll):
                mem = rmt_step(i * unroll + u, mem, early)
            return mem

        return lax.fori_loop(lo, hi, body, mem)

    def rmt_layer(layer):
        xn_a[...] = _layernorm(xres[0:seg, :])
        split = jnp.where(layer == 0, n_early // unroll, 0)
        mem = rmt_steps(0, split, mem0_ref[...].astype(F32), True)
        rmt_steps(split, n_seg // unroll, mem, False)
        last = slice(seq - seg, seq)
        xn_b[last, :] = _layernorm(xres[last, :]).astype(BF16)

    chunk = 4
    n_chunk = n_grp // chunk

    def blk_rows(i):
        return pl.ds(pl.multiple_of(i * tb, tb), tb)

    def kv_block(i, carry):
        xn = xn_b[blk_rows(i), :]
        proj = {}
        for c in range(n_chunk + 1):
            if c < n_chunk:
                proj[c] = _nt(bw1[2 * c * chunk * gw:2 * (c + 1) * chunk * gw, :], xn)
            if c >= 1:
                t = proj[c - 1]
                for j in range(chunk):
                    g = (c - 1) * chunk + j
                    phi = _feature_map(t[2 * j * gw:(2 * j + 1) * gw])
                    kv_acc[g] += _nt(t[(2 * j + 1) * gw:(2 * j + 2) * gw], phi.astype(BF16))
                    z_acc[g] += functools.reduce(jnp.add, [phi[:, i:i + 128] for i in range(0, tb, 128)])
        return carry

    def out_copy(i):
        return pltpu.make_async_copy(out_stage.at[blk_rows(i)], out_hbm.at[blk_rows(i)], out_sem.at[i])

    def out_block(i, layer):
        rows = blk_rows(i)
        xn = xn_b[rows, :]
        sublane = _iota((8, tb), 0)
        proj, outs = {}, []

        def out_proj(y, lo, hi):
            o = jnp.concatenate(outs, axis=0)[lo:hi].astype(BF16).T
            return _nn(o, _unpack(bwo[lo // 2:hi // 2, :])) + y

        y = xres[rows, :]
        for c in range(n_chunk + 1):
            if c < n_chunk:
                proj[c] = _nt(bwq[c * chunk * gw:(c + 1) * chunk * gw, :], xn)
            else:
                y = out_proj(y, 0, 256)
            if c >= 1:
                for j in range(chunk):
                    g = (c - 1) * chunk + j
                    phi = _feature_map(proj[c - 1][j * gw:(j + 1) * gw])
                    z = jnp.concatenate([z_acc[g]] * (tb // 128), axis=1)
                    inv = _recip(_over_features(phi * z, jnp.add) + DEN_EPS)
                    swapped = pltpu.roll(inv, 1, 0)
                    inv_a = jnp.where(sublane % 2 == 0, inv, swapped)
                    inv_b = jnp.where(sublane % 2 == 0, swapped, inv)
                    inv_ab = jnp.where(sublane < bdh % 8, inv_a, inv_b)
                    outs.append(_nn(kv_acc[g], phi.astype(BF16))
                                * jnp.concatenate([inv_a, inv_a, inv_ab, inv_b, inv_b], axis=0))
        y = out_proj(out_proj(y, 256, 384), 384, dm)
        xres[rows, :] = y
        out_stage[rows, :] = y.astype(BF16)

        @pl.when(layer == n_layers - 1)
        def _():
            out_copy(i).start()

        return layer

    def hedgehog_layer(layer):
        kv_acc[...] = jnp.zeros(kv_acc.shape, F32)
        z_acc[...] = jnp.zeros(z_acc.shape, F32)
        lax.fori_loop(0, seq // tb, kv_block, 0)
        shape = kv_acc.shape[1:]
        same_head = _iota(shape, 0) // bdh == _iota(shape, 1) % 2
        for g in range(n_grp):
            kv_acc[g] = jnp.where(same_head, kv_acc[g], 0.0)
            z_acc[g] = jnp.broadcast_to(jnp.sum(z_acc[g], axis=1, keepdims=True), z_acc.shape[1:])
        lax.fori_loop(0, seq // tb, out_block, layer)

    def layer_pair(layer, carry):
        with jax.named_scope("rmt"):
            rmt_layer(layer)
        pl.when(layer == 0)(hedgehog_weights)
        with jax.named_scope("hedgehog"):
            hedgehog_layer(layer)
        return carry

    lax.fori_loop(0, n_layers, layer_pair, 0)
    for i in range(seq // tb):
        out_copy(i).wait()


@functools.partial(jax.jit, static_argnames=("A_seg_len",))
def pallas_interleave_layers__memory_aug_recurrent_mem_tr__linear_kernel_hedgehog__prompt_kernel(
    A_x: jax.Array,
    A_mem0: jax.Array,
    A_Wq: jax.Array,
    A_Wk: jax.Array,
    A_Wv: jax.Array,
    A_Wo: jax.Array,
    A_seg_len: int,
    B_x: jax.Array,
    B_wqkv: jax.Array,
    B_w_phi: jax.Array,
    B_wo: jax.Array,
):
    del B_x
    batch, seq, dm = A_x.shape
    _, heads, dh = A_Wq.shape
    n_mem = A_mem0.shape[1]
    bh, bdh, _ = B_w_phi.shape
    seg = int(A_seg_len)
    assert batch == 1 and bdh == 20 and bh * bdh == dm and heads % 2 == 0
    assert (2 * dh) % 128 == 0 and n_mem % 8 == 0 and seg % 16 == 0 and 2 * (n_mem + seg) <= 128
    n_pairs, pw, hd = heads // 2, 2 * dh, heads * dh
    tb, unroll, n_early = 512, 2, 48

    def feature_major(w):
        return jnp.transpose(w, (1, 2, 0)).reshape(hd, dm)

    hbm = pl.BlockSpec(memory_space=pl.ANY)
    vmem = pl.BlockSpec(memory_space=pltpu.VMEM)
    out = pl.pallas_call(
        functools.partial(_kernel, seg=seg, dh=dh, n_layers=2, tb=tb, unroll=unroll),
        out_shape=jax.ShapeDtypeStruct((seq, dm), A_x.dtype),
        in_specs=[hbm, vmem, hbm, hbm, hbm, hbm, hbm, vmem, hbm],
        out_specs=hbm,
        scratch_shapes=[
            pltpu.VMEM((4, hd, dm), BF16),
            pltpu.VMEM((n_pairs, dm // 2, 3 * pw), U32),
            pltpu.VMEM((hd // 2, dm), U32),
            pltpu.VMEM((seq // seg, seg, dm), BF16),
            pltpu.VMEM((seq, dm), BF16),
            pltpu.VMEM((dm, 3 * dm), BF16),
            pltpu.VMEM((dm, dm), BF16),
            pltpu.VMEM((dm // 128, 8 * bdh, 128), BF16),
            pltpu.VMEM((2 * dm, dm), F32),
            pltpu.VMEM((dm, dm), F32),
            pltpu.VMEM((dm // 2, dm), U32),
            pltpu.VMEM((seq, dm), F32),
            pltpu.VMEM((seg, dm), F32),
            pltpu.VMEM((seq, dm), BF16),
            pltpu.VMEM((n_mem + seg, hd), F32),
            pltpu.VMEM((n_pairs, n_mem + 8, pw), F32),
            pltpu.VMEM((bh // 2, 2 * bdh, 4 * bdh), F32),
            pltpu.VMEM((bh // 2, 4 * bdh, 128), F32),
            pltpu.VMEM((n_early, EARLY_ROWS, dm), BF16),
            pltpu.VMEM((n_early * EARLY_ROWS, dm), BF16),
            pltpu.VMEM((n_pairs, n_early * EARLY_ROWS, 3 * pw), F32),
            pltpu.SemaphoreType.DMA((5, n_pairs)),
            pltpu.SemaphoreType.DMA((3,)),
            pltpu.SemaphoreType.DMA((seq // tb,)),
        ],
        compiler_params=pltpu.CompilerParams(vmem_limit_bytes=120 * 1024 * 1024),
        name="rmt_hedgehog",
    )(
        A_x.reshape(seq // seg, seg, dm),
        A_mem0.reshape(n_mem, dm),
        feature_major(A_Wq),
        feature_major(A_Wk),
        feature_major(A_Wv),
        A_Wo.reshape(hd, dm),
        B_wqkv,
        jnp.transpose(B_w_phi, (1, 2, 0)),
        B_wo,
    )
    return out.reshape(batch, seq, dm)
```

```python
import functools
import math

import jax
import jax.numpy as jnp
from jax import lax
import jax.experimental.pallas as pl
import jax.experimental.pallas.tpu as pltpu

F32 = jnp.float32
BF16 = jnp.bfloat16
U32 = jnp.uint32
I32 = jnp.int32

LN_EPS = 1e-5
DEN_EPS = 1e-6
LOG2E = math.log2(math.e)
EARLY_ROWS = 8
STEP_REGULAR = ("0000000001111111222", range(0, 15), 1, "qosv", 256)
STEP_EARLY = ("0000000001111111222", range(0, 15), 1, "qosv", 256)


def _nn(a, b):
    return lax.dot_general(a, b, (((1,), (0,)), ((), ())), preferred_element_type=F32)


def _nt(a, b):
    return lax.dot_general(a, b, (((1,), (1,)), ((), ())), preferred_element_type=F32)


def _unpack(x):
    return pltpu.bitcast(x, BF16)


def _pack(x):
    return pltpu.bitcast(x, U32)


def _iota(shape, dim):
    return lax.broadcasted_iota(I32, shape, dim)


def _recip(x):
    r = pltpu.reciprocal(x, approx=True)
    return r * (2.0 - x * r)


def _layernorm(x):
    inv_n = 1.0 / x.shape[-1]
    m = jnp.sum(x, axis=-1, keepdims=True) * inv_n
    d = x - m
    v = jnp.sum(d * d, axis=-1, keepdims=True) * inv_n
    return d * lax.rsqrt(v + LN_EPS)


def _pair_blockdiag(x, dh):
    rows, width = x.shape
    top, bot = [], []
    zero = jnp.zeros((rows, 128), F32)
    for c in range(0, width, 128):
        t = x[:, c:c + 128]
        if c + 128 <= dh:
            top.append(t)
            bot.append(zero)
        elif c >= dh:
            top.append(zero)
            bot.append(t)
        else:
            first = _iota((rows, 128), 1) < dh - c
            top.append(jnp.where(first, t, 0.0))
            bot.append(jnp.where(first, 0.0, t))
    return jnp.concatenate(
        [jnp.concatenate(top, axis=1), jnp.concatenate(bot, axis=1)], axis=0
    ).astype(BF16)


def _pair_softmax(s, n_mem, scale):
    rows = s.shape[0]
    row = _iota(s.shape, 0)
    col = _iota(s.shape, 1)
    is_a = col < rows
    key = jnp.where(is_a, col, col - rows)
    s = jnp.where((row < n_mem) | (row >= key), s * scale, -1000000000.0)
    ma = jnp.max(jnp.where(is_a, s, -jnp.inf), axis=1, keepdims=True)
    mb = jnp.max(jnp.where(is_a, -jnp.inf, s), axis=1, keepdims=True)
    e = jnp.exp(s - jnp.where(is_a, ma, mb))
    la = jnp.sum(jnp.where(is_a, e, 0.0), axis=1, keepdims=True)
    lb = jnp.sum(jnp.where(is_a, 0.0, e), axis=1, keepdims=True)
    return e / jnp.where(is_a, la, lb)


def _over_features(x, op):
    r = functools.reduce(op, [x[i:i + 8] for i in range(0, x.shape[0], 8)])
    r = op(r, pltpu.roll(r, 4, 0))
    return op(r, pltpu.roll(r, 2, 0))


def _feature_map(p):
    def tile(r):
        return jnp.concatenate([r] * (p.shape[0] // 8), axis=0)

    ep = jnp.exp2(p - tile(_over_features(p, jnp.maximum)))
    en = jnp.exp2(tile(_over_features(p, jnp.minimum)) - p)
    return jnp.concatenate([e * tile(_recip(_over_features(e, jnp.add))) for e in (ep, en)], axis=0)


def _kernel(x_hbm, mem0_ref, wq_hbm, wk_hbm, wv_hbm, wo_hbm, bqkv_hbm, wphi_ref, bwo_hbm,
            out_hbm,
            stage, wqkv, wo, x_stage, out_stage, bqkv_stage, bwo_stage, fold, bw1, bwq, bwo,
            xres, xn_a, xn_b, o_scr, v_scr, kv_acc, z_acc, early_x, early_xn, early_qkv,
            w_sem, b_sem, out_sem,
            *, seg, dh, n_layers, tb, unroll):
    n_pairs = wqkv.shape[0]
    pw = 2 * dh
    half = pw // 2
    seq, dm = xres.shape
    n_mem = mem0_ref.shape[0]
    n_seg = seq // seg
    scale = dh ** -0.5
    bdh, _, bh = wphi_ref.shape
    n_grp = bh // 2
    gw = 2 * bdh
    n_early = early_xn.shape[0] // EARLY_ROWS

    x_chunk = n_seg // n_pairs

    def pair_rows(p):
        return pl.ds(pl.multiple_of(p * pw, pw), pw)

    def pair_copies(p):
        rows = pair_rows(p)
        segs = pl.ds(p * x_chunk, x_chunk)
        return [pltpu.make_async_copy(src.at[rows], stage.at[i, rows], w_sem.at[i, p])
                for i, src in enumerate((wq_hbm, wk_hbm, wv_hbm, wo_hbm))] + [
            pltpu.make_async_copy(x_hbm.at[segs], x_stage.at[segs], w_sem.at[4, p])]

    early_copy = pltpu.make_async_copy(
        x_hbm.at[pl.ds(0, n_early), pl.ds(seg - EARLY_ROWS, EARLY_ROWS)], early_x, b_sem.at[0])
    bqkv_copy = pltpu.make_async_copy(bqkv_hbm, bqkv_stage, b_sem.at[1])
    bwo_copy = pltpu.make_async_copy(bwo_hbm, bwo_stage, b_sem.at[2])
    early_copy.start()

    wphi = wphi_ref[...].astype(F32)
    wf = jnp.concatenate([wphi[d] for d in range(bdh)], axis=1)
    src = _iota((dm, 128), 0)
    natural = (src % bh) * bdh + src // bh
    first_grp = [c // gw for c in range(0, dm, 128)]
    r = _iota((4 * gw, 128), 0)
    lane = _iota((4 * gw, 128), 1)
    pick = ((r % gw) // 2 == lane).astype(BF16)
    head_start = ((r // gw) * 2 + r % 2) * bdh
    for j, g0 in enumerate(first_grp):
        wj = _nn(wf, (natural == _iota((dm, 128), 1) + j * 128).astype(BF16))
        wj = jnp.concatenate([wj, jnp.zeros((128 - bdh, 128), F32)], axis=0).astype(BF16)
        d = lane + (j * 128 - g0 * gw) - head_start
        fold[j] = jnp.where((d >= 0) & (d < bdh), _nn(pick, wj), 0.0).astype(BF16)

    for c in pair_copies(0):
        c.start()
    early_copy.wait()
    early_xn[...] = _layernorm(
        early_x[...].astype(F32).reshape(n_early * EARLY_ROWS, dm)).astype(BF16)

    for c in pair_copies(1):
        c.start()

    def load_pair(p, carry):
        for c in pair_copies(p):
            c.wait()

        def prefetch():
            for c in pair_copies(p + 2):
                c.start()

        for i in range(3):
            w = stage[i, pair_rows(p), :]
            early_qkv[p, :, i * pw:(i + 1) * pw] = _nt(early_xn[...], w)
            wqkv[p, :, i * pw:(i + 1) * pw] = _pack(w.T)
            if i == 0:
                pl.when(p + 2 < n_pairs)(prefetch)
        wo[pl.ds(pl.multiple_of(p * half, half), half), :] = _pack(stage[3, pair_rows(p), :])
        wide = x_stage[pl.ds(p * x_chunk, x_chunk)].astype(F32).reshape(x_chunk * seg, dm)
        xres[pl.ds(pl.multiple_of(p * x_chunk * seg, x_chunk * seg), x_chunk * seg), :] = wide
        return carry

    with jax.named_scope("load"):
        lax.fori_loop(0, n_pairs, load_pair, 0)
    bqkv_copy.start()
    bwo_copy.start()

    def fold_phi(base):
        groups = [None] * n_grp
        for j, g0 in enumerate(first_grp):
            t = _nt(fold[j], bqkv_stage[:, base + j * 128:base + (j + 1) * 128]) * LOG2E
            for i in range(4):
                part = t[i * gw:(i + 1) * gw]
                groups[g0 + i] = part if groups[g0 + i] is None else groups[g0 + i] + part
        return groups

    def hedgehog_weights():
        bqkv_copy.wait()
        bwo_copy.wait()
        wvt = bqkv_stage[:, 2 * dm:].astype(F32).T
        for g, (wpq, wpk) in enumerate(zip(fold_phi(0), fold_phi(dm))):
            bwq[g * gw:(g + 1) * gw, :] = wpq
            bw1[2 * g * gw:(2 * g + 1) * gw, :] = wpk
            bw1[(2 * g + 1) * gw:(2 * g + 2) * gw, :] = wvt[g * gw:(g + 1) * gw]
        bwo[...] = _pack(bwo_stage[...])

    def seg_rows(s):
        return pl.ds(pl.multiple_of(s * seg, seg), seg)

    def rmt_step(s, mem, early):
        plan, vpu_pairs, norm_pair, order, ks = STEP_EARLY if early else STEP_REGULAR
        if early:
            h = jnp.concatenate([mem, xn_a[:seg - EARLY_ROWS, :]], axis=0).astype(BF16)
            early_rows = pl.ds(pl.multiple_of(s * EARLY_ROWS, EARLY_ROWS), EARLY_ROWS)
        else:
            h = jnp.concatenate([mem, xn_a[...]], axis=0)
        xn_next = _layernorm(xres[seg_rows(jnp.minimum(s + 1, n_seg - 1)), :])
        prev = seg_rows(jnp.maximum(s - 1, 0))
        xn_b[prev, :] = _layernorm(xres[prev, :]).astype(BF16)
        pending = {norm_pair: [xn_b[seg_rows(jnp.maximum(s, 1) - 1), :128].astype(F32)[:8]]}

        def project(p):
            if p == 0:
                start = _nn(h[:, :ks], _unpack(wqkv[p, :ks // 2, :]))
                t = _nn(h[:, ks:], _unpack(wqkv[p, ks // 2:, :])) + start
            else:
                t = _nn(h, _unpack(wqkv[p]))
            return jnp.concatenate([t, early_qkv[p, early_rows, :]], axis=0) if early else t

        def weighted_values(p, prob, v):
            head = prob[:n_mem]
            if p in pending:
                work = functools.reduce(jnp.add, pending[p])[:, :prob.shape[1]]
                head = jnp.where(s < 0, work, head)
            if p not in vpu_pairs:
                return _nn(jnp.concatenate([head, prob[n_mem:]], axis=0), _pair_blockdiag(v, dh))
            seen = n_mem + 8
            o = _nn(jnp.concatenate([head, prob[seen:]], axis=0), _pair_blockdiag(v, dh))
            v_scr[p, :seen, :] = v[:seen]
            v_scr[p, seen:seen + 1, :] = jnp.sum(v[seen:], axis=0, keepdims=True)
            first = jnp.concatenate(
                [prob[n_mem:seen], jnp.zeros((8, 128 - prob.shape[1]), F32)], axis=1)
            lane = _iota(first.shape, 1)
            tiles = [None] * (pw // 128)
            for k in range(seen + 1):
                wa, wb = (jnp.sum(jnp.where(lane == col, first, 0.0), axis=1, keepdims=True)
                          for col in (k, prob.shape[0] + k))
                for t, c in enumerate(range(0, pw, 128)):
                    w = wa if c + 128 <= dh else wb if c >= dh else jnp.where(lane < dh - c, wa, wb)
                    term = w * jnp.broadcast_to(v_scr[p, k:k + 1, c:c + 128], (8, 128))
                    tiles[t] = term if k == 0 else tiles[t] + term
            pending.setdefault(p + 1, []).extend(tiles)
            return jnp.concatenate([o[:n_mem], jnp.concatenate(tiles, axis=1), o[n_mem:]], axis=0)

        def out_proj(acc, lo, hi, cols=slice(None)):
            t = _nn(o_scr[:, lo * pw:hi * pw], _unpack(wo[lo * half:hi * half, cols]))
            return t if acc is None else t + acc[:, cols]

        qkv, prob = {}, {}
        acc, done = None, 0
        for p in range(len(plan)):
            r = p - (len(plan) - n_pairs)
            for what in order:
                if what == "q" and p < n_pairs:
                    qkv[p] = project(p)
                if what == "o" and plan[p] != "0":
                    acc = out_proj(acc, done, done + int(plan[p]))
                    done += int(plan[p])
                if what == "s" and 0 <= p - 1 < n_pairs:
                    t = qkv[p - 1]
                    scores = _nt(t[:, :pw], _pair_blockdiag(t[:, pw:2 * pw], dh))
                    prob[p - 1] = _pair_softmax(scores, n_mem, scale)
                if what == "v" and r >= 0:
                    o_scr[:, r * pw:(r + 1) * pw] = weighted_values(r, prob[r], qkv[r][:, 2 * pw:])
        acc = out_proj(acc, done, done + 1)
        acc = jnp.concatenate(
            [out_proj(acc, done + 1, n_pairs, cols) for cols in (slice(0, ks), slice(ks, dm))], axis=1)
        xn_a[...] = xn_next
        rows = seg_rows(s)
        xres[rows, :] = xres[rows, :] + acc[n_mem:]
        return acc[:n_mem]

    def rmt_steps(lo, hi, mem, early):
        def body(i, mem):
            for u in range(unroll):
                mem = rmt_step(i * unroll + u, mem, early)
            return mem

        return lax.fori_loop(lo, hi, body, mem)

    def rmt_layer(layer):
        xn_a[...] = _layernorm(xres[0:seg, :])
        split = jnp.where(layer == 0, n_early // unroll, 0)
        mem = rmt_steps(0, split, mem0_ref[...].astype(F32), True)
        rmt_steps(split, n_seg // unroll, mem, False)
        last = slice(seq - seg, seq)
        xn_b[last, :] = _layernorm(xres[last, :]).astype(BF16)

    chunk = 4
    n_chunk = n_grp // chunk

    def blk_rows(i):
        return pl.ds(pl.multiple_of(i * tb, tb), tb)

    def kv_block(i, carry):
        xn = xn_b[blk_rows(i), :]
        proj = {}
        for c in range(n_chunk + 1):
            if c < n_chunk:
                proj[c] = _nt(bw1[2 * c * chunk * gw:2 * (c + 1) * chunk * gw, :], xn)
            if c >= 1:
                t = proj[c - 1]
                for j in range(chunk):
                    g = (c - 1) * chunk + j
                    phi = _feature_map(t[2 * j * gw:(2 * j + 1) * gw])
                    kv_acc[g] += _nt(t[(2 * j + 1) * gw:(2 * j + 2) * gw], phi.astype(BF16))
                    z_acc[g] += functools.reduce(jnp.add, [phi[:, i:i + 128] for i in range(0, tb, 128)])
        return carry

    def out_copy(i):
        return pltpu.make_async_copy(out_stage.at[blk_rows(i)], out_hbm.at[blk_rows(i)], out_sem.at[i])

    def out_block(i, layer):
        rows = blk_rows(i)
        xn = xn_b[rows, :]
        sublane = _iota((8, tb), 0)
        proj, outs = {}, []

        def out_proj(y, lo, hi):
            o = jnp.concatenate(outs, axis=0)[lo:hi].astype(BF16).T
            return _nn(o, _unpack(bwo[lo // 2:hi // 2, :])) + y

        y = xres[rows, :]
        for c in range(n_chunk + 1):
            if c < n_chunk:
                proj[c] = _nt(bwq[c * chunk * gw:(c + 1) * chunk * gw, :], xn)
            else:
                y = out_proj(y, 0, 256)
            if c >= 1:
                for j in range(chunk):
                    g = (c - 1) * chunk + j
                    phi = _feature_map(proj[c - 1][j * gw:(j + 1) * gw])
                    z = jnp.concatenate([z_acc[g]] * (tb // 128), axis=1)
                    inv = _recip(_over_features(phi * z, jnp.add) + DEN_EPS)
                    swapped = pltpu.roll(inv, 1, 0)
                    inv_a = jnp.where(sublane % 2 == 0, inv, swapped)
                    inv_b = jnp.where(sublane % 2 == 0, swapped, inv)
                    inv_ab = jnp.where(sublane < bdh % 8, inv_a, inv_b)
                    outs.append(_nn(kv_acc[g], phi.astype(BF16))
                                * jnp.concatenate([inv_a, inv_a, inv_ab, inv_b, inv_b], axis=0))
        y = out_proj(out_proj(y, 256, 384), 384, dm)
        xres[rows, :] = y
        out_stage[rows, :] = y.astype(BF16)

        @pl.when(layer == n_layers - 1)
        def _():
            out_copy(i).start()

        return layer

    def hedgehog_layer(layer):
        kv_acc[...] = jnp.zeros(kv_acc.shape, F32)
        z_acc[...] = jnp.zeros(z_acc.shape, F32)
        lax.fori_loop(0, seq // tb, kv_block, 0)
        shape = kv_acc.shape[1:]
        same_head = _iota(shape, 0) // bdh == _iota(shape, 1) % 2
        for g in range(n_grp):
            kv_acc[g] = jnp.where(same_head, kv_acc[g], 0.0)
            z_acc[g] = jnp.broadcast_to(jnp.sum(z_acc[g], axis=1, keepdims=True), z_acc.shape[1:])
        lax.fori_loop(0, seq // tb, out_block, layer)

    def layer_pair(layer, carry):
        with jax.named_scope("rmt"):
            rmt_layer(layer)
        pl.when(layer == 0)(hedgehog_weights)
        with jax.named_scope("hedgehog"):
            hedgehog_layer(layer)
        return carry

    lax.fori_loop(0, n_layers, layer_pair, 0)
    for i in range(seq // tb):
        out_copy(i).wait()


@functools.partial(jax.jit, static_argnames=("A_seg_len",))
def pallas_interleave_layers__memory_aug_recurrent_mem_tr__linear_kernel_hedgehog__prompt_kernel(
    A_x: jax.Array,
    A_mem0: jax.Array,
    A_Wq: jax.Array,
    A_Wk: jax.Array,
    A_Wv: jax.Array,
    A_Wo: jax.Array,
    A_seg_len: int,
    B_x: jax.Array,
    B_wqkv: jax.Array,
    B_w_phi: jax.Array,
    B_wo: jax.Array,
):
    del B_x
    batch, seq, dm = A_x.shape
    _, heads, dh = A_Wq.shape
    n_mem = A_mem0.shape[1]
    bh, bdh, _ = B_w_phi.shape
    seg = int(A_seg_len)
    assert batch == 1 and bdh == 20 and bh * bdh == dm and heads % 2 == 0
    assert (2 * dh) % 128 == 0 and n_mem % 8 == 0 and seg % 16 == 0 and 2 * (n_mem + seg) <= 128
    n_pairs, pw, hd = heads // 2, 2 * dh, heads * dh
    tb, unroll, n_early = 512, 2, 48

    def feature_major(w):
        return jnp.transpose(w, (1, 2, 0)).reshape(hd, dm)

    hbm = pl.BlockSpec(memory_space=pl.ANY)
    vmem = pl.BlockSpec(memory_space=pltpu.VMEM)
    out = pl.pallas_call(
        functools.partial(_kernel, seg=seg, dh=dh, n_layers=2, tb=tb, unroll=unroll),
        out_shape=jax.ShapeDtypeStruct((seq, dm), A_x.dtype),
        in_specs=[hbm, vmem, hbm, hbm, hbm, hbm, hbm, vmem, hbm],
        out_specs=hbm,
        scratch_shapes=[
            pltpu.VMEM((4, hd, dm), BF16),
            pltpu.VMEM((n_pairs, dm // 2, 3 * pw), U32),
            pltpu.VMEM((hd // 2, dm), U32),
            pltpu.VMEM((seq // seg, seg, dm), BF16),
            pltpu.VMEM((seq, dm), BF16),
            pltpu.VMEM((dm, 3 * dm), BF16),
            pltpu.VMEM((dm, dm), BF16),
            pltpu.VMEM((dm // 128, 8 * bdh, 128), BF16),
            pltpu.VMEM((2 * dm, dm), F32),
            pltpu.VMEM((dm, dm), F32),
            pltpu.VMEM((dm // 2, dm), U32),
            pltpu.VMEM((seq, dm), F32),
            pltpu.VMEM((seg, dm), F32),
            pltpu.VMEM((seq, dm), BF16),
            pltpu.VMEM((n_mem + seg, hd), F32),
            pltpu.VMEM((n_pairs, n_mem + 16, pw), F32),
            pltpu.VMEM((bh // 2, 2 * bdh, 4 * bdh), F32),
            pltpu.VMEM((bh // 2, 4 * bdh, 128), F32),
            pltpu.VMEM((n_early, EARLY_ROWS, dm), BF16),
            pltpu.VMEM((n_early * EARLY_ROWS, dm), BF16),
            pltpu.VMEM((n_pairs, n_early * EARLY_ROWS, 3 * pw), F32),
            pltpu.SemaphoreType.DMA((5, n_pairs)),
            pltpu.SemaphoreType.DMA((3,)),
            pltpu.SemaphoreType.DMA((seq // tb,)),
        ],
        compiler_params=pltpu.CompilerParams(vmem_limit_bytes=120 * 1024 * 1024),
        name="rmt_hedgehog",
    )(
        A_x.reshape(seq // seg, seg, dm),
        A_mem0.reshape(n_mem, dm),
        feature_major(A_Wq),
        feature_major(A_Wk),
        feature_major(A_Wv),
        A_Wo.reshape(hd, dm),
        B_wqkv,
        jnp.transpose(B_w_phi, (1, 2, 0)),
        B_wo,
    )
    return out.reshape(batch, seq, dm)
```

```python
import functools
import math

import jax
import jax.numpy as jnp
from jax import lax
import jax.experimental.pallas as pl
import jax.experimental.pallas.tpu as pltpu

F32 = jnp.float32
BF16 = jnp.bfloat16
U32 = jnp.uint32
I32 = jnp.int32

LN_EPS = 1e-5
DEN_EPS = 1e-6
LOG2E = math.log2(math.e)
EARLY_ROWS = 8
EARLY_TILES = ((0, 3), (4, 6), (7, 9))
STEP_REGULAR = ("00000000000111112222", range(0, 16), 9, "qosv", 256)
STEP_EARLY = ("00000000000111112222", range(0, 16), 9, "qosv", 256)


def _nn(a, b):
    return lax.dot_general(a, b, (((1,), (0,)), ((), ())), preferred_element_type=F32)


def _nt(a, b):
    return lax.dot_general(a, b, (((1,), (1,)), ((), ())), preferred_element_type=F32)


def _unpack(x):
    return pltpu.bitcast(x, BF16)


def _pack(x):
    return pltpu.bitcast(x, U32)


def _iota(shape, dim):
    return lax.broadcasted_iota(I32, shape, dim)


def _recip(x):
    r = pltpu.reciprocal(x, approx=True)
    return r * (2.0 - x * r)


def _layernorm(x):
    inv_n = 1.0 / x.shape[-1]
    m = jnp.sum(x, axis=-1, keepdims=True) * inv_n
    d = x - m
    v = jnp.sum(d * d, axis=-1, keepdims=True) * inv_n
    return d * lax.rsqrt(v + LN_EPS)


def _pair_blockdiag(x, dh):
    rows, width = x.shape
    top, bot = [], []
    zero = jnp.zeros((rows, 128), F32)
    for c in range(0, width, 128):
        t = x[:, c:c + 128]
        if c + 128 <= dh:
            top.append(t)
            bot.append(zero)
        elif c >= dh:
            top.append(zero)
            bot.append(t)
        else:
            first = _iota((rows, 128), 1) < dh - c
            top.append(jnp.where(first, t, 0.0))
            bot.append(jnp.where(first, 0.0, t))
    return jnp.concatenate(
        [jnp.concatenate(top, axis=1), jnp.concatenate(bot, axis=1)], axis=0
    ).astype(BF16)


def _pair_softmax(s, n_mem, scale):
    rows = s.shape[0]
    row = _iota(s.shape, 0)
    col = _iota(s.shape, 1)
    is_a = col < rows
    key = jnp.where(is_a, col, col - rows)
    s = jnp.where((row < n_mem) | (row >= key), s * scale, -1000000000.0)
    ma = jnp.max(jnp.where(is_a, s, -jnp.inf), axis=1, keepdims=True)
    mb = jnp.max(jnp.where(is_a, -jnp.inf, s), axis=1, keepdims=True)
    e = jnp.exp(s - jnp.where(is_a, ma, mb))
    la = jnp.sum(jnp.where(is_a, e, 0.0), axis=1, keepdims=True)
    lb = jnp.sum(jnp.where(is_a, 0.0, e), axis=1, keepdims=True)
    return e / jnp.where(is_a, la, lb)


def _over_features(x, op):
    r = functools.reduce(op, [x[i:i + 8] for i in range(0, x.shape[0], 8)])
    r = op(r, pltpu.roll(r, 4, 0))
    return op(r, pltpu.roll(r, 2, 0))


def _feature_map(p):
    def tile(r):
        return jnp.concatenate([r] * (p.shape[0] // 8), axis=0)

    ep = jnp.exp2(p - tile(_over_features(p, jnp.maximum)))
    en = jnp.exp2(tile(_over_features(p, jnp.minimum)) - p)
    return jnp.concatenate([e * tile(_recip(_over_features(e, jnp.add))) for e in (ep, en)], axis=0)


def _kernel(x_hbm, mem0_ref, wq_hbm, wk_hbm, wv_hbm, wo_hbm, bqkv_hbm, wphi_ref, bwo_hbm,
            out_hbm,
            stage, wqkv, wo, x_stage, out_stage, bqkv_stage, bwo_stage, fold, bw1, bwq, bwo,
            xres, xn_a, xn_b, o_scr, v_scr, kv_acc, z_acc, early_x, early_xn, early_qkv,
            w_sem, b_sem, out_sem,
            *, seg, dh, n_layers, tb, unroll):
    n_pairs = wqkv.shape[0]
    pw = 2 * dh
    half = pw // 2
    seq, dm = xres.shape
    n_mem = mem0_ref.shape[0]
    n_seg = seq // seg
    scale = dh ** -0.5
    bdh, _, bh = wphi_ref.shape
    n_grp = bh // 2
    gw = 2 * bdh

    x_chunk = n_seg // n_pairs

    def pair_rows(p):
        return pl.ds(pl.multiple_of(p * pw, pw), pw)

    def pair_copies(p):
        rows = pair_rows(p)
        segs = pl.ds(p * x_chunk, x_chunk)
        return [pltpu.make_async_copy(src.at[rows], stage.at[i, rows], w_sem.at[i, p])
                for i, src in enumerate((wq_hbm, wk_hbm, wv_hbm, wo_hbm))] + [
            pltpu.make_async_copy(x_hbm.at[segs], x_stage.at[segs], w_sem.at[4, p])]

    early_copy = pltpu.make_async_copy(
        x_hbm.at[:, pl.ds(seg - EARLY_ROWS, EARLY_ROWS)], early_x, b_sem.at[0])
    bqkv_copy = pltpu.make_async_copy(bqkv_hbm, bqkv_stage, b_sem.at[1])
    bwo_copy = pltpu.make_async_copy(bwo_hbm, bwo_stage, b_sem.at[2])
    early_copy.start()

    with jax.named_scope("phi_blocks"):
        wphi = wphi_ref[...].astype(F32)
        wf = jnp.concatenate([wphi[d] for d in range(bdh)], axis=1)
        src = _iota((dm, 128), 0)
        natural = (src % bh) * bdh + src // bh
        first_grp = [c // gw for c in range(0, dm, 128)]
        r = _iota((4 * gw, 128), 0)
        lane = _iota((4 * gw, 128), 1)
        pick = ((r % gw) // 2 == lane).astype(BF16)
        head_start = ((r // gw) * 2 + r % 2) * bdh
        for j, g0 in enumerate(first_grp):
            wj = _nn(wf, (natural == _iota((dm, 128), 1) + j * 128).astype(BF16))
            wj = jnp.concatenate([wj, jnp.zeros((128 - bdh, 128), F32)], axis=0).astype(BF16)
            d = lane + (j * 128 - g0 * gw) - head_start
            fold[j] = jnp.where((d >= 0) & (d < bdh), _nn(pick, wj), 0.0).astype(BF16)

        for c in pair_copies(0):
            c.start()
    with jax.named_scope("early_norm"):
        early_copy.wait()
        early_xn[...] = _layernorm(
            early_x[...].astype(F32).reshape(early_xn.shape)).astype(BF16)

        for c in pair_copies(1):
            c.start()

    def load_pair(p, carry):
        for c in pair_copies(p):
            c.wait()

        @pl.when(p + 2 < n_pairs)
        def _():
            for c in pair_copies(p + 2):
                c.start()

        col = 0
        for i, (lo, hi) in enumerate(EARLY_TILES):
            w = stage[i, pair_rows(p), :]
            early_qkv[p, :, col:col + (hi - lo) * 128] = _nt(
                early_xn[...], w[lo * 128 - i * pw:hi * 128 - i * pw])
            col += (hi - lo) * 128
            wqkv[p, :, i * pw:(i + 1) * pw] = _pack(w.T)
        wo[pl.ds(pl.multiple_of(p * half, half), half), :] = _pack(stage[3, pair_rows(p), :])
        wide = x_stage[pl.ds(p * x_chunk, x_chunk)].astype(F32).reshape(x_chunk * seg, dm)
        xres[pl.ds(pl.multiple_of(p * x_chunk * seg, x_chunk * seg), x_chunk * seg), :] = wide
        return carry

    with jax.named_scope("load"):
        lax.fori_loop(0, n_pairs, load_pair, 0)
    bqkv_copy.start()
    bwo_copy.start()

    def fold_phi(base):
        groups = [None] * n_grp
        for j, g0 in enumerate(first_grp):
            t = _nt(fold[j], bqkv_stage[:, base + j * 128:base + (j + 1) * 128]) * LOG2E
            for i in range(4):
                part = t[i * gw:(i + 1) * gw]
                groups[g0 + i] = part if groups[g0 + i] is None else groups[g0 + i] + part
        return groups

    def hedgehog_weights():
        bqkv_copy.wait()
        bwo_copy.wait()
        wvt = bqkv_stage[:, 2 * dm:].astype(F32).T
        for g, (wpq, wpk) in enumerate(zip(fold_phi(0), fold_phi(dm))):
            bwq[g * gw:(g + 1) * gw, :] = wpq
            bw1[2 * g * gw:(2 * g + 1) * gw, :] = wpk
            bw1[(2 * g + 1) * gw:(2 * g + 2) * gw, :] = wvt[g * gw:(g + 1) * gw]
        bwo[...] = _pack(bwo_stage[...])

    def seg_rows(s):
        return pl.ds(pl.multiple_of(s * seg, seg), seg)

    def rmt_step(s, mem, early):
        plan, vpu_pairs, norm_pair, order, ks = STEP_EARLY if early else STEP_REGULAR
        h = jnp.concatenate([mem, xn_a[...]], axis=0)
        h_short = h[:-EARLY_ROWS].astype(BF16)
        early_rows = pl.ds(pl.multiple_of(s * EARLY_ROWS, EARLY_ROWS), EARLY_ROWS)
        xn_next = _layernorm(xres[seg_rows(jnp.minimum(s + 1, n_seg - 1)), :])
        prev = seg_rows(jnp.maximum(s - 1, 0))
        xn_b[prev, :] = _layernorm(xres[prev, :]).astype(BF16)
        pending = {norm_pair: [xn_b[seg_rows(jnp.maximum(s, 1) - 1), :128].astype(F32)[:8]]}

        def project(p):
            spans, end = [], 0
            for lo, hi in EARLY_TILES if early else ():
                spans += [(h, end, lo)] * (end < lo) + [(h_short, lo, hi)]
                end = hi
            spans += [(h, end, 3 * pw // 128)] * (end < 3 * pw // 128)
            spans = [(x, slice(lo * 128, hi * 128)) for x, lo, hi in spans]
            if p > 0:
                parts = [_nn(x, _unpack(wqkv[p, :, cols])) for x, cols in spans]
            else:
                parts = [_nn(x[:, :ks], _unpack(wqkv[p, :ks // 2, cols])) for x, cols in spans]
                parts = [_nn(x[:, ks:], _unpack(wqkv[p, ks // 2:, cols])) + start
                         for start, (x, cols) in zip(parts, spans)]
            col = 0
            for i, t in enumerate(parts):
                if t.shape[0] < h.shape[0]:
                    known = early_qkv[p, early_rows, col:col + t.shape[1]]
                    parts[i] = jnp.concatenate([t, known], axis=0)
                    col += t.shape[1]
            return jnp.concatenate(parts, axis=1)

        def weighted_values(p, prob, v):
            head = prob[:n_mem]
            if p in pending:
                work = functools.reduce(jnp.add, pending[p])[:, :prob.shape[1]]
                head = jnp.where(s < 0, work, head)
            if p not in vpu_pairs:
                return _nn(jnp.concatenate([head, prob[n_mem:]], axis=0), _pair_blockdiag(v, dh))
            seen = n_mem + 8
            o = _nn(jnp.concatenate([head, prob[seen:]], axis=0), _pair_blockdiag(v, dh))
            v_scr[p, :seen, :] = v[:seen]
            v_scr[p, seen:seen + 1, :] = jnp.sum(v[seen:], axis=0, keepdims=True)
            first = jnp.concatenate(
                [prob[n_mem:seen], jnp.zeros((8, 128 - prob.shape[1]), F32)], axis=1)
            lane = _iota(first.shape, 1)
            tiles = [None] * (pw // 128)
            for k in range(seen + 1):
                wa, wb = (jnp.sum(jnp.where(lane == col, first, 0.0), axis=1, keepdims=True)
                          for col in (k, prob.shape[0] + k))
                for t, c in enumerate(range(0, pw, 128)):
                    w = wa if c + 128 <= dh else wb if c >= dh else jnp.where(lane < dh - c, wa, wb)
                    term = w * jnp.broadcast_to(v_scr[p, k:k + 1, c:c + 128], (8, 128))
                    tiles[t] = term if k == 0 else tiles[t] + term
            pending.setdefault(p + 1, []).extend(tiles)
            return jnp.concatenate([o[:n_mem], jnp.concatenate(tiles, axis=1), o[n_mem:]], axis=0)

        def out_proj(acc, lo, hi, cols=slice(None)):
            t = _nn(o_scr[:, lo * pw:hi * pw], _unpack(wo[lo * half:hi * half, cols]))
            return t if acc is None else t + acc[:, cols]

        qkv, prob = {}, {}
        acc, done = None, 0
        for p in range(len(plan)):
            r = p - (len(plan) - n_pairs)
            for what in order:
                if what == "q" and p < n_pairs:
                    qkv[p] = project(p)
                if what == "o" and plan[p] != "0":
                    acc = out_proj(acc, done, done + int(plan[p]))
                    done += int(plan[p])
                if what == "s" and 0 <= p - 1 < n_pairs:
                    t = qkv[p - 1]
                    scores = _nt(t[:, :pw], _pair_blockdiag(t[:, pw:2 * pw], dh))
                    prob[p - 1] = _pair_softmax(scores, n_mem, scale)
                if what == "v" and r >= 0:
                    o_scr[:, r * pw:(r + 1) * pw] = weighted_values(r, prob[r], qkv[r][:, 2 * pw:])
        acc = out_proj(acc, done, done + 1)
        acc = jnp.concatenate(
            [out_proj(acc, done + 1, n_pairs, cols) for cols in (slice(0, ks), slice(ks, dm))], axis=1)
        xn_a[...] = xn_next
        rows = seg_rows(s)
        xres[rows, :] = xres[rows, :] + acc[n_mem:]
        return acc[:n_mem]

    def rmt_steps(early):
        def body(i, mem):
            for u in range(unroll):
                mem = rmt_step(i * unroll + u, mem, early)
            return mem

        lax.fori_loop(0, n_seg // unroll, body, mem0_ref[...].astype(F32))

    def rmt_layer(layer):
        xn_a[...] = _layernorm(xres[0:seg, :])
        pl.when(layer == 0)(functools.partial(rmt_steps, True))
        pl.when(layer > 0)(functools.partial(rmt_steps, False))
        last = slice(seq - seg, seq)
        xn_b[last, :] = _layernorm(xres[last, :]).astype(BF16)

    chunk = 4
    n_chunk = n_grp // chunk

    def blk_rows(i):
        return pl.ds(pl.multiple_of(i * tb, tb), tb)

    def kv_block(i, carry):
        xn = xn_b[blk_rows(i), :]
        proj = {}
        for c in range(n_chunk + 1):
            if c < n_chunk:
                proj[c] = _nt(bw1[2 * c * chunk * gw:2 * (c + 1) * chunk * gw, :], xn)
            if c >= 1:
                t = proj[c - 1]
                for j in range(chunk):
                    g = (c - 1) * chunk + j
                    phi = _feature_map(t[2 * j * gw:(2 * j + 1) * gw])
                    kv_acc[g] += _nt(t[(2 * j + 1) * gw:(2 * j + 2) * gw], phi.astype(BF16))
                    z_acc[g] += functools.reduce(jnp.add, [phi[:, i:i + 128] for i in range(0, tb, 128)])
        return carry

    def out_copy(i):
        return pltpu.make_async_copy(out_stage.at[blk_rows(i)], out_hbm.at[blk_rows(i)], out_sem.at[i])

    def out_block(i, layer):
        rows = blk_rows(i)
        xn = xn_b[rows, :]
        sublane = _iota((8, tb), 0)
        proj, outs = {}, []

        def out_proj(y, lo, hi):
            o = jnp.concatenate(outs, axis=0)[lo:hi].astype(BF16).T
            return _nn(o, _unpack(bwo[lo // 2:hi // 2, :])) + y

        y = xres[rows, :]
        for c in range(n_chunk + 1):
            if c < n_chunk:
                proj[c] = _nt(bwq[c * chunk * gw:(c + 1) * chunk * gw, :], xn)
            else:
                y = out_proj(y, 0, 256)
            if c >= 1:
                for j in range(chunk):
                    g = (c - 1) * chunk + j
                    phi = _feature_map(proj[c - 1][j * gw:(j + 1) * gw])
                    z = jnp.concatenate([z_acc[g]] * (tb // 128), axis=1)
                    inv = _recip(_over_features(phi * z, jnp.add) + DEN_EPS)
                    swapped = pltpu.roll(inv, 1, 0)
                    inv_a = jnp.where(sublane % 2 == 0, inv, swapped)
                    inv_b = jnp.where(sublane % 2 == 0, swapped, inv)
                    inv_ab = jnp.where(sublane < bdh % 8, inv_a, inv_b)
                    outs.append(_nn(kv_acc[g], phi.astype(BF16))
                                * jnp.concatenate([inv_a, inv_a, inv_ab, inv_b, inv_b], axis=0))
        y = out_proj(out_proj(y, 256, 384), 384, dm)
        xres[rows, :] = y
        out_stage[rows, :] = y.astype(BF16)

        @pl.when(layer == n_layers - 1)
        def _():
            out_copy(i).start()

        return layer

    def hedgehog_layer(layer):
        kv_acc[...] = jnp.zeros(kv_acc.shape, F32)
        z_acc[...] = jnp.zeros(z_acc.shape, F32)
        lax.fori_loop(0, seq // tb, kv_block, 0)
        shape = kv_acc.shape[1:]
        same_head = _iota(shape, 0) // bdh == _iota(shape, 1) % 2
        for g in range(n_grp):
            kv_acc[g] = jnp.where(same_head, kv_acc[g], 0.0)
            z_acc[g] = jnp.broadcast_to(jnp.sum(z_acc[g], axis=1, keepdims=True), z_acc.shape[1:])
        lax.fori_loop(0, seq // tb, out_block, layer)

    def layer_pair(layer, carry):
        with jax.named_scope("rmt"):
            rmt_layer(layer)
        pl.when(layer == 0)(hedgehog_weights)
        with jax.named_scope("hedgehog"):
            hedgehog_layer(layer)
        return carry

    lax.fori_loop(0, n_layers, layer_pair, 0)
    for i in range(seq // tb):
        out_copy(i).wait()


@functools.partial(jax.jit, static_argnames=("A_seg_len",))
def pallas_interleave_layers__memory_aug_recurrent_mem_tr__linear_kernel_hedgehog__prompt_kernel(
    A_x: jax.Array,
    A_mem0: jax.Array,
    A_Wq: jax.Array,
    A_Wk: jax.Array,
    A_Wv: jax.Array,
    A_Wo: jax.Array,
    A_seg_len: int,
    B_x: jax.Array,
    B_wqkv: jax.Array,
    B_w_phi: jax.Array,
    B_wo: jax.Array,
):
    del B_x
    batch, seq, dm = A_x.shape
    _, heads, dh = A_Wq.shape
    n_mem = A_mem0.shape[1]
    bh, bdh, _ = B_w_phi.shape
    seg = int(A_seg_len)
    assert batch == 1 and bdh == 20 and bh * bdh == dm and heads % 2 == 0
    assert (2 * dh) % 128 == 0 and n_mem % 8 == 0 and seg % 16 == 0 and 2 * (n_mem + seg) <= 128
    n_pairs, pw, hd = heads // 2, 2 * dh, heads * dh
    tb, unroll = 512, 2
    early_rows = seq // seg * EARLY_ROWS
    early_cols = 128 * sum(hi - lo for lo, hi in EARLY_TILES)

    def feature_major(w):
        return jnp.transpose(w, (1, 2, 0)).reshape(hd, dm)

    hbm = pl.BlockSpec(memory_space=pl.ANY)
    vmem = pl.BlockSpec(memory_space=pltpu.VMEM)
    out = pl.pallas_call(
        functools.partial(_kernel, seg=seg, dh=dh, n_layers=2, tb=tb, unroll=unroll),
        out_shape=jax.ShapeDtypeStruct((seq, dm), A_x.dtype),
        in_specs=[hbm, vmem, hbm, hbm, hbm, hbm, hbm, vmem, hbm],
        out_specs=hbm,
        scratch_shapes=[
            pltpu.VMEM((4, hd, dm), BF16),
            pltpu.VMEM((n_pairs, dm // 2, 3 * pw), U32),
            pltpu.VMEM((hd // 2, dm), U32),
            pltpu.VMEM((seq // seg, seg, dm), BF16),
            pltpu.VMEM((seq, dm), BF16),
            pltpu.VMEM((dm, 3 * dm), BF16),
            pltpu.VMEM((dm, dm), BF16),
            pltpu.VMEM((dm // 128, 8 * bdh, 128), BF16),
            pltpu.VMEM((2 * dm, dm), F32),
            pltpu.VMEM((dm, dm), F32),
            pltpu.VMEM((dm // 2, dm), U32),
            pltpu.VMEM((seq, dm), F32),
            pltpu.VMEM((seg, dm), F32),
            pltpu.VMEM((seq, dm), BF16),
            pltpu.VMEM((n_mem + seg, hd), F32),
            pltpu.VMEM((n_pairs, n_mem + 16, pw), F32),
            pltpu.VMEM((bh // 2, 2 * bdh, 4 * bdh), F32),
            pltpu.VMEM((bh // 2, 4 * bdh, 128), F32),
            pltpu.VMEM((seq // seg, EARLY_ROWS, dm), BF16),
            pltpu.VMEM((early_rows, dm), BF16),
            pltpu.VMEM((n_pairs, early_rows, early_cols), F32),
            pltpu.SemaphoreType.DMA((5, n_pairs)),
            pltpu.SemaphoreType.DMA((3,)),
            pltpu.SemaphoreType.DMA((seq // tb,)),
        ],
        compiler_params=pltpu.CompilerParams(vmem_limit_bytes=120 * 1024 * 1024),
        name="rmt_hedgehog",
    )(
        A_x.reshape(seq // seg, seg, dm),
        A_mem0.reshape(n_mem, dm),
        feature_major(A_Wq),
        feature_major(A_Wk),
        feature_major(A_Wv),
        A_Wo.reshape(hd, dm),
        B_wqkv,
        jnp.transpose(B_w_phi, (1, 2, 0)),
        B_wo,
    )
    return out.reshape(batch, seq, dm)
```

```python
import functools
import math

import jax
import jax.numpy as jnp
from jax import lax
import jax.experimental.pallas as pl
import jax.experimental.pallas.tpu as pltpu

F32 = jnp.float32
BF16 = jnp.bfloat16
U32 = jnp.uint32
I32 = jnp.int32

LN_EPS = 1e-5
DEN_EPS = 1e-6
LOG2E = math.log2(math.e)
EARLY_ROWS = 8
EARLY_TILES = ((0, 3), (4, 6), (7, 9))
STEP_REGULAR = ("00000000000111112222", range(0, 16), 9, "qosv", 256)
STEP_EARLY = ("00000000000111112222", range(0, 16), 9, "qosv", 256)


def _nn(a, b):
    return lax.dot_general(a, b, (((1,), (0,)), ((), ())), preferred_element_type=F32)


def _nt(a, b):
    return lax.dot_general(a, b, (((1,), (1,)), ((), ())), preferred_element_type=F32)


def _unpack(x):
    return pltpu.bitcast(x, BF16)


def _pack(x):
    return pltpu.bitcast(x, U32)


def _iota(shape, dim):
    return lax.broadcasted_iota(I32, shape, dim)


def _recip(x):
    r = pltpu.reciprocal(x, approx=True)
    return r * (2.0 - x * r)


def _layernorm(x):
    inv_n = 1.0 / x.shape[-1]
    m = jnp.sum(x, axis=-1, keepdims=True) * inv_n
    d = x - m
    v = jnp.sum(d * d, axis=-1, keepdims=True) * inv_n
    return d * lax.rsqrt(v + LN_EPS)


def _pair_blockdiag(x, dh):
    rows, width = x.shape
    top, bot = [], []
    zero = jnp.zeros((rows, 128), F32)
    for c in range(0, width, 128):
        t = x[:, c:c + 128]
        if c + 128 <= dh:
            top.append(t)
            bot.append(zero)
        elif c >= dh:
            top.append(zero)
            bot.append(t)
        else:
            first = _iota((rows, 128), 1) < dh - c
            top.append(jnp.where(first, t, 0.0))
            bot.append(jnp.where(first, 0.0, t))
    return jnp.concatenate(
        [jnp.concatenate(top, axis=1), jnp.concatenate(bot, axis=1)], axis=0
    ).astype(BF16)


def _pair_softmax(s, n_mem, scale):
    rows = s.shape[0]
    row = _iota(s.shape, 0)
    col = _iota(s.shape, 1)
    is_a = col < rows
    key = jnp.where(is_a, col, col - rows)
    s = jnp.where((row < n_mem) | (row >= key), s * scale, -1000000000.0)
    ma = jnp.max(jnp.where(is_a, s, -jnp.inf), axis=1, keepdims=True)
    mb = jnp.max(jnp.where(is_a, -jnp.inf, s), axis=1, keepdims=True)
    e = jnp.exp(s - jnp.where(is_a, ma, mb))
    la = jnp.sum(jnp.where(is_a, e, 0.0), axis=1, keepdims=True)
    lb = jnp.sum(jnp.where(is_a, 0.0, e), axis=1, keepdims=True)
    return e / jnp.where(is_a, la, lb)


def _over_features(x, op):
    r = functools.reduce(op, [x[i:i + 8] for i in range(0, x.shape[0], 8)])
    r = op(r, pltpu.roll(r, 4, 0))
    return op(r, pltpu.roll(r, 2, 0))


def _feature_map(p):
    def tile(r):
        return jnp.concatenate([r] * (p.shape[0] // 8), axis=0)

    ep = jnp.exp2(p - tile(_over_features(p, jnp.maximum)))
    en = jnp.exp2(tile(_over_features(p, jnp.minimum)) - p)
    return jnp.concatenate([e * tile(_recip(_over_features(e, jnp.add))) for e in (ep, en)], axis=0)


def _kernel(x_hbm, mem0_ref, wq_hbm, wk_hbm, wv_hbm, wo_hbm, bqkv_hbm, wphi_ref, bwo_hbm,
            out_hbm,
            stage, wqkv, wo, x_stage, out_stage, bqkv_stage, bwo_stage, fold, bw1, bwq, bwo,
            xres, xn_a, xn_b, o_scr, v_scr, kv_acc, z_acc, early_x, early_xn, early_qkv,
            w_sem, b_sem, out_sem,
            *, seg, dh, n_layers, tb, unroll):
    n_pairs = wqkv.shape[0]
    pw = 2 * dh
    half = pw // 2
    seq, dm = xres.shape
    n_mem = mem0_ref.shape[0]
    n_seg = seq // seg
    scale = dh ** -0.5
    bdh, _, bh = wphi_ref.shape
    n_grp = bh // 2
    gw = 2 * bdh

    x_chunk = n_seg // n_pairs

    def pair_rows(p):
        return pl.ds(pl.multiple_of(p * pw, pw), pw)

    def pair_copies(p):
        rows = pair_rows(p)
        segs = pl.ds(p * x_chunk, x_chunk)
        return [pltpu.make_async_copy(src.at[rows], stage.at[i, rows], w_sem.at[i, p])
                for i, src in enumerate((wq_hbm, wk_hbm, wv_hbm, wo_hbm))] + [
            pltpu.make_async_copy(x_hbm.at[segs], x_stage.at[segs], w_sem.at[4, p])]

    early_copy = pltpu.make_async_copy(
        x_hbm.at[:, pl.ds(seg - EARLY_ROWS, EARLY_ROWS)], early_x, b_sem.at[0])
    bqkv_copy = pltpu.make_async_copy(bqkv_hbm, bqkv_stage, b_sem.at[1])
    bwo_copy = pltpu.make_async_copy(bwo_hbm, bwo_stage, b_sem.at[2])
    early_copy.start()

    wphi = wphi_ref[...].astype(F32)
    wf = jnp.concatenate([wphi[d] for d in range(bdh)], axis=1)
    src = _iota((dm, 128), 0)
    natural = (src % bh) * bdh + src // bh
    first_grp = [c // gw for c in range(0, dm, 128)]
    r = _iota((4 * gw, 128), 0)
    lane = _iota((4 * gw, 128), 1)
    pick = ((r % gw) // 2 == lane).astype(BF16)
    head_start = ((r // gw) * 2 + r % 2) * bdh
    for j, g0 in enumerate(first_grp):
        wj = _nn(wf, (natural == _iota((dm, 128), 1) + j * 128).astype(BF16))
        wj = jnp.concatenate([wj, jnp.zeros((128 - bdh, 128), F32)], axis=0).astype(BF16)
        d = lane + (j * 128 - g0 * gw) - head_start
        fold[j] = jnp.where((d >= 0) & (d < bdh), _nn(pick, wj), 0.0).astype(BF16)

    for c in pair_copies(0):
        c.start()
    early_copy.wait()
    early_xn[...] = _layernorm(
        early_x[...].astype(F32).reshape(early_xn.shape)).astype(BF16)

    for c in pair_copies(1):
        c.start()

    def load_pair(p, carry):
        for c in pair_copies(p):
            c.wait()

        @pl.when(p + 2 < n_pairs)
        def _():
            for c in pair_copies(p + 2):
                c.start()

        col = 0
        for i, (lo, hi) in enumerate(EARLY_TILES):
            w = stage[i, pair_rows(p), :]
            early_qkv[p, :, col:col + (hi - lo) * 128] = _nt(
                early_xn[...], w[lo * 128 - i * pw:hi * 128 - i * pw])
            col += (hi - lo) * 128
            wqkv[p, :, i * pw:(i + 1) * pw] = _pack(w.T)
        wo[pl.ds(pl.multiple_of(p * half, half), half), :] = _pack(stage[3, pair_rows(p), :])
        wide = x_stage[pl.ds(p * x_chunk, x_chunk)].astype(F32).reshape(x_chunk * seg, dm)
        xres[pl.ds(pl.multiple_of(p * x_chunk * seg, x_chunk * seg), x_chunk * seg), :] = wide
        return carry

    with jax.named_scope("load"):
        lax.fori_loop(0, n_pairs, load_pair, 0)
    bqkv_copy.start()
    bwo_copy.start()

    def fold_phi(base):
        groups = [None] * n_grp
        for j, g0 in enumerate(first_grp):
            t = _nt(fold[j], bqkv_stage[:, base + j * 128:base + (j + 1) * 128]) * LOG2E
            for i in range(4):
                part = t[i * gw:(i + 1) * gw]
                groups[g0 + i] = part if groups[g0 + i] is None else groups[g0 + i] + part
        return groups

    def hedgehog_weights():
        bqkv_copy.wait()
        bwo_copy.wait()
        wvt = bqkv_stage[:, 2 * dm:].astype(F32).T
        for g, (wpq, wpk) in enumerate(zip(fold_phi(0), fold_phi(dm))):
            bwq[g * gw:(g + 1) * gw, :] = wpq
            bw1[2 * g * gw:(2 * g + 1) * gw, :] = wpk
            bw1[(2 * g + 1) * gw:(2 * g + 2) * gw, :] = wvt[g * gw:(g + 1) * gw]
        bwo[...] = _pack(bwo_stage[...])

    def seg_rows(s):
        return pl.ds(pl.multiple_of(s * seg, seg), seg)

    def rmt_step(s, mem, early):
        plan, vpu_pairs, norm_pair, order, ks = STEP_EARLY if early else STEP_REGULAR
        h = jnp.concatenate([mem, xn_a[...]], axis=0)
        h_short = h[:-EARLY_ROWS].astype(BF16)
        early_rows = pl.ds(pl.multiple_of(s * EARLY_ROWS, EARLY_ROWS), EARLY_ROWS)
        xn_next = _layernorm(xres[seg_rows(jnp.minimum(s + 1, n_seg - 1)), :])
        prev = seg_rows(jnp.maximum(s - 1, 0))
        xn_b[prev, :] = _layernorm(xres[prev, :]).astype(BF16)
        pending = {norm_pair: [xn_b[seg_rows(jnp.maximum(s, 1) - 1), :128].astype(F32)[:8]]}

        def project(p):
            spans, end = [], 0
            for lo, hi in EARLY_TILES if early else ():
                spans += [(h, end, lo)] * (end < lo) + [(h_short, lo, hi)]
                end = hi
            spans += [(h, end, 3 * pw // 128)] * (end < 3 * pw // 128)
            spans = [(x, slice(lo * 128, hi * 128)) for x, lo, hi in spans]
            if p > 0:
                parts = [_nn(x, _unpack(wqkv[p, :, cols])) for x, cols in spans]
            else:
                parts = [_nn(x[:, :ks], _unpack(wqkv[p, :ks // 2, cols])) for x, cols in spans]
                parts = [_nn(x[:, ks:], _unpack(wqkv[p, ks // 2:, cols])) + start
                         for start, (x, cols) in zip(parts, spans)]
            col = 0
            for i, t in enumerate(parts):
                if t.shape[0] < h.shape[0]:
                    known = early_qkv[p, early_rows, col:col + t.shape[1]]
                    parts[i] = jnp.concatenate([t, known], axis=0)
                    col += t.shape[1]
            return jnp.concatenate(parts, axis=1)

        def weighted_values(p, prob, v):
            head = prob[:n_mem]
            if p in pending:
                work = functools.reduce(jnp.add, pending[p])[:, :prob.shape[1]]
                head = jnp.where(s < 0, work, head)
            if p not in vpu_pairs:
                return _nn(jnp.concatenate([head, prob[n_mem:]], axis=0), _pair_blockdiag(v, dh))
            seen = n_mem + 8
            o = _nn(jnp.concatenate([head, prob[seen:]], axis=0), _pair_blockdiag(v, dh))
            v_scr[p, :seen, :] = v[:seen]
            v_scr[p, seen:seen + 1, :] = jnp.sum(v[seen:], axis=0, keepdims=True)
            first = jnp.concatenate(
                [prob[n_mem:seen], jnp.zeros((8, 128 - prob.shape[1]), F32)], axis=1)
            lane = _iota(first.shape, 1)
            tiles = [None] * (pw // 128)
            for k in range(seen + 1):
                wa, wb = (jnp.sum(jnp.where(lane == col, first, 0.0), axis=1, keepdims=True)
                          for col in (k, prob.shape[0] + k))
                for t, c in enumerate(range(0, pw, 128)):
                    w = wa if c + 128 <= dh else wb if c >= dh else jnp.where(lane < dh - c, wa, wb)
                    term = w * jnp.broadcast_to(v_scr[p, k:k + 1, c:c + 128], (8, 128))
                    tiles[t] = term if k == 0 else tiles[t] + term
            pending.setdefault(p + 1, []).extend(tiles)
            return jnp.concatenate([o[:n_mem], jnp.concatenate(tiles, axis=1), o[n_mem:]], axis=0)

        def out_proj(acc, lo, hi, cols=slice(None)):
            t = _nn(o_scr[:, lo * pw:hi * pw], _unpack(wo[lo * half:hi * half, cols]))
            return t if acc is None else t + acc[:, cols]

        qkv, prob = {}, {}
        acc, done = None, 0
        for p in range(len(plan)):
            r = p - (len(plan) - n_pairs)
            for what in order:
                if what == "q" and p < n_pairs:
                    qkv[p] = project(p)
                if what == "o" and plan[p] != "0":
                    acc = out_proj(acc, done, done + int(plan[p]))
                    done += int(plan[p])
                if what == "s" and 0 <= p - 1 < n_pairs:
                    t = qkv[p - 1]
                    scores = _nt(t[:, :pw], _pair_blockdiag(t[:, pw:2 * pw], dh))
                    prob[p - 1] = _pair_softmax(scores, n_mem, scale)
                if what == "v" and r >= 0:
                    o_scr[:, r * pw:(r + 1) * pw] = weighted_values(r, prob[r], qkv[r][:, 2 * pw:])
        acc = out_proj(acc, done, done + 1)
        acc = jnp.concatenate(
            [out_proj(acc, done + 1, n_pairs, cols) for cols in (slice(0, ks), slice(ks, dm))], axis=1)
        xn_a[...] = xn_next
        rows = seg_rows(s)
        xres[rows, :] = xres[rows, :] + acc[n_mem:]
        return acc[:n_mem]

    def rmt_steps(early):
        def body(i, mem):
            for u in range(unroll):
                mem = rmt_step(i * unroll + u, mem, early)
            return mem

        lax.fori_loop(0, n_seg // unroll, body, mem0_ref[...].astype(F32))

    def rmt_layer(layer):
        xn_a[...] = _layernorm(xres[0:seg, :])
        pl.when(layer == 0)(functools.partial(rmt_steps, True))
        pl.when(layer > 0)(functools.partial(rmt_steps, False))
        last = slice(seq - seg, seq)
        xn_b[last, :] = _layernorm(xres[last, :]).astype(BF16)

    chunk = 4
    n_chunk = n_grp // chunk

    def blk_rows(i):
        return pl.ds(pl.multiple_of(i * tb, tb), tb)

    def kv_block(i, carry):
        xn = xn_b[blk_rows(i), :]
        proj = {}
        for c in range(n_chunk + 1):
            if c < n_chunk:
                proj[c] = _nt(bw1[2 * c * chunk * gw:2 * (c + 1) * chunk * gw, :], xn)
            if c >= 1:
                t = proj[c - 1]
                for j in range(chunk):
                    g = (c - 1) * chunk + j
                    phi = _feature_map(t[2 * j * gw:(2 * j + 1) * gw])
                    kv_acc[g] += _nt(t[(2 * j + 1) * gw:(2 * j + 2) * gw], phi.astype(BF16))
                    z_acc[g] += functools.reduce(jnp.add, [phi[:, i:i + 128] for i in range(0, tb, 128)])
        return carry

    def out_copy(i):
        return pltpu.make_async_copy(out_stage.at[blk_rows(i)], out_hbm.at[blk_rows(i)], out_sem.at[i])

    def out_block(i, layer):
        rows = blk_rows(i)
        xn = xn_b[rows, :]
        sublane = _iota((8, tb), 0)
        proj, outs = {}, []

        def out_proj(y, lo, hi):
            o = jnp.concatenate(outs, axis=0)[lo:hi].astype(BF16).T
            return _nn(o, _unpack(bwo[lo // 2:hi // 2, :])) + y

        y = xres[rows, :]
        for c in range(n_chunk + 1):
            if c < n_chunk:
                proj[c] = _nt(bwq[c * chunk * gw:(c + 1) * chunk * gw, :], xn)
            else:
                y = out_proj(y, 0, 256)
            if c >= 1:
                for j in range(chunk):
                    g = (c - 1) * chunk + j
                    phi = _feature_map(proj[c - 1][j * gw:(j + 1) * gw])
                    z = jnp.concatenate([z_acc[g]] * (tb // 128), axis=1)
                    inv = _recip(_over_features(phi * z, jnp.add) + DEN_EPS)
                    swapped = pltpu.roll(inv, 1, 0)
                    inv_a = jnp.where(sublane % 2 == 0, inv, swapped)
                    inv_b = jnp.where(sublane % 2 == 0, swapped, inv)
                    inv_ab = jnp.where(sublane < bdh % 8, inv_a, inv_b)
                    outs.append(_nn(kv_acc[g], phi.astype(BF16))
                                * jnp.concatenate([inv_a, inv_a, inv_ab, inv_b, inv_b], axis=0))
        y = out_proj(out_proj(y, 256, 384), 384, dm)
        xres[rows, :] = y
        out_stage[rows, :] = y.astype(BF16)

        @pl.when(layer == n_layers - 1)
        def _():
            out_copy(i).start()

        return layer

    def hedgehog_layer(layer):
        kv_acc[...] = jnp.zeros(kv_acc.shape, F32)
        z_acc[...] = jnp.zeros(z_acc.shape, F32)
        lax.fori_loop(0, seq // tb, kv_block, 0)
        shape = kv_acc.shape[1:]
        same_head = _iota(shape, 0) // bdh == _iota(shape, 1) % 2
        for g in range(n_grp):
            kv_acc[g] = jnp.where(same_head, kv_acc[g], 0.0)
            z_acc[g] = jnp.broadcast_to(jnp.sum(z_acc[g], axis=1, keepdims=True), z_acc.shape[1:])
        lax.fori_loop(0, seq // tb, out_block, layer)

    def layer_pair(layer, carry):
        with jax.named_scope("rmt"):
            rmt_layer(layer)
        pl.when(layer == 0)(hedgehog_weights)
        with jax.named_scope("hedgehog"):
            hedgehog_layer(layer)
        return carry

    lax.fori_loop(0, n_layers, layer_pair, 0)
    for i in range(seq // tb):
        out_copy(i).wait()


@functools.partial(jax.jit, static_argnames=("A_seg_len",))
def pallas_interleave_layers__memory_aug_recurrent_mem_tr__linear_kernel_hedgehog__prompt_kernel(
    A_x: jax.Array,
    A_mem0: jax.Array,
    A_Wq: jax.Array,
    A_Wk: jax.Array,
    A_Wv: jax.Array,
    A_Wo: jax.Array,
    A_seg_len: int,
    B_x: jax.Array,
    B_wqkv: jax.Array,
    B_w_phi: jax.Array,
    B_wo: jax.Array,
):
    del B_x
    batch, seq, dm = A_x.shape
    _, heads, dh = A_Wq.shape
    n_mem = A_mem0.shape[1]
    bh, bdh, _ = B_w_phi.shape
    seg = int(A_seg_len)
    assert batch == 1 and bdh == 20 and bh * bdh == dm and heads % 2 == 0
    assert (2 * dh) % 128 == 0 and n_mem % 8 == 0 and seg % 16 == 0 and 2 * (n_mem + seg) <= 128
    n_pairs, pw, hd = heads // 2, 2 * dh, heads * dh
    tb, unroll = 512, 2
    early_rows = seq // seg * EARLY_ROWS
    early_cols = 128 * sum(hi - lo for lo, hi in EARLY_TILES)

    def feature_major(w):
        return jnp.transpose(w, (1, 2, 0)).reshape(hd, dm)

    hbm = pl.BlockSpec(memory_space=pl.ANY)
    vmem = pl.BlockSpec(memory_space=pltpu.VMEM)
    out = pl.pallas_call(
        functools.partial(_kernel, seg=seg, dh=dh, n_layers=2, tb=tb, unroll=unroll),
        out_shape=jax.ShapeDtypeStruct((seq, dm), A_x.dtype),
        in_specs=[hbm, vmem, hbm, hbm, hbm, hbm, hbm, vmem, hbm],
        out_specs=hbm,
        scratch_shapes=[
            pltpu.VMEM((4, hd, dm), BF16),
            pltpu.VMEM((n_pairs, dm // 2, 3 * pw), U32),
            pltpu.VMEM((hd // 2, dm), U32),
            pltpu.VMEM((seq // seg, seg, dm), BF16),
            pltpu.VMEM((seq, dm), BF16),
            pltpu.VMEM((dm, 3 * dm), BF16),
            pltpu.VMEM((dm, dm), BF16),
            pltpu.VMEM((dm // 128, 8 * bdh, 128), BF16),
            pltpu.VMEM((2 * dm, dm), F32),
            pltpu.VMEM((dm, dm), F32),
            pltpu.VMEM((dm // 2, dm), U32),
            pltpu.VMEM((seq, dm), F32),
            pltpu.VMEM((seg, dm), F32),
            pltpu.VMEM((seq, dm), BF16),
            pltpu.VMEM((n_mem + seg, hd), F32),
            pltpu.VMEM((n_pairs, n_mem + 16, pw), F32),
            pltpu.VMEM((bh // 2, 2 * bdh, 4 * bdh), F32),
            pltpu.VMEM((bh // 2, 4 * bdh, 128), F32),
            pltpu.VMEM((seq // seg, EARLY_ROWS, dm), BF16),
            pltpu.VMEM((early_rows, dm), BF16),
            pltpu.VMEM((n_pairs, early_rows, early_cols), F32),
            pltpu.SemaphoreType.DMA((5, n_pairs)),
            pltpu.SemaphoreType.DMA((3,)),
            pltpu.SemaphoreType.DMA((seq // tb,)),
        ],
        compiler_params=pltpu.CompilerParams(vmem_limit_bytes=120 * 1024 * 1024, disable_bounds_checks=True),
        name="rmt_hedgehog",
    )(
        A_x.reshape(seq // seg, seg, dm),
        A_mem0.reshape(n_mem, dm),
        feature_major(A_Wq),
        feature_major(A_Wk),
        feature_major(A_Wv),
        A_Wo.reshape(hd, dm),
        B_wqkv,
        jnp.transpose(B_w_phi, (1, 2, 0)),
        B_wo,
    )
    return out.reshape(batch, seq, dm)
```

```python
import functools
import math

import jax
import jax.numpy as jnp
from jax import lax
import jax.experimental.pallas as pl
import jax.experimental.pallas.tpu as pltpu

F32 = jnp.float32
BF16 = jnp.bfloat16
U32 = jnp.uint32
I32 = jnp.int32

LN_EPS = 1e-5
DEN_EPS = 1e-6
LOG2E = math.log2(math.e)
EARLY_ROWS = 8
EARLY_TILES = ((0, 3), (4, 6), (7, 9))
STEP_REGULAR = ("00000000000111112222", range(0, 16), 9, "qosv", 256)
STEP_EARLY = ("00000000000111112222", range(0, 16), 9, "qosv", 256)


def _nn(a, b):
    return lax.dot_general(a, b, (((1,), (0,)), ((), ())), preferred_element_type=F32)


def _nt(a, b):
    return lax.dot_general(a, b, (((1,), (1,)), ((), ())), preferred_element_type=F32)


def _unpack(x):
    return pltpu.bitcast(x, BF16)


def _pack(x):
    return pltpu.bitcast(x, U32)


def _iota(shape, dim):
    return lax.broadcasted_iota(I32, shape, dim)


def _recip(x):
    r = pltpu.reciprocal(x, approx=True)
    return r * (2.0 - x * r)


def _layernorm(x):
    inv_n = 1.0 / x.shape[-1]
    m = jnp.sum(x, axis=-1, keepdims=True) * inv_n
    d = x - m
    v = jnp.sum(d * d, axis=-1, keepdims=True) * inv_n
    return d * lax.rsqrt(v + LN_EPS)


def _pair_blockdiag(x, dh):
    rows, width = x.shape
    top, bot = [], []
    zero = jnp.zeros((rows, 128), F32)
    for c in range(0, width, 128):
        t = x[:, c:c + 128]
        if c + 128 <= dh:
            top.append(t)
            bot.append(zero)
        elif c >= dh:
            top.append(zero)
            bot.append(t)
        else:
            first = _iota((rows, 128), 1) < dh - c
            top.append(jnp.where(first, t, 0.0))
            bot.append(jnp.where(first, 0.0, t))
    return jnp.concatenate(
        [jnp.concatenate(top, axis=1), jnp.concatenate(bot, axis=1)], axis=0
    ).astype(BF16)


def _pair_softmax(s, n_mem, scale):
    rows = s.shape[0]
    row = _iota(s.shape, 0)
    col = _iota(s.shape, 1)
    is_a = col < rows
    key = jnp.where(is_a, col, col - rows)
    s = jnp.where((row < n_mem) | (row >= key), s * scale, -1000000000.0)
    ma = jnp.max(jnp.where(is_a, s, -jnp.inf), axis=1, keepdims=True)
    mb = jnp.max(jnp.where(is_a, -jnp.inf, s), axis=1, keepdims=True)
    e = jnp.exp(s - jnp.where(is_a, ma, mb))
    la = jnp.sum(jnp.where(is_a, e, 0.0), axis=1, keepdims=True)
    lb = jnp.sum(jnp.where(is_a, 0.0, e), axis=1, keepdims=True)
    return e / jnp.where(is_a, la, lb)


def _over_features(x, op):
    r = functools.reduce(op, [x[i:i + 8] for i in range(0, x.shape[0], 8)])
    r = op(r, pltpu.roll(r, 4, 0))
    return op(r, pltpu.roll(r, 2, 0))


def _feature_map(p):
    def tile(r):
        return jnp.concatenate([r] * (p.shape[0] // 8), axis=0)

    ep = jnp.exp2(p - tile(_over_features(p, jnp.maximum)))
    en = jnp.exp2(tile(_over_features(p, jnp.minimum)) - p)
    return jnp.concatenate([e * tile(_recip(_over_features(e, jnp.add))) for e in (ep, en)], axis=0)


def _kernel(x_hbm, mem0_ref, wq_hbm, wk_hbm, wv_hbm, wo_hbm, bqkv_hbm, wphi_ref, bwo_hbm,
            out_hbm,
            stage, wqkv, wo, x_stage, out_stage, bqkv_stage, bwo_stage, fold, bw1, bwq, bwo,
            xres, xn_a, xn_b, o_scr, v_scr, kv_acc, z_acc, early_x, early_xn, early_qkv,
            w_sem, b_sem, out_sem,
            *, seg, dh, n_layers, tb, unroll):
    n_pairs = wqkv.shape[0]
    pw = 2 * dh
    half = pw // 2
    seq, dm = xres.shape
    n_mem = mem0_ref.shape[0]
    n_seg = seq // seg
    scale = dh ** -0.5
    bdh, _, bh = wphi_ref.shape
    n_grp = bh // 2
    gw = 2 * bdh

    x_chunk = n_seg // n_pairs

    def pair_rows(p):
        return pl.ds(pl.multiple_of(p * pw, pw), pw)

    def pair_copies(p):
        rows = pair_rows(p)
        segs = pl.ds(p * x_chunk, x_chunk)
        return [pltpu.make_async_copy(src.at[rows], stage.at[i, rows], w_sem.at[i, p])
                for i, src in enumerate((wq_hbm, wk_hbm, wv_hbm, wo_hbm))] + [
            pltpu.make_async_copy(x_hbm.at[segs], x_stage.at[segs], w_sem.at[4, p])]

    early_copy = pltpu.make_async_copy(
        x_hbm.at[:, pl.ds(seg - EARLY_ROWS, EARLY_ROWS)], early_x, b_sem.at[0])
    bqkv_copy = pltpu.make_async_copy(bqkv_hbm, bqkv_stage, b_sem.at[1])
    bwo_copy = pltpu.make_async_copy(bwo_hbm, bwo_stage, b_sem.at[2])
    early_copy.start()

    wphi = wphi_ref[...].astype(F32)
    wf = jnp.concatenate([wphi[d] for d in range(bdh)], axis=1)
    src = _iota((dm, 128), 0)
    natural = (src % bh) * bdh + src // bh
    first_grp = [c // gw for c in range(0, dm, 128)]
    r = _iota((4 * gw, 128), 0)
    lane = _iota((4 * gw, 128), 1)
    pick = ((r % gw) // 2 == lane).astype(BF16)
    head_start = ((r // gw) * 2 + r % 2) * bdh
    for j, g0 in enumerate(first_grp):
        wj = _nn(wf, (natural == _iota((dm, 128), 1) + j * 128).astype(BF16))
        wj = jnp.concatenate([wj, jnp.zeros((128 - bdh, 128), F32)], axis=0).astype(BF16)
        d = lane + (j * 128 - g0 * gw) - head_start
        fold[j] = jnp.where((d >= 0) & (d < bdh), _nn(pick, wj), 0.0).astype(BF16)

    for c in pair_copies(0):
        c.start()
    early_copy.wait()
    early_xn[...] = _layernorm(
        early_x[...].astype(F32).reshape(early_xn.shape)).astype(BF16)

    for c in pair_copies(1):
        c.start()

    def load_pair(p, carry):
        for c in pair_copies(p):
            c.wait()

        @pl.when(p + 2 < n_pairs)
        def _():
            for c in pair_copies(p + 2):
                c.start()

        col = 0
        for i, (lo, hi) in enumerate(EARLY_TILES):
            w = stage[i, pair_rows(p), :]
            early_qkv[p, :, col:col + (hi - lo) * 128] = _nt(
                early_xn[...], w[lo * 128 - i * pw:hi * 128 - i * pw])
            col += (hi - lo) * 128
            wqkv[p, :, i * pw:(i + 1) * pw] = _pack(w.T)
        wo[pl.ds(pl.multiple_of(p * half, half), half), :] = _pack(stage[3, pair_rows(p), :])
        wide = x_stage[pl.ds(p * x_chunk, x_chunk)].astype(F32).reshape(x_chunk * seg, dm)
        xres[pl.ds(pl.multiple_of(p * x_chunk * seg, x_chunk * seg), x_chunk * seg), :] = wide
        return carry

    with jax.named_scope("load"):
        lax.fori_loop(0, n_pairs, load_pair, 0)
    bqkv_copy.start()
    bwo_copy.start()

    def fold_phi(base):
        groups = [None] * n_grp
        for j, g0 in enumerate(first_grp):
            t = _nt(fold[j], bqkv_stage[:, base + j * 128:base + (j + 1) * 128]) * LOG2E
            for i in range(4):
                part = t[i * gw:(i + 1) * gw]
                groups[g0 + i] = part if groups[g0 + i] is None else groups[g0 + i] + part
        return groups

    def hedgehog_weights():
        bqkv_copy.wait()
        bwo_copy.wait()
        wvt = bqkv_stage[:, 2 * dm:].astype(F32).T
        bwq[...] = _pack(jnp.concatenate(fold_phi(0), axis=0).astype(BF16))
        bw1[...] = _pack(jnp.concatenate(
            [t for g, wpk in enumerate(fold_phi(dm)) for t in (wpk, wvt[g * gw:(g + 1) * gw])],
            axis=0).astype(BF16))
        bwo[...] = _pack(bwo_stage[...])

    def seg_rows(s):
        return pl.ds(pl.multiple_of(s * seg, seg), seg)

    def rmt_step(s, mem, early):
        plan, vpu_pairs, norm_pair, order, ks = STEP_EARLY if early else STEP_REGULAR
        h = jnp.concatenate([mem, xn_a[...]], axis=0)
        h_short = h[:-EARLY_ROWS].astype(BF16)
        early_rows = pl.ds(pl.multiple_of(s * EARLY_ROWS, EARLY_ROWS), EARLY_ROWS)
        xn_next = _layernorm(xres[seg_rows(jnp.minimum(s + 1, n_seg - 1)), :])
        prev = seg_rows(jnp.maximum(s - 1, 0))
        xn_b[prev, :] = _layernorm(xres[prev, :]).astype(BF16)
        pending = {norm_pair: [xn_b[seg_rows(jnp.maximum(s, 1) - 1), :128].astype(F32)[:8]]}

        def project(p):
            spans, end = [], 0
            for lo, hi in EARLY_TILES if early else ():
                spans += [(h, end, lo)] * (end < lo) + [(h_short, lo, hi)]
                end = hi
            spans += [(h, end, 3 * pw // 128)] * (end < 3 * pw // 128)
            spans = [(x, slice(lo * 128, hi * 128)) for x, lo, hi in spans]
            if p > 0:
                parts = [_nn(x, _unpack(wqkv[p, :, cols])) for x, cols in spans]
            else:
                parts = [_nn(x[:, :ks], _unpack(wqkv[p, :ks // 2, cols])) for x, cols in spans]
                parts = [_nn(x[:, ks:], _unpack(wqkv[p, ks // 2:, cols])) + start
                         for start, (x, cols) in zip(parts, spans)]
            col = 0
            for i, t in enumerate(parts):
                if t.shape[0] < h.shape[0]:
                    known = early_qkv[p, early_rows, col:col + t.shape[1]]
                    parts[i] = jnp.concatenate([t, known], axis=0)
                    col += t.shape[1]
            return jnp.concatenate(parts, axis=1)

        def weighted_values(p, prob, v):
            head = prob[:n_mem]
            if p in pending:
                work = functools.reduce(jnp.add, pending[p])[:, :prob.shape[1]]
                head = jnp.where(s < 0, work, head)
            if p not in vpu_pairs:
                return _nn(jnp.concatenate([head, prob[n_mem:]], axis=0), _pair_blockdiag(v, dh))
            seen = n_mem + 8
            o = _nn(jnp.concatenate([head, prob[seen:]], axis=0), _pair_blockdiag(v, dh))
            v_scr[p, :seen, :] = v[:seen]
            v_scr[p, seen:seen + 1, :] = jnp.sum(v[seen:], axis=0, keepdims=True)
            first = jnp.concatenate(
                [prob[n_mem:seen], jnp.zeros((8, 128 - prob.shape[1]), F32)], axis=1)
            lane = _iota(first.shape, 1)
            tiles = [None] * (pw // 128)
            for k in range(seen + 1):
                wa, wb = (jnp.sum(jnp.where(lane == col, first, 0.0), axis=1, keepdims=True)
                          for col in (k, prob.shape[0] + k))
                for t, c in enumerate(range(0, pw, 128)):
                    w = wa if c + 128 <= dh else wb if c >= dh else jnp.where(lane < dh - c, wa, wb)
                    term = w * jnp.broadcast_to(v_scr[p, k:k + 1, c:c + 128], (8, 128))
                    tiles[t] = term if k == 0 else tiles[t] + term
            pending.setdefault(p + 1, []).extend(tiles)
            return jnp.concatenate([o[:n_mem], jnp.concatenate(tiles, axis=1), o[n_mem:]], axis=0)

        def out_proj(acc, lo, hi, cols=slice(None)):
            t = _nn(o_scr[:, lo * pw:hi * pw], _unpack(wo[lo * half:hi * half, cols]))
            return t if acc is None else t + acc[:, cols]

        qkv, prob = {}, {}
        acc, done = None, 0
        for p in range(len(plan)):
            r = p - (len(plan) - n_pairs)
            for what in order:
                if what == "q" and p < n_pairs:
                    qkv[p] = project(p)
                if what == "o" and plan[p] != "0":
                    acc = out_proj(acc, done, done + int(plan[p]))
                    done += int(plan[p])
                if what == "s" and 0 <= p - 1 < n_pairs:
                    t = qkv[p - 1]
                    scores = _nt(t[:, :pw], _pair_blockdiag(t[:, pw:2 * pw], dh))
                    prob[p - 1] = _pair_softmax(scores, n_mem, scale)
                if what == "v" and r >= 0:
                    o_scr[:, r * pw:(r + 1) * pw] = weighted_values(r, prob[r], qkv[r][:, 2 * pw:])
        acc = out_proj(acc, done, done + 1)
        acc = jnp.concatenate(
            [out_proj(acc, done + 1, n_pairs, cols) for cols in (slice(0, ks), slice(ks, dm))], axis=1)
        xn_a[...] = xn_next
        rows = seg_rows(s)
        xres[rows, :] = xres[rows, :] + acc[n_mem:]
        return acc[:n_mem]

    def rmt_steps(early):
        def body(i, mem):
            for u in range(unroll):
                mem = rmt_step(i * unroll + u, mem, early)
            return mem

        lax.fori_loop(0, n_seg // unroll, body, mem0_ref[...].astype(F32))

    def rmt_layer(layer):
        xn_a[...] = _layernorm(xres[0:seg, :])
        pl.when(layer == 0)(functools.partial(rmt_steps, True))
        pl.when(layer > 0)(functools.partial(rmt_steps, False))
        last = slice(seq - seg, seq)
        xn_b[last, :] = _layernorm(xres[last, :]).astype(BF16)

    chunk = 4
    n_chunk = n_grp // chunk

    def blk_rows(i):
        return pl.ds(pl.multiple_of(i * tb, tb), tb)

    def kv_block(i, carry):
        xn = xn_b[blk_rows(i), :]
        proj = {}
        for c in range(n_chunk + 1):
            if c < n_chunk:
                proj[c] = _nt(_unpack(bw1[c * chunk * gw:(c + 1) * chunk * gw, :]), xn)
            if c >= 1:
                t = proj[c - 1]
                for j in range(chunk):
                    g = (c - 1) * chunk + j
                    phi = _feature_map(t[2 * j * gw:(2 * j + 1) * gw])
                    kv_acc[g] += _nt(t[(2 * j + 1) * gw:(2 * j + 2) * gw], phi.astype(BF16))
                    z_acc[g] += functools.reduce(jnp.add, [phi[:, i:i + 128] for i in range(0, tb, 128)])
        return carry

    def out_copy(i):
        return pltpu.make_async_copy(out_stage.at[blk_rows(i)], out_hbm.at[blk_rows(i)], out_sem.at[i])

    def out_block(i, layer):
        rows = blk_rows(i)
        xn = xn_b[rows, :]
        sublane = _iota((8, tb), 0)
        proj, outs = {}, []

        def out_proj(y, lo, hi):
            o = jnp.concatenate(outs, axis=0)[lo:hi].astype(BF16).T
            return _nn(o, _unpack(bwo[lo // 2:hi // 2, :])) + y

        y = xres[rows, :]
        for c in range(n_chunk + 1):
            if c < n_chunk:
                proj[c] = _nt(_unpack(bwq[c * chunk * bdh:(c + 1) * chunk * bdh, :]), xn)
            else:
                y = out_proj(y, 0, 256)
            if c >= 1:
                for j in range(chunk):
                    g = (c - 1) * chunk + j
                    phi = _feature_map(proj[c - 1][j * gw:(j + 1) * gw])
                    z = jnp.concatenate([z_acc[g]] * (tb // 128), axis=1)
                    inv = _recip(_over_features(phi * z, jnp.add) + DEN_EPS)
                    swapped = pltpu.roll(inv, 1, 0)
                    inv_a = jnp.where(sublane % 2 == 0, inv, swapped)
                    inv_b = jnp.where(sublane % 2 == 0, swapped, inv)
                    inv_ab = jnp.where(sublane < bdh % 8, inv_a, inv_b)
                    outs.append(_nn(kv_acc[g], phi.astype(BF16))
                                * jnp.concatenate([inv_a, inv_a, inv_ab, inv_b, inv_b], axis=0))
        y = out_proj(out_proj(y, 256, 384), 384, dm)
        xres[rows, :] = y
        out_stage[rows, :] = y.astype(BF16)

        @pl.when(layer == n_layers - 1)
        def _():
            out_copy(i).start()

        return layer

    def hedgehog_layer(layer):
        kv_acc[...] = jnp.zeros(kv_acc.shape, F32)
        z_acc[...] = jnp.zeros(z_acc.shape, F32)
        lax.fori_loop(0, seq // tb, kv_block, 0)
        shape = kv_acc.shape[1:]
        same_head = _iota(shape, 0) // bdh == _iota(shape, 1) % 2
        for g in range(n_grp):
            kv_acc[g] = jnp.where(same_head, kv_acc[g], 0.0)
            z_acc[g] = jnp.broadcast_to(jnp.sum(z_acc[g], axis=1, keepdims=True), z_acc.shape[1:])
        lax.fori_loop(0, seq // tb, out_block, layer)

    def layer_pair(layer, carry):
        with jax.named_scope("rmt"):
            rmt_layer(layer)
        pl.when(layer == 0)(hedgehog_weights)
        with jax.named_scope("hedgehog"):
            hedgehog_layer(layer)
        return carry

    lax.fori_loop(0, n_layers, layer_pair, 0)
    for i in range(seq // tb):
        out_copy(i).wait()


@functools.partial(jax.jit, static_argnames=("A_seg_len",))
def pallas_interleave_layers__memory_aug_recurrent_mem_tr__linear_kernel_hedgehog__prompt_kernel(
    A_x: jax.Array,
    A_mem0: jax.Array,
    A_Wq: jax.Array,
    A_Wk: jax.Array,
    A_Wv: jax.Array,
    A_Wo: jax.Array,
    A_seg_len: int,
    B_x: jax.Array,
    B_wqkv: jax.Array,
    B_w_phi: jax.Array,
    B_wo: jax.Array,
):
    del B_x
    batch, seq, dm = A_x.shape
    _, heads, dh = A_Wq.shape
    n_mem = A_mem0.shape[1]
    bh, bdh, _ = B_w_phi.shape
    seg = int(A_seg_len)
    assert batch == 1 and bdh == 20 and bh * bdh == dm and heads % 2 == 0
    assert (2 * dh) % 128 == 0 and n_mem % 8 == 0 and seg % 16 == 0 and 2 * (n_mem + seg) <= 128
    n_pairs, pw, hd = heads // 2, 2 * dh, heads * dh
    tb, unroll = 512, 2
    early_rows = seq // seg * EARLY_ROWS
    early_cols = 128 * sum(hi - lo for lo, hi in EARLY_TILES)

    def feature_major(w):
        return jnp.transpose(w, (1, 2, 0)).reshape(hd, dm)

    hbm = pl.BlockSpec(memory_space=pl.ANY)
    vmem = pl.BlockSpec(memory_space=pltpu.VMEM)
    out = pl.pallas_call(
        functools.partial(_kernel, seg=seg, dh=dh, n_layers=2, tb=tb, unroll=unroll),
        out_shape=jax.ShapeDtypeStruct((seq, dm), A_x.dtype),
        in_specs=[hbm, vmem, hbm, hbm, hbm, hbm, hbm, vmem, hbm],
        out_specs=hbm,
        scratch_shapes=[
            pltpu.VMEM((4, hd, dm), BF16),
            pltpu.VMEM((n_pairs, dm // 2, 3 * pw), U32),
            pltpu.VMEM((hd // 2, dm), U32),
            pltpu.VMEM((seq // seg, seg, dm), BF16),
            pltpu.VMEM((seq, dm), BF16),
            pltpu.VMEM((dm, 3 * dm), BF16),
            pltpu.VMEM((dm, dm), BF16),
            pltpu.VMEM((dm // 128, 8 * bdh, 128), BF16),
            pltpu.VMEM((dm, dm), U32),
            pltpu.VMEM((dm // 2, dm), U32),
            pltpu.VMEM((dm // 2, dm), U32),
            pltpu.VMEM((seq, dm), F32),
            pltpu.VMEM((seg, dm), F32),
            pltpu.VMEM((seq, dm), BF16),
            pltpu.VMEM((n_mem + seg, hd), F32),
            pltpu.VMEM((n_pairs, n_mem + 16, pw), F32),
            pltpu.VMEM((bh // 2, 2 * bdh, 4 * bdh), F32),
            pltpu.VMEM((bh // 2, 4 * bdh, 128), F32),
            pltpu.VMEM((seq // seg, EARLY_ROWS, dm), BF16),
            pltpu.VMEM((early_rows, dm), BF16),
            pltpu.VMEM((n_pairs, early_rows, early_cols), F32),
            pltpu.SemaphoreType.DMA((5, n_pairs)),
            pltpu.SemaphoreType.DMA((3,)),
            pltpu.SemaphoreType.DMA((seq // tb,)),
        ],
        compiler_params=pltpu.CompilerParams(vmem_limit_bytes=120 * 1024 * 1024, disable_bounds_checks=True),
        name="rmt_hedgehog",
    )(
        A_x.reshape(seq // seg, seg, dm),
        A_mem0.reshape(n_mem, dm),
        feature_major(A_Wq),
        feature_major(A_Wk),
        feature_major(A_Wv),
        A_Wo.reshape(hd, dm),
        B_wqkv,
        jnp.transpose(B_w_phi, (1, 2, 0)),
        B_wo,
    )
    return out.reshape(batch, seq, dm)
```

```python
import functools
import math

import jax
import jax.numpy as jnp
from jax import lax
import jax.experimental.pallas as pl
import jax.experimental.pallas.tpu as pltpu

F32 = jnp.float32
BF16 = jnp.bfloat16
U32 = jnp.uint32
I32 = jnp.int32

LN_EPS = 1e-5
DEN_EPS = 1e-6
LOG2E = math.log2(math.e)
EARLY_ROWS = 8
EARLY_TILES = ((0, 3), (4, 6), (7, 9))
STEP_REGULAR = ("00000000000111111223", range(0, 16), 1, "qosv", 256)
STEP_EARLY = ("00000000001111112212", range(0, 16), 9, "qosv", 256)


def _nn(a, b):
    return lax.dot_general(a, b, (((1,), (0,)), ((), ())), preferred_element_type=F32)


def _nt(a, b):
    return lax.dot_general(a, b, (((1,), (1,)), ((), ())), preferred_element_type=F32)


def _unpack(x):
    return pltpu.bitcast(x, BF16)


def _pack(x):
    return pltpu.bitcast(x, U32)


def _iota(shape, dim):
    return lax.broadcasted_iota(I32, shape, dim)


def _recip(x):
    r = pltpu.reciprocal(x, approx=True)
    return r * (2.0 - x * r)


def _layernorm(x):
    inv_n = 1.0 / x.shape[-1]
    m = jnp.sum(x, axis=-1, keepdims=True) * inv_n
    d = x - m
    v = jnp.sum(d * d, axis=-1, keepdims=True) * inv_n
    return d * lax.rsqrt(v + LN_EPS)


def _pair_blockdiag(x, dh):
    rows, width = x.shape
    top, bot = [], []
    zero = jnp.zeros((rows, 128), F32)
    for c in range(0, width, 128):
        t = x[:, c:c + 128]
        if c + 128 <= dh:
            top.append(t)
            bot.append(zero)
        elif c >= dh:
            top.append(zero)
            bot.append(t)
        else:
            first = _iota((rows, 128), 1) < dh - c
            top.append(jnp.where(first, t, 0.0))
            bot.append(jnp.where(first, 0.0, t))
    return jnp.concatenate(
        [jnp.concatenate(top, axis=1), jnp.concatenate(bot, axis=1)], axis=0
    ).astype(BF16)


def _pair_softmax(s, n_mem, scale):
    rows = s.shape[0]
    row = _iota(s.shape, 0)
    col = _iota(s.shape, 1)
    is_a = col < rows
    key = jnp.where(is_a, col, col - rows)
    s = jnp.where((row < n_mem) | (row >= key), s * scale, -1000000000.0)
    ma = jnp.max(jnp.where(is_a, s, -jnp.inf), axis=1, keepdims=True)
    mb = jnp.max(jnp.where(is_a, -jnp.inf, s), axis=1, keepdims=True)
    e = jnp.exp(s - jnp.where(is_a, ma, mb))
    la = jnp.sum(jnp.where(is_a, e, 0.0), axis=1, keepdims=True)
    lb = jnp.sum(jnp.where(is_a, 0.0, e), axis=1, keepdims=True)
    return e / jnp.where(is_a, la, lb)


def _over_features(x, op):
    r = functools.reduce(op, [x[i:i + 8] for i in range(0, x.shape[0], 8)])
    r = op(r, pltpu.roll(r, 4, 0))
    return op(r, pltpu.roll(r, 2, 0))


def _feature_map(p):
    def tile(r):
        return jnp.concatenate([r] * (p.shape[0] // 8), axis=0)

    ep = jnp.exp2(p - tile(_over_features(p, jnp.maximum)))
    en = jnp.exp2(tile(_over_features(p, jnp.minimum)) - p)
    return jnp.concatenate([e * tile(_recip(_over_features(e, jnp.add))) for e in (ep, en)], axis=0)


def _kernel(x_hbm, mem0_ref, wq_hbm, wk_hbm, wv_hbm, wo_hbm, bqkv_hbm, wphi_ref, bwo_hbm,
            out_hbm,
            stage, wqkv, wo, x_stage, out_stage, bqkv_stage, bwo_stage, fold, bw1, bwq, bwo,
            xres, xn_a, xn_b, o_scr, v_scr, kv_acc, z_acc, early_x, early_xn, early_qkv,
            w_sem, b_sem, out_sem,
            *, seg, dh, n_layers, tb, unroll):
    n_pairs = wqkv.shape[0]
    pw = 2 * dh
    half = pw // 2
    seq, dm = xres.shape
    n_mem = mem0_ref.shape[0]
    n_seg = seq // seg
    scale = dh ** -0.5
    bdh, _, bh = wphi_ref.shape
    n_grp = bh // 2
    gw = 2 * bdh

    x_chunk = n_seg // n_pairs

    def pair_rows(p):
        return pl.ds(pl.multiple_of(p * pw, pw), pw)

    def weight_copy(i, p):
        src = (wq_hbm, wk_hbm, wv_hbm, wo_hbm)[i]
        return pltpu.make_async_copy(src.at[pair_rows(p)], stage.at[i, pair_rows(p)], w_sem.at[i, p])

    def pair_copies(p, first=False):
        segs = pl.ds(p * x_chunk, x_chunk)
        return [weight_copy(i, p) for i in range(3)] + [
            pltpu.make_async_copy(x_hbm.at[segs], x_stage.at[segs], w_sem.at[4, p])
        ] + ([] if first else [weight_copy(3, p - 1)])

    def pack_wo(i, p):
        wo[pl.ds(pl.multiple_of(p * half, half), half), :] = _pack(stage[i, pair_rows(p), :])

    early_copy = pltpu.make_async_copy(
        x_hbm.at[:, pl.ds(seg - EARLY_ROWS, EARLY_ROWS)], early_x, b_sem.at[0])
    bqkv_copy = pltpu.make_async_copy(bqkv_hbm, bqkv_stage, b_sem.at[1])
    bwo_copy = pltpu.make_async_copy(bwo_hbm, bwo_stage, b_sem.at[2])
    early_copy.start()

    wphi = wphi_ref[...].astype(F32)
    wf = jnp.concatenate([wphi[d] for d in range(bdh)], axis=1)
    src = _iota((dm, 128), 0)
    natural = (src % bh) * bdh + src // bh
    first_grp = [c // gw for c in range(0, dm, 128)]
    r = _iota((4 * gw, 128), 0)
    lane = _iota((4 * gw, 128), 1)
    pick = ((r % gw) // 2 == lane).astype(BF16)
    head_start = ((r // gw) * 2 + r % 2) * bdh
    for j, g0 in enumerate(first_grp):
        wj = _nn(wf, (natural == _iota((dm, 128), 1) + j * 128).astype(BF16))
        wj = jnp.concatenate([wj, jnp.zeros((128 - bdh, 128), F32)], axis=0).astype(BF16)
        d = lane + (j * 128 - g0 * gw) - head_start
        fold[j] = jnp.where((d >= 0) & (d < bdh), _nn(pick, wj), 0.0).astype(BF16)

    for c in pair_copies(0, first=True):
        c.start()
    early_copy.wait()
    early_xn[...] = _layernorm(
        early_x[...].astype(F32).reshape(early_xn.shape)).astype(BF16)

    for c in pair_copies(1):
        c.start()

    def load_pair(p, carry):
        for c in pair_copies(p, first=True):
            c.wait()
        pl.when(p > 0)(lambda: weight_copy(3, p - 1).wait())
        pl.when(p == n_pairs - 2)(lambda: weight_copy(3, n_pairs - 1).start())

        @pl.when(p + 2 < n_pairs)
        def _():
            for c in pair_copies(p + 2):
                c.start()

        col = 0
        for i, (lo, hi) in enumerate(EARLY_TILES):
            w = stage[i, pair_rows(p), :]
            early_qkv[p, :, col:col + (hi - lo) * 128] = _nt(
                early_xn[...], w[lo * 128 - i * pw:hi * 128 - i * pw])
            col += (hi - lo) * 128
            wqkv[p, :, i * pw:(i + 1) * pw] = _pack(w.T)
        pack_wo(jnp.where(p > 0, 3, 0), jnp.maximum(p - 1, 0))
        wide = x_stage[pl.ds(p * x_chunk, x_chunk)].astype(F32).reshape(x_chunk * seg, dm)
        xres[pl.ds(pl.multiple_of(p * x_chunk * seg, x_chunk * seg), x_chunk * seg), :] = wide
        return carry

    with jax.named_scope("load"):
        lax.fori_loop(0, n_pairs, load_pair, 0)
    weight_copy(3, n_pairs - 1).wait()
    pack_wo(3, n_pairs - 1)
    bqkv_copy.start()
    bwo_copy.start()

    def fold_phi(base):
        groups = [None] * n_grp
        for j, g0 in enumerate(first_grp):
            t = _nt(fold[j], bqkv_stage[:, base + j * 128:base + (j + 1) * 128]) * LOG2E
            for i in range(4):
                part = t[i * gw:(i + 1) * gw]
                groups[g0 + i] = part if groups[g0 + i] is None else groups[g0 + i] + part
        return groups

    def hedgehog_weights():
        bqkv_copy.wait()
        bwo_copy.wait()
        wvt = bqkv_stage[:, 2 * dm:].astype(F32).T
        bwq[...] = _pack(jnp.concatenate(fold_phi(0), axis=0).astype(BF16))
        bw1[...] = _pack(jnp.concatenate(
            [t for g, wpk in enumerate(fold_phi(dm)) for t in (wpk, wvt[g * gw:(g + 1) * gw])],
            axis=0).astype(BF16))
        bwo[...] = _pack(bwo_stage[...])

    def seg_rows(s):
        return pl.ds(pl.multiple_of(s * seg, seg), seg)

    def rmt_step(s, mem, early):
        plan, vpu_pairs, norm_pair, order, ks = STEP_EARLY if early else STEP_REGULAR
        h = jnp.concatenate([mem, xn_a[...]], axis=0)
        h_short = h[:-EARLY_ROWS].astype(BF16)
        early_rows = pl.ds(pl.multiple_of(s * EARLY_ROWS, EARLY_ROWS), EARLY_ROWS)
        xn_next = _layernorm(xres[seg_rows(jnp.minimum(s + 1, n_seg - 1)), :])
        prev = seg_rows(jnp.maximum(s - 1, 0))
        xn_b[prev, :] = _layernorm(xres[prev, :]).astype(BF16)
        pending = {norm_pair: [xn_b[seg_rows(jnp.maximum(s, 1) - 1), :128].astype(F32)[:8]]}

        def project(p):
            spans, end = [], 0
            for lo, hi in EARLY_TILES if early else ():
                spans += [(h, end, lo)] * (end < lo) + [(h_short, lo, hi)]
                end = hi
            spans += [(h, end, 3 * pw // 128)] * (end < 3 * pw // 128)
            spans = [(x, slice(lo * 128, hi * 128)) for x, lo, hi in spans]
            if p > 0:
                parts = [_nn(x, _unpack(wqkv[p, :, cols])) for x, cols in spans]
            else:
                parts = [_nn(x[:, :ks], _unpack(wqkv[p, :ks // 2, cols])) for x, cols in spans]
                parts = [_nn(x[:, ks:], _unpack(wqkv[p, ks // 2:, cols])) + start
                         for start, (x, cols) in zip(parts, spans)]
            col = 0
            for i, t in enumerate(parts):
                if t.shape[0] < h.shape[0]:
                    known = early_qkv[p, early_rows, col:col + t.shape[1]]
                    parts[i] = jnp.concatenate([t, known], axis=0)
                    col += t.shape[1]
            return jnp.concatenate(parts, axis=1)

        def weighted_values(p, prob, v):
            head = prob[:n_mem]
            if p in pending:
                work = functools.reduce(jnp.add, pending[p])[:, :prob.shape[1]]
                head = jnp.where(s < 0, work, head)
            if p not in vpu_pairs:
                return _nn(jnp.concatenate([head, prob[n_mem:]], axis=0), _pair_blockdiag(v, dh))
            seen = n_mem + 8
            o = _nn(jnp.concatenate([head, prob[seen:]], axis=0), _pair_blockdiag(v, dh))
            v_scr[p, :seen, :] = v[:seen]
            v_scr[p, seen:seen + 1, :] = jnp.sum(v[seen:], axis=0, keepdims=True)
            first = jnp.concatenate(
                [prob[n_mem:seen], jnp.zeros((8, 128 - prob.shape[1]), F32)], axis=1)
            lane = _iota(first.shape, 1)
            tiles = [None] * (pw // 128)
            for k in range(seen + 1):
                wa, wb = (jnp.sum(jnp.where(lane == col, first, 0.0), axis=1, keepdims=True)
                          for col in (k, prob.shape[0] + k))
                for t, c in enumerate(range(0, pw, 128)):
                    w = wa if c + 128 <= dh else wb if c >= dh else jnp.where(lane < dh - c, wa, wb)
                    term = w * jnp.broadcast_to(v_scr[p, k:k + 1, c:c + 128], (8, 128))
                    tiles[t] = term if k == 0 else tiles[t] + term
            pending.setdefault(p + 1, []).extend(tiles)
            return jnp.concatenate([o[:n_mem], jnp.concatenate(tiles, axis=1), o[n_mem:]], axis=0)

        def out_proj(acc, lo, hi, cols=slice(None)):
            t = _nn(o_scr[:, lo * pw:hi * pw], _unpack(wo[lo * half:hi * half, cols]))
            return t if acc is None else t + acc[:, cols]

        qkv, prob = {}, {}
        acc, done = None, 0
        for p in range(len(plan)):
            r = p - (len(plan) - n_pairs)
            for what in order:
                if what == "q" and p < n_pairs:
                    qkv[p] = project(p)
                if what == "o" and plan[p] != "0":
                    acc = out_proj(acc, done, done + int(plan[p]))
                    done += int(plan[p])
                if what == "s" and 0 <= p - 1 < n_pairs:
                    t = qkv[p - 1]
                    scores = _nt(t[:, :pw], _pair_blockdiag(t[:, pw:2 * pw], dh))
                    prob[p - 1] = _pair_softmax(scores, n_mem, scale)
                if what == "v" and r >= 0:
                    o_scr[:, r * pw:(r + 1) * pw] = weighted_values(r, prob[r], qkv[r][:, 2 * pw:])
        acc = out_proj(acc, done, done + 1)
        acc = jnp.concatenate(
            [out_proj(acc, done + 1, n_pairs, cols) for cols in (slice(0, ks), slice(ks, dm))], axis=1)
        xn_a[...] = xn_next
        rows = seg_rows(s)
        xres[rows, :] = xres[rows, :] + acc[n_mem:]
        return acc[:n_mem]

    def rmt_steps(early):
        def body(i, mem):
            for u in range(unroll):
                mem = rmt_step(i * unroll + u, mem, early)
            return mem

        lax.fori_loop(0, n_seg // unroll, body, mem0_ref[...].astype(F32))

    def rmt_layer(layer):
        xn_a[...] = _layernorm(xres[0:seg, :])
        pl.when(layer == 0)(functools.partial(rmt_steps, True))
        pl.when(layer > 0)(functools.partial(rmt_steps, False))
        last = slice(seq - seg, seq)
        xn_b[last, :] = _layernorm(xres[last, :]).astype(BF16)

    chunk = 4
    n_chunk = n_grp // chunk

    def blk_rows(i):
        return pl.ds(pl.multiple_of(i * tb, tb), tb)

    def kv_block(i, carry):
        xn = xn_b[blk_rows(i), :]
        proj = {}
        for c in range(n_chunk + 1):
            if c < n_chunk:
                proj[c] = _nt(_unpack(bw1[c * chunk * gw:(c + 1) * chunk * gw, :]), xn)
            if c >= 1:
                t = proj[c - 1]
                for j in range(chunk):
                    g = (c - 1) * chunk + j
                    phi = _feature_map(t[2 * j * gw:(2 * j + 1) * gw])
                    kv_acc[g] += _nt(t[(2 * j + 1) * gw:(2 * j + 2) * gw], phi.astype(BF16))
                    z_acc[g] += functools.reduce(jnp.add, [phi[:, i:i + 128] for i in range(0, tb, 128)])
        return carry

    def out_copy(i):
        return pltpu.make_async_copy(out_stage.at[blk_rows(i)], out_hbm.at[blk_rows(i)], out_sem.at[i])

    def out_block(i, layer):
        rows = blk_rows(i)
        xn = xn_b[rows, :]
        sublane = _iota((8, tb), 0)
        proj, outs = {}, []

        def out_proj(y, lo, hi):
            o = jnp.concatenate(outs, axis=0)[lo:hi].astype(BF16).T
            return _nn(o, _unpack(bwo[lo // 2:hi // 2, :])) + y

        y = xres[rows, :]
        for c in range(n_chunk + 1):
            if c < n_chunk:
                proj[c] = _nt(_unpack(bwq[c * chunk * bdh:(c + 1) * chunk * bdh, :]), xn)
            else:
                y = out_proj(y, 0, 256)
            if c >= 1:
                for j in range(chunk):
                    g = (c - 1) * chunk + j
                    phi = _feature_map(proj[c - 1][j * gw:(j + 1) * gw])
                    z = jnp.concatenate([z_acc[g]] * (tb // 128), axis=1)
                    inv = _recip(_over_features(phi * z, jnp.add) + DEN_EPS)
                    swapped = pltpu.roll(inv, 1, 0)
                    inv_a = jnp.where(sublane % 2 == 0, inv, swapped)
                    inv_b = jnp.where(sublane % 2 == 0, swapped, inv)
                    inv_ab = jnp.where(sublane < bdh % 8, inv_a, inv_b)
                    outs.append(_nn(kv_acc[g], phi.astype(BF16))
                                * jnp.concatenate([inv_a, inv_a, inv_ab, inv_b, inv_b], axis=0))
        y = out_proj(out_proj(y, 256, 384), 384, dm)
        xres[rows, :] = y
        out_stage[rows, :] = y.astype(BF16)

        @pl.when(layer == n_layers - 1)
        def _():
            out_copy(i).start()

        return layer

    def hedgehog_layer(layer):
        kv_acc[...] = jnp.zeros(kv_acc.shape, F32)
        z_acc[...] = jnp.zeros(z_acc.shape, F32)
        lax.fori_loop(0, seq // tb, kv_block, 0)
        shape = kv_acc.shape[1:]
        same_head = _iota(shape, 0) // bdh == _iota(shape, 1) % 2
        for g in range(n_grp):
            kv_acc[g] = jnp.where(same_head, kv_acc[g], 0.0)
            z_acc[g] = jnp.broadcast_to(jnp.sum(z_acc[g], axis=1, keepdims=True), z_acc.shape[1:])
        lax.fori_loop(0, seq // tb, out_block, layer)

    def layer_pair(layer, carry):
        with jax.named_scope("rmt"):
            rmt_layer(layer)
        pl.when(layer == 0)(hedgehog_weights)
        with jax.named_scope("hedgehog"):
            hedgehog_layer(layer)
        return carry

    lax.fori_loop(0, n_layers, layer_pair, 0)
    for i in range(seq // tb):
        out_copy(i).wait()


@functools.partial(jax.jit, static_argnames=("A_seg_len",))
def pallas_interleave_layers__memory_aug_recurrent_mem_tr__linear_kernel_hedgehog__prompt_kernel(
    A_x: jax.Array,
    A_mem0: jax.Array,
    A_Wq: jax.Array,
    A_Wk: jax.Array,
    A_Wv: jax.Array,
    A_Wo: jax.Array,
    A_seg_len: int,
    B_x: jax.Array,
    B_wqkv: jax.Array,
    B_w_phi: jax.Array,
    B_wo: jax.Array,
):
    del B_x
    batch, seq, dm = A_x.shape
    _, heads, dh = A_Wq.shape
    n_mem = A_mem0.shape[1]
    bh, bdh, _ = B_w_phi.shape
    seg = int(A_seg_len)
    assert batch == 1 and bdh == 20 and bh * bdh == dm and heads % 2 == 0
    assert (2 * dh) % 128 == 0 and n_mem % 8 == 0 and seg % 16 == 0 and 2 * (n_mem + seg) <= 128
    n_pairs, pw, hd = heads // 2, 2 * dh, heads * dh
    tb, unroll = 512, 2
    early_rows = seq // seg * EARLY_ROWS
    early_cols = 128 * sum(hi - lo for lo, hi in EARLY_TILES)

    def feature_major(w):
        return jnp.transpose(w, (1, 2, 0)).reshape(hd, dm)

    hbm = pl.BlockSpec(memory_space=pl.ANY)
    vmem = pl.BlockSpec(memory_space=pltpu.VMEM)
    out = pl.pallas_call(
        functools.partial(_kernel, seg=seg, dh=dh, n_layers=2, tb=tb, unroll=unroll),
        out_shape=jax.ShapeDtypeStruct((seq, dm), A_x.dtype),
        in_specs=[hbm, vmem, hbm, hbm, hbm, hbm, hbm, vmem, hbm],
        out_specs=hbm,
        scratch_shapes=[
            pltpu.VMEM((4, hd, dm), BF16),
            pltpu.VMEM((n_pairs, dm // 2, 3 * pw), U32),
            pltpu.VMEM((hd // 2, dm), U32),
            pltpu.VMEM((seq // seg, seg, dm), BF16),
            pltpu.VMEM((seq, dm), BF16),
            pltpu.VMEM((dm, 3 * dm), BF16),
            pltpu.VMEM((dm, dm), BF16),
            pltpu.VMEM((dm // 128, 8 * bdh, 128), BF16),
            pltpu.VMEM((dm, dm), U32),
            pltpu.VMEM((dm // 2, dm), U32),
            pltpu.VMEM((dm // 2, dm), U32),
            pltpu.VMEM((seq, dm), F32),
            pltpu.VMEM((seg, dm), F32),
            pltpu.VMEM((seq, dm), BF16),
            pltpu.VMEM((n_mem + seg, hd), F32),
            pltpu.VMEM((n_pairs, n_mem + 16, pw), F32),
            pltpu.VMEM((bh // 2, 2 * bdh, 4 * bdh), F32),
            pltpu.VMEM((bh // 2, 4 * bdh, 128), F32),
            pltpu.VMEM((seq // seg, EARLY_ROWS, dm), BF16),
            pltpu.VMEM((early_rows, dm), BF16),
            pltpu.VMEM((n_pairs, early_rows, early_cols), F32),
            pltpu.SemaphoreType.DMA((5, n_pairs)),
            pltpu.SemaphoreType.DMA((3,)),
            pltpu.SemaphoreType.DMA((seq // tb,)),
        ],
        compiler_params=pltpu.CompilerParams(vmem_limit_bytes=120 * 1024 * 1024, disable_bounds_checks=True),
        name="rmt_hedgehog",
    )(
        A_x.reshape(seq // seg, seg, dm),
        A_mem0.reshape(n_mem, dm),
        feature_major(A_Wq),
        feature_major(A_Wk),
        feature_major(A_Wv),
        A_Wo.reshape(hd, dm),
        B_wqkv,
        jnp.transpose(B_w_phi, (1, 2, 0)),
        B_wo,
    )
    return out.reshape(batch, seq, dm)
```

```python
import functools
import math

import jax
import jax.numpy as jnp
from jax import lax
import jax.experimental.pallas as pl
import jax.experimental.pallas.tpu as pltpu

F32 = jnp.float32
BF16 = jnp.bfloat16
U32 = jnp.uint32
I32 = jnp.int32

LN_EPS = 1e-5
DEN_EPS = 1e-6
LOG2E = math.log2(math.e)
EARLY_ROWS = 8
EARLY_TILES = ((0, 3), (4, 6), (7, 9))
STEP_REGULAR = ("00000000000111111223", 1, "qosv", 256)
STEP_EARLY = ("00000000001111112212", 9, "qosv", 256)


def _nn(a, b):
    return lax.dot_general(a, b, (((1,), (0,)), ((), ())), preferred_element_type=F32)


def _nt(a, b):
    return lax.dot_general(a, b, (((1,), (1,)), ((), ())), preferred_element_type=F32)


def _unpack(x):
    return pltpu.bitcast(x, BF16)


def _pack(x):
    return pltpu.bitcast(x, U32)


def _iota(shape, dim):
    return lax.broadcasted_iota(I32, shape, dim)


def _recip(x):
    r = pltpu.reciprocal(x, approx=True)
    return r * (2.0 - x * r)


def _layernorm(x):
    inv_n = 1.0 / x.shape[-1]
    m = jnp.sum(x, axis=-1, keepdims=True) * inv_n
    d = x - m
    v = jnp.sum(d * d, axis=-1, keepdims=True) * inv_n
    return d * lax.rsqrt(v + LN_EPS)


def _pair_blockdiag(x, dh):
    rows, width = x.shape
    top, bot = [], []
    zero = jnp.zeros((rows, 128), F32)
    for c in range(0, width, 128):
        t = x[:, c:c + 128]
        if c + 128 <= dh:
            top.append(t)
            bot.append(zero)
        elif c >= dh:
            top.append(zero)
            bot.append(t)
        else:
            first = _iota((rows, 128), 1) < dh - c
            top.append(jnp.where(first, t, 0.0))
            bot.append(jnp.where(first, 0.0, t))
    return jnp.concatenate(
        [jnp.concatenate(top, axis=1), jnp.concatenate(bot, axis=1)], axis=0
    ).astype(BF16)


def _pair_softmax(s, n_mem, scale):
    rows = s.shape[0]
    row = _iota(s.shape, 0)
    col = _iota(s.shape, 1)
    is_a = col < rows
    key = jnp.where(is_a, col, col - rows)
    s = jnp.where((row < n_mem) | (row >= key), s * scale, -1000000000.0)
    ma = jnp.max(jnp.where(is_a, s, -jnp.inf), axis=1, keepdims=True)
    mb = jnp.max(jnp.where(is_a, -jnp.inf, s), axis=1, keepdims=True)
    e = jnp.exp(s - jnp.where(is_a, ma, mb))
    la = jnp.sum(jnp.where(is_a, e, 0.0), axis=1, keepdims=True)
    lb = jnp.sum(jnp.where(is_a, 0.0, e), axis=1, keepdims=True)
    return e / jnp.where(is_a, la, lb)


def _over_features(x, op):
    r = functools.reduce(op, [x[i:i + 8] for i in range(0, x.shape[0], 8)])
    r = op(r, pltpu.roll(r, 4, 0))
    return op(r, pltpu.roll(r, 2, 0))


def _feature_map(p):
    def tile(r):
        return jnp.concatenate([r] * (p.shape[0] // 8), axis=0)

    ep = jnp.exp2(p - tile(_over_features(p, jnp.maximum)))
    en = jnp.exp2(tile(_over_features(p, jnp.minimum)) - p)
    return jnp.concatenate([e * tile(_recip(_over_features(e, jnp.add))) for e in (ep, en)], axis=0)


def _kernel(x_hbm, mem0_ref, wq_hbm, wk_hbm, wv_hbm, wo_hbm, bqkv_hbm, wphi_ref, bwo_hbm,
            out_hbm,
            stage, wqkv, wo, x_stage, out_stage, bqkv_stage, bwo_stage, fold, bw1, bwq, bwo,
            xres, xn_a, xn_b, o_scr, v_scr, kv_acc, z_acc, early_x, early_xn, early_qkv,
            w_sem, b_sem, out_sem,
            *, seg, dh, n_layers, tb, unroll):
    n_pairs = wqkv.shape[0]
    pw = 2 * dh
    half = pw // 2
    seq, dm = xres.shape
    n_mem = mem0_ref.shape[0]
    n_seg = seq // seg
    scale = dh ** -0.5
    bdh, _, bh = wphi_ref.shape
    n_grp = bh // 2
    gw = 2 * bdh

    x_chunk = n_seg // n_pairs

    def pair_rows(p):
        return pl.ds(pl.multiple_of(p * pw, pw), pw)

    def weight_copy(i, p):
        src = (wq_hbm, wk_hbm, wv_hbm, wo_hbm)[i]
        return pltpu.make_async_copy(src.at[pair_rows(p)], stage.at[i, pair_rows(p)], w_sem.at[i, p])

    def pair_copies(p):
        segs = pl.ds(p * x_chunk, x_chunk)
        return [weight_copy(i, p) for i in range(3)] + [
            pltpu.make_async_copy(x_hbm.at[segs], x_stage.at[segs], w_sem.at[4, p])]

    def start_pair(p):
        for c in pair_copies(p) + [weight_copy(3, p - 1)]:
            c.start()

    def pack_wo(i, p):
        wo[pl.ds(pl.multiple_of(p * half, half), half), :] = _pack(stage[i, pair_rows(p), :])

    early_copy = pltpu.make_async_copy(
        x_hbm.at[:, pl.ds(seg - EARLY_ROWS, EARLY_ROWS)], early_x, b_sem.at[0])
    bqkv_copy = pltpu.make_async_copy(bqkv_hbm, bqkv_stage, b_sem.at[1])
    bwo_copy = pltpu.make_async_copy(bwo_hbm, bwo_stage, b_sem.at[2])
    early_copy.start()

    wphi = wphi_ref[...].astype(F32)
    wf = jnp.concatenate([wphi[d] for d in range(bdh)], axis=1)
    src = _iota((dm, 128), 0)
    natural = (src % bh) * bdh + src // bh
    first_grp = [c // gw for c in range(0, dm, 128)]
    r = _iota((4 * gw, 128), 0)
    lane = _iota((4 * gw, 128), 1)
    pick = ((r % gw) // 2 == lane).astype(BF16)
    head_start = ((r // gw) * 2 + r % 2) * bdh
    for j, g0 in enumerate(first_grp):
        wj = _nn(wf, (natural == _iota((dm, 128), 1) + j * 128).astype(BF16))
        wj = jnp.concatenate([wj, jnp.zeros((128 - bdh, 128), F32)], axis=0).astype(BF16)
        d = lane + (j * 128 - g0 * gw) - head_start
        fold[j] = jnp.where((d >= 0) & (d < bdh), _nn(pick, wj), 0.0).astype(BF16)

    for c in pair_copies(0):
        c.start()
    early_copy.wait()
    early_xn[...] = _layernorm(
        early_x[...].astype(F32).reshape(early_xn.shape)).astype(BF16)

    start_pair(1)

    def load_pair(p, carry):
        for c in pair_copies(p):
            c.wait()
        pl.when(p > 0)(lambda: weight_copy(3, p - 1).wait())
        pl.when(p == n_pairs - 2)(lambda: weight_copy(3, n_pairs - 1).start())
        pl.when(p + 2 < n_pairs)(lambda: start_pair(p + 2))
        col = 0
        for i, (lo, hi) in enumerate(EARLY_TILES):
            w = stage[i, pair_rows(p), :]
            early_qkv[p, :, col:col + (hi - lo) * 128] = _nt(
                early_xn[...], w[lo * 128 - i * pw:hi * 128 - i * pw])
            col += (hi - lo) * 128
            wqkv[p, :, i * pw:(i + 1) * pw] = _pack(w.T)
        pack_wo(jnp.where(p > 0, 3, 0), jnp.maximum(p - 1, 0))
        wide = x_stage[pl.ds(p * x_chunk, x_chunk)].astype(F32).reshape(x_chunk * seg, dm)
        xres[pl.ds(pl.multiple_of(p * x_chunk * seg, x_chunk * seg), x_chunk * seg), :] = wide
        return carry

    lax.fori_loop(0, n_pairs, load_pair, 0)
    weight_copy(3, n_pairs - 1).wait()
    pack_wo(3, n_pairs - 1)
    bqkv_copy.start()
    bwo_copy.start()

    def fold_phi(base):
        groups = [None] * n_grp
        for j, g0 in enumerate(first_grp):
            t = _nt(fold[j], bqkv_stage[:, base + j * 128:base + (j + 1) * 128]) * LOG2E
            for i in range(4):
                part = t[i * gw:(i + 1) * gw]
                groups[g0 + i] = part if groups[g0 + i] is None else groups[g0 + i] + part
        return groups

    def hedgehog_weights():
        bqkv_copy.wait()
        bwo_copy.wait()
        wvt = bqkv_stage[:, 2 * dm:].astype(F32).T
        bwq[...] = _pack(jnp.concatenate(fold_phi(0), axis=0).astype(BF16))
        bw1[...] = _pack(jnp.concatenate(
            [t for g, wpk in enumerate(fold_phi(dm)) for t in (wpk, wvt[g * gw:(g + 1) * gw])],
            axis=0).astype(BF16))
        bwo[...] = _pack(bwo_stage[...])

    def seg_rows(s):
        return pl.ds(pl.multiple_of(s * seg, seg), seg)

    def rmt_step(s, mem, early):
        plan, norm_pair, order, ks = STEP_EARLY if early else STEP_REGULAR
        h = jnp.concatenate([mem, xn_a[...]], axis=0)
        h_short = h[:-EARLY_ROWS].astype(BF16)
        early_rows = pl.ds(pl.multiple_of(s * EARLY_ROWS, EARLY_ROWS), EARLY_ROWS)
        xn_next = _layernorm(xres[seg_rows(jnp.minimum(s + 1, n_seg - 1)), :])
        prev = seg_rows(jnp.maximum(s - 1, 0))
        xn_b[prev, :] = _layernorm(xres[prev, :]).astype(BF16)
        pending = {norm_pair: [xn_b[seg_rows(jnp.maximum(s, 1) - 1), :128].astype(F32)[:8]]}

        def project(p):
            spans, end = [], 0
            for lo, hi in EARLY_TILES if early else ():
                spans += [(h, end, lo)] * (end < lo) + [(h_short, lo, hi)]
                end = hi
            spans += [(h, end, 3 * pw // 128)] * (end < 3 * pw // 128)
            spans = [(x, slice(lo * 128, hi * 128)) for x, lo, hi in spans]
            if p > 0:
                parts = [_nn(x, _unpack(wqkv[p, :, cols])) for x, cols in spans]
            else:
                parts = [_nn(x[:, :ks], _unpack(wqkv[p, :ks // 2, cols])) for x, cols in spans]
                parts = [_nn(x[:, ks:], _unpack(wqkv[p, ks // 2:, cols])) + start
                         for start, (x, cols) in zip(parts, spans)]
            col = 0
            for i, t in enumerate(parts):
                if t.shape[0] < h.shape[0]:
                    known = early_qkv[p, early_rows, col:col + t.shape[1]]
                    parts[i] = jnp.concatenate([t, known], axis=0)
                    col += t.shape[1]
            return jnp.concatenate(parts, axis=1)

        def weighted_values(p, prob, v):
            head = prob[:n_mem]
            if p in pending:
                work = functools.reduce(jnp.add, pending[p])[:, :prob.shape[1]]
                head = jnp.where(s < 0, work, head)
            seen = n_mem + 8
            o = _nn(jnp.concatenate([head, prob[seen:]], axis=0), _pair_blockdiag(v, dh))
            v_scr[p, :seen, :] = v[:seen]
            v_scr[p, seen:seen + 1, :] = jnp.sum(v[seen:], axis=0, keepdims=True)
            first = jnp.concatenate(
                [prob[n_mem:seen], jnp.zeros((8, 128 - prob.shape[1]), F32)], axis=1)
            lane = _iota(first.shape, 1)
            tiles = [None] * (pw // 128)
            for k in range(seen + 1):
                wa, wb = (jnp.sum(jnp.where(lane == col, first, 0.0), axis=1, keepdims=True)
                          for col in (k, prob.shape[0] + k))
                for t, c in enumerate(range(0, pw, 128)):
                    w = wa if c + 128 <= dh else wb if c >= dh else jnp.where(lane < dh - c, wa, wb)
                    term = w * jnp.broadcast_to(v_scr[p, k:k + 1, c:c + 128], (8, 128))
                    tiles[t] = term if k == 0 else tiles[t] + term
            pending.setdefault(p + 1, []).extend(tiles)
            return jnp.concatenate([o[:n_mem], jnp.concatenate(tiles, axis=1), o[n_mem:]], axis=0)

        def out_proj(acc, lo, hi, cols=slice(None)):
            t = _nn(o_scr[:, lo * pw:hi * pw], _unpack(wo[lo * half:hi * half, cols]))
            return t if acc is None else t + acc[:, cols]

        qkv, prob = {}, {}
        acc, done = None, 0
        for p in range(len(plan)):
            r = p - (len(plan) - n_pairs)
            for what in order:
                if what == "q" and p < n_pairs:
                    qkv[p] = project(p)
                if what == "o" and plan[p] != "0":
                    acc = out_proj(acc, done, done + int(plan[p]))
                    done += int(plan[p])
                if what == "s" and 0 <= p - 1 < n_pairs:
                    t = qkv[p - 1]
                    scores = _nt(t[:, :pw], _pair_blockdiag(t[:, pw:2 * pw], dh))
                    prob[p - 1] = _pair_softmax(scores, n_mem, scale)
                if what == "v" and r >= 0:
                    o_scr[:, r * pw:(r + 1) * pw] = weighted_values(r, prob[r], qkv[r][:, 2 * pw:])
        acc = out_proj(acc, done, done + 1)
        acc = jnp.concatenate(
            [out_proj(acc, done + 1, n_pairs, cols) for cols in (slice(0, ks), slice(ks, dm))], axis=1)
        xn_a[...] = xn_next
        rows = seg_rows(s)
        xres[rows, :] = xres[rows, :] + acc[n_mem:]
        return acc[:n_mem]

    def rmt_steps(early):
        def body(i, mem):
            for u in range(unroll):
                mem = rmt_step(i * unroll + u, mem, early)
            return mem

        lax.fori_loop(0, n_seg // unroll, body, mem0_ref[...].astype(F32))

    def rmt_layer(layer):
        xn_a[...] = _layernorm(xres[0:seg, :])
        pl.when(layer == 0)(functools.partial(rmt_steps, True))
        pl.when(layer > 0)(functools.partial(rmt_steps, False))
        last = slice(seq - seg, seq)
        xn_b[last, :] = _layernorm(xres[last, :]).astype(BF16)

    chunk = 4
    n_chunk = n_grp // chunk

    def blk_rows(i):
        return pl.ds(pl.multiple_of(i * tb, tb), tb)

    def kv_block(i, carry):
        xn = xn_b[blk_rows(i), :]
        proj = {}
        for c in range(n_chunk + 1):
            if c < n_chunk:
                proj[c] = _nt(_unpack(bw1[c * chunk * gw:(c + 1) * chunk * gw, :]), xn)
            if c >= 1:
                t = proj[c - 1]
                for j in range(chunk):
                    g = (c - 1) * chunk + j
                    phi = _feature_map(t[2 * j * gw:(2 * j + 1) * gw])
                    kv_acc[g] += _nt(t[(2 * j + 1) * gw:(2 * j + 2) * gw], phi.astype(BF16))
                    z_acc[g] += functools.reduce(jnp.add, [phi[:, i:i + 128] for i in range(0, tb, 128)])
        return carry

    def out_copy(i):
        return pltpu.make_async_copy(out_stage.at[blk_rows(i)], out_hbm.at[blk_rows(i)], out_sem.at[i])

    def out_block(i, layer):
        rows = blk_rows(i)
        xn = xn_b[rows, :]
        sublane = _iota((8, tb), 0)
        proj, outs = {}, []

        def out_proj(y, lo, hi):
            o = jnp.concatenate(outs, axis=0)[lo:hi].astype(BF16).T
            return _nn(o, _unpack(bwo[lo // 2:hi // 2, :])) + y

        y = xres[rows, :]
        for c in range(n_chunk + 1):
            if c < n_chunk:
                proj[c] = _nt(_unpack(bwq[c * chunk * bdh:(c + 1) * chunk * bdh, :]), xn)
            else:
                y = out_proj(y, 0, 256)
            if c >= 1:
                for j in range(chunk):
                    g = (c - 1) * chunk + j
                    phi = _feature_map(proj[c - 1][j * gw:(j + 1) * gw])
                    z = jnp.concatenate([z_acc[g]] * (tb // 128), axis=1)
                    inv = _recip(_over_features(phi * z, jnp.add) + DEN_EPS)
                    swapped = pltpu.roll(inv, 1, 0)
                    inv_a = jnp.where(sublane % 2 == 0, inv, swapped)
                    inv_b = jnp.where(sublane % 2 == 0, swapped, inv)
                    inv_ab = jnp.where(sublane < bdh % 8, inv_a, inv_b)
                    outs.append(_nn(kv_acc[g], phi.astype(BF16))
                                * jnp.concatenate([inv_a, inv_a, inv_ab, inv_b, inv_b], axis=0))
        y = out_proj(out_proj(y, 256, 384), 384, dm)
        xres[rows, :] = y
        out_stage[rows, :] = y.astype(BF16)

        @pl.when(layer == n_layers - 1)
        def _():
            out_copy(i).start()

        return layer

    def hedgehog_layer(layer):
        kv_acc[...] = jnp.zeros(kv_acc.shape, F32)
        z_acc[...] = jnp.zeros(z_acc.shape, F32)
        lax.fori_loop(0, seq // tb, kv_block, 0)
        shape = kv_acc.shape[1:]
        same_head = _iota(shape, 0) // bdh == _iota(shape, 1) % 2
        for g in range(n_grp):
            kv_acc[g] = jnp.where(same_head, kv_acc[g], 0.0)
            z_acc[g] = jnp.broadcast_to(jnp.sum(z_acc[g], axis=1, keepdims=True), z_acc.shape[1:])
        lax.fori_loop(0, seq // tb, out_block, layer)

    def layer_pair(layer, carry):
        rmt_layer(layer)
        pl.when(layer == 0)(hedgehog_weights)
        hedgehog_layer(layer)
        return carry

    lax.fori_loop(0, n_layers, layer_pair, 0)
    for i in range(seq // tb):
        out_copy(i).wait()


@functools.partial(jax.jit, static_argnames=("A_seg_len",))
def pallas_interleave_layers__memory_aug_recurrent_mem_tr__linear_kernel_hedgehog__prompt_kernel(
    A_x: jax.Array,
    A_mem0: jax.Array,
    A_Wq: jax.Array,
    A_Wk: jax.Array,
    A_Wv: jax.Array,
    A_Wo: jax.Array,
    A_seg_len: int,
    B_x: jax.Array,
    B_wqkv: jax.Array,
    B_w_phi: jax.Array,
    B_wo: jax.Array,
):
    del B_x
    batch, seq, dm = A_x.shape
    _, heads, dh = A_Wq.shape
    n_mem = A_mem0.shape[1]
    bh, bdh, _ = B_w_phi.shape
    seg = int(A_seg_len)
    assert batch == 1 and bdh == 20 and bh * bdh == dm and heads % 2 == 0
    assert (2 * dh) % 128 == 0 and n_mem % 8 == 0 and seg % 16 == 0 and 2 * (n_mem + seg) <= 128
    n_pairs, pw, hd = heads // 2, 2 * dh, heads * dh
    tb, unroll = 512, 2
    early_rows = seq // seg * EARLY_ROWS
    early_cols = 128 * sum(hi - lo for lo, hi in EARLY_TILES)

    def feature_major(w):
        return jnp.transpose(w, (1, 2, 0)).reshape(hd, dm)

    hbm = pl.BlockSpec(memory_space=pl.ANY)
    vmem = pl.BlockSpec(memory_space=pltpu.VMEM)
    out = pl.pallas_call(
        functools.partial(_kernel, seg=seg, dh=dh, n_layers=2, tb=tb, unroll=unroll),
        out_shape=jax.ShapeDtypeStruct((seq, dm), A_x.dtype),
        in_specs=[hbm, vmem, hbm, hbm, hbm, hbm, hbm, vmem, hbm],
        out_specs=hbm,
        scratch_shapes=[
            pltpu.VMEM((4, hd, dm), BF16),
            pltpu.VMEM((n_pairs, dm // 2, 3 * pw), U32),
            pltpu.VMEM((hd // 2, dm), U32),
            pltpu.VMEM((seq // seg, seg, dm), BF16),
            pltpu.VMEM((seq, dm), BF16),
            pltpu.VMEM((dm, 3 * dm), BF16),
            pltpu.VMEM((dm, dm), BF16),
            pltpu.VMEM((dm // 128, 8 * bdh, 128), BF16),
            pltpu.VMEM((dm, dm), U32),
            pltpu.VMEM((dm // 2, dm), U32),
            pltpu.VMEM((dm // 2, dm), U32),
            pltpu.VMEM((seq, dm), F32),
            pltpu.VMEM((seg, dm), F32),
            pltpu.VMEM((seq, dm), BF16),
            pltpu.VMEM((n_mem + seg, hd), F32),
            pltpu.VMEM((n_pairs, n_mem + 16, pw), F32),
            pltpu.VMEM((bh // 2, 2 * bdh, 4 * bdh), F32),
            pltpu.VMEM((bh // 2, 4 * bdh, 128), F32),
            pltpu.VMEM((seq // seg, EARLY_ROWS, dm), BF16),
            pltpu.VMEM((early_rows, dm), BF16),
            pltpu.VMEM((n_pairs, early_rows, early_cols), F32),
            pltpu.SemaphoreType.DMA((5, n_pairs)),
            pltpu.SemaphoreType.DMA((3,)),
            pltpu.SemaphoreType.DMA((seq // tb,)),
        ],
        compiler_params=pltpu.CompilerParams(vmem_limit_bytes=120 * 1024 * 1024, disable_bounds_checks=True),
        name="rmt_hedgehog",
    )(
        A_x.reshape(seq // seg, seg, dm),
        A_mem0.reshape(n_mem, dm),
        feature_major(A_Wq),
        feature_major(A_Wk),
        feature_major(A_Wv),
        A_Wo.reshape(hd, dm),
        B_wqkv,
        jnp.transpose(B_w_phi, (1, 2, 0)),
        B_wo,
    )
    return out.reshape(batch, seq, dm)
```

```python
import functools
import math

import jax
import jax.numpy as jnp
from jax import lax
import jax.experimental.pallas as pl
import jax.experimental.pallas.tpu as pltpu

F32 = jnp.float32
BF16 = jnp.bfloat16
U32 = jnp.uint32
I32 = jnp.int32

LN_EPS = 1e-5
DEN_EPS = 1e-6
LOG2E = math.log2(math.e)
EARLY_ROWS = 8
EARLY_TILES = ((0, 3), (4, 6), (7, 9))
STEP_REGULAR = ("00000000000111111223", 1, "qosv", 256)
STEP_EARLY = ("00000001110111002221", 2, "qosv", 256)


def _nn(a, b):
    return lax.dot_general(a, b, (((1,), (0,)), ((), ())), preferred_element_type=F32)


def _nt(a, b):
    return lax.dot_general(a, b, (((1,), (1,)), ((), ())), preferred_element_type=F32)


def _unpack(x):
    return pltpu.bitcast(x, BF16)


def _pack(x):
    return pltpu.bitcast(x, U32)


def _iota(shape, dim):
    return lax.broadcasted_iota(I32, shape, dim)


def _recip(x):
    r = pltpu.reciprocal(x, approx=True)
    return r * (2.0 - x * r)


def _layernorm(x):
    inv_n = 1.0 / x.shape[-1]
    m = jnp.sum(x, axis=-1, keepdims=True) * inv_n
    d = x - m
    v = jnp.sum(d * d, axis=-1, keepdims=True) * inv_n
    return d * lax.rsqrt(v + LN_EPS)


def _pair_blockdiag(x, dh):
    rows, width = x.shape
    top, bot = [], []
    zero = jnp.zeros((rows, 128), F32)
    for c in range(0, width, 128):
        t = x[:, c:c + 128]
        if c + 128 <= dh:
            top.append(t)
            bot.append(zero)
        elif c >= dh:
            top.append(zero)
            bot.append(t)
        else:
            first = _iota((rows, 128), 1) < dh - c
            top.append(jnp.where(first, t, 0.0))
            bot.append(jnp.where(first, 0.0, t))
    return jnp.concatenate(
        [jnp.concatenate(top, axis=1), jnp.concatenate(bot, axis=1)], axis=0
    ).astype(BF16)


def _pair_softmax(s, n_mem, scale):
    rows = s.shape[0]
    row = _iota(s.shape, 0)
    col = _iota(s.shape, 1)
    is_a = col < rows
    key = jnp.where(is_a, col, col - rows)
    s = jnp.where((row < n_mem) | (row >= key), s * scale, -1000000000.0)
    ma = jnp.max(jnp.where(is_a, s, -jnp.inf), axis=1, keepdims=True)
    mb = jnp.max(jnp.where(is_a, -jnp.inf, s), axis=1, keepdims=True)
    e = jnp.exp(s - jnp.where(is_a, ma, mb))
    la = jnp.sum(jnp.where(is_a, e, 0.0), axis=1, keepdims=True)
    lb = jnp.sum(jnp.where(is_a, 0.0, e), axis=1, keepdims=True)
    return e / jnp.where(is_a, la, lb)


def _over_features(x, op):
    r = functools.reduce(op, [x[i:i + 8] for i in range(0, x.shape[0], 8)])
    r = op(r, pltpu.roll(r, 4, 0))
    return op(r, pltpu.roll(r, 2, 0))


def _feature_map(p):
    def tile(r):
        return jnp.concatenate([r] * (p.shape[0] // 8), axis=0)

    ep = jnp.exp2(p - tile(_over_features(p, jnp.maximum)))
    en = jnp.exp2(tile(_over_features(p, jnp.minimum)) - p)
    return jnp.concatenate([e * tile(_recip(_over_features(e, jnp.add))) for e in (ep, en)], axis=0)


def _kernel(x_hbm, mem0_hbm, wq_hbm, wk_hbm, wv_hbm, wo_hbm, bqkv_hbm, wphi_hbm, bwo_hbm,
            out_hbm,
            stage, wqkv, wo, x_stage, out_stage, bqkv_stage, bwo_stage, fold, bw1, bwq, bwo,
            xres, xn_a, xn_b, o_scr, v_scr, kv_acc, z_acc, early_x, early_xn, early_qkv,
            mem0_ref, wphi_ref,
            w_sem, b_sem, out_sem,
            *, seg, dh, n_layers, tb, unroll):
    n_pairs = wqkv.shape[0]
    pw = 2 * dh
    half = pw // 2
    seq, dm = xres.shape
    n_mem = mem0_ref.shape[0]
    n_seg = seq // seg
    scale = dh ** -0.5
    bdh, _, bh = wphi_ref.shape
    n_grp = bh // 2
    gw = 2 * bdh

    x_chunk = n_seg // n_pairs

    def pair_rows(p):
        return pl.ds(pl.multiple_of(p * pw, pw), pw)

    def weight_copy(i, p):
        src = (wq_hbm, wk_hbm, wv_hbm, wo_hbm)[i]
        return pltpu.make_async_copy(src.at[pair_rows(p)], stage.at[i, pair_rows(p)], w_sem.at[i, p])

    def pair_copies(p):
        segs = pl.ds(p * x_chunk, x_chunk)
        return [weight_copy(i, p) for i in range(3)] + [
            pltpu.make_async_copy(x_hbm.at[segs], x_stage.at[segs], w_sem.at[4, p])]

    def start_pair(p):
        for c in pair_copies(p) + [weight_copy(3, p - 1)]:
            c.start()

    def pack_wo(i, p):
        wo[pl.ds(pl.multiple_of(p * half, half), half), :] = _pack(stage[i, pair_rows(p), :])

    early_copy = pltpu.make_async_copy(
        x_hbm.at[:, pl.ds(seg - EARLY_ROWS, EARLY_ROWS)], early_x, b_sem.at[0])
    bqkv_copy = pltpu.make_async_copy(bqkv_hbm, bqkv_stage, b_sem.at[1])
    bwo_copy = pltpu.make_async_copy(bwo_hbm, bwo_stage, b_sem.at[2])
    mem0_copy = pltpu.make_async_copy(mem0_hbm, mem0_ref, b_sem.at[3])
    wphi_copy = pltpu.make_async_copy(wphi_hbm, wphi_ref, b_sem.at[4])
    for c in [wphi_copy, early_copy] + pair_copies(0) + [mem0_copy]:
        c.start()
    wphi_copy.wait()

    wphi = wphi_ref[...].astype(F32)
    wf = jnp.concatenate([wphi[d] for d in range(bdh)], axis=1)
    src = _iota((dm, 128), 0)
    natural = (src % bh) * bdh + src // bh
    first_grp = [c // gw for c in range(0, dm, 128)]
    r = _iota((4 * gw, 128), 0)
    lane = _iota((4 * gw, 128), 1)
    pick = ((r % gw) // 2 == lane).astype(BF16)
    head_start = ((r // gw) * 2 + r % 2) * bdh
    for j, g0 in enumerate(first_grp):
        wj = _nn(wf, (natural == _iota((dm, 128), 1) + j * 128).astype(BF16))
        wj = jnp.concatenate([wj, jnp.zeros((128 - bdh, 128), F32)], axis=0).astype(BF16)
        d = lane + (j * 128 - g0 * gw) - head_start
        fold[j] = jnp.where((d >= 0) & (d < bdh), _nn(pick, wj), 0.0).astype(BF16)

    early_copy.wait()
    early_xn[...] = _layernorm(
        early_x[...].astype(F32).reshape(early_xn.shape)).astype(BF16)

    start_pair(1)

    def load_pair(p, carry):
        for c in pair_copies(p):
            c.wait()
        pl.when(p > 0)(lambda: weight_copy(3, p - 1).wait())
        pl.when(p == n_pairs - 2)(lambda: weight_copy(3, n_pairs - 1).start())
        pl.when(p + 2 < n_pairs)(lambda: start_pair(p + 2))
        col = 0
        for i, (lo, hi) in enumerate(EARLY_TILES):
            w = stage[i, pair_rows(p), :]
            early_qkv[p, :, col:col + (hi - lo) * 128] = _nt(
                early_xn[...], w[lo * 128 - i * pw:hi * 128 - i * pw])
            col += (hi - lo) * 128
            wqkv[p, :, i * pw:(i + 1) * pw] = _pack(w.T)
        pack_wo(jnp.where(p > 0, 3, 0), jnp.maximum(p - 1, 0))
        wide = x_stage[pl.ds(p * x_chunk, x_chunk)].astype(F32).reshape(x_chunk * seg, dm)
        xres[pl.ds(pl.multiple_of(p * x_chunk * seg, x_chunk * seg), x_chunk * seg), :] = wide
        return carry

    lax.fori_loop(0, n_pairs, load_pair, 0)
    weight_copy(3, n_pairs - 1).wait()
    pack_wo(3, n_pairs - 1)
    mem0_copy.wait()
    bqkv_copy.start()
    bwo_copy.start()

    def fold_phi(base):
        groups = [None] * n_grp
        for j, g0 in enumerate(first_grp):
            t = _nt(fold[j], bqkv_stage[:, base + j * 128:base + (j + 1) * 128]) * LOG2E
            for i in range(4):
                part = t[i * gw:(i + 1) * gw]
                groups[g0 + i] = part if groups[g0 + i] is None else groups[g0 + i] + part
        return groups

    def hedgehog_weights():
        bqkv_copy.wait()
        bwo_copy.wait()
        wvt = bqkv_stage[:, 2 * dm:].astype(F32).T
        bwq[...] = _pack(jnp.concatenate(fold_phi(0), axis=0).astype(BF16))
        bw1[...] = _pack(jnp.concatenate(
            [t for g, wpk in enumerate(fold_phi(dm)) for t in (wpk, wvt[g * gw:(g + 1) * gw])],
            axis=0).astype(BF16))
        bwo[...] = _pack(bwo_stage[...])

    def seg_rows(s):
        return pl.ds(pl.multiple_of(s * seg, seg), seg)

    def rmt_step(s, mem, early):
        plan, norm_pair, order, ks = STEP_EARLY if early else STEP_REGULAR
        h = jnp.concatenate([mem, xn_a[...]], axis=0)
        h_short = h[:-EARLY_ROWS].astype(BF16)
        early_rows = pl.ds(pl.multiple_of(s * EARLY_ROWS, EARLY_ROWS), EARLY_ROWS)
        xn_next = _layernorm(xres[seg_rows(jnp.minimum(s + 1, n_seg - 1)), :])
        prev = seg_rows(jnp.maximum(s - 1, 0))
        xn_b[prev, :] = _layernorm(xres[prev, :]).astype(BF16)
        pending = {norm_pair: [xn_b[seg_rows(jnp.maximum(s, 1) - 1), :128].astype(F32)[:8]]}

        def project(p):
            spans, end = [], 0
            for lo, hi in EARLY_TILES if early else ():
                spans += [(h, end, lo)] * (end < lo) + [(h_short, lo, hi)]
                end = hi
            spans += [(h, end, 3 * pw // 128)] * (end < 3 * pw // 128)
            spans = [(x, slice(lo * 128, hi * 128)) for x, lo, hi in spans]
            if p > 0:
                parts = [_nn(x, _unpack(wqkv[p, :, cols])) for x, cols in spans]
            else:
                parts = [_nn(x[:, :ks], _unpack(wqkv[p, :ks // 2, cols])) for x, cols in spans]
                parts = [_nn(x[:, ks:], _unpack(wqkv[p, ks // 2:, cols])) + start
                         for start, (x, cols) in zip(parts, spans)]
            col = 0
            for i, t in enumerate(parts):
                if t.shape[0] < h.shape[0]:
                    known = early_qkv[p, early_rows, col:col + t.shape[1]]
                    parts[i] = jnp.concatenate([t, known], axis=0)
                    col += t.shape[1]
            return jnp.concatenate(parts, axis=1)

        def weighted_values(p, prob, v):
            head = prob[:n_mem]
            if p in pending:
                work = functools.reduce(jnp.add, pending[p])[:, :prob.shape[1]]
                head = jnp.where(s < 0, work, head)
            seen = n_mem + 8
            o = _nn(jnp.concatenate([head, prob[seen:]], axis=0), _pair_blockdiag(v, dh))
            v_scr[p, :seen, :] = v[:seen]
            v_scr[p, seen:seen + 1, :] = jnp.sum(v[seen:], axis=0, keepdims=True)
            first = jnp.concatenate(
                [prob[n_mem:seen], jnp.zeros((8, 128 - prob.shape[1]), F32)], axis=1)
            lane = _iota(first.shape, 1)
            tiles = [None] * (pw // 128)
            for k in range(seen + 1):
                wa, wb = (jnp.sum(jnp.where(lane == col, first, 0.0), axis=1, keepdims=True)
                          for col in (k, prob.shape[0] + k))
                for t, c in enumerate(range(0, pw, 128)):
                    w = wa if c + 128 <= dh else wb if c >= dh else jnp.where(lane < dh - c, wa, wb)
                    term = w * jnp.broadcast_to(v_scr[p, k:k + 1, c:c + 128], (8, 128))
                    tiles[t] = term if k == 0 else tiles[t] + term
            pending.setdefault(p + 1, []).extend(tiles)
            return jnp.concatenate([o[:n_mem], jnp.concatenate(tiles, axis=1), o[n_mem:]], axis=0)

        def out_proj(acc, lo, hi, cols=slice(None)):
            t = _nn(o_scr[:, lo * pw:hi * pw], _unpack(wo[lo * half:hi * half, cols]))
            return t if acc is None else t + acc[:, cols]

        qkv, prob = {}, {}
        acc, done = None, 0
        for p in range(len(plan)):
            r = p - (len(plan) - n_pairs)
            for what in order:
                if what == "q" and p < n_pairs:
                    qkv[p] = project(p)
                if what == "o" and plan[p] != "0":
                    acc = out_proj(acc, done, done + int(plan[p]))
                    done += int(plan[p])
                if what == "s" and 0 <= p - 1 < n_pairs:
                    t = qkv[p - 1]
                    scores = _nt(t[:, :pw], _pair_blockdiag(t[:, pw:2 * pw], dh))
                    prob[p - 1] = _pair_softmax(scores, n_mem, scale)
                if what == "v" and r >= 0:
                    o_scr[:, r * pw:(r + 1) * pw] = weighted_values(r, prob[r], qkv[r][:, 2 * pw:])
        acc = out_proj(acc, done, done + 1)
        acc = jnp.concatenate(
            [out_proj(acc, done + 1, n_pairs, cols) for cols in (slice(0, ks), slice(ks, dm))], axis=1)
        xn_a[...] = xn_next
        rows = seg_rows(s)
        xres[rows, :] = xres[rows, :] + acc[n_mem:]
        return acc[:n_mem]

    def rmt_steps(early):
        def body(i, mem):
            for u in range(unroll):
                mem = rmt_step(i * unroll + u, mem, early)
            return mem

        lax.fori_loop(0, n_seg // unroll, body, mem0_ref[...].astype(F32))

    def rmt_layer(layer):
        xn_a[...] = _layernorm(xres[0:seg, :])
        pl.when(layer == 0)(functools.partial(rmt_steps, True))
        pl.when(layer > 0)(functools.partial(rmt_steps, False))
        last = slice(seq - seg, seq)
        xn_b[last, :] = _layernorm(xres[last, :]).astype(BF16)

    chunk = 4
    n_chunk = n_grp // chunk

    def blk_rows(i):
        return pl.ds(pl.multiple_of(i * tb, tb), tb)

    def kv_block(i, carry):
        xn = xn_b[blk_rows(i), :]
        proj = {}
        for c in range(n_chunk + 1):
            if c < n_chunk:
                proj[c] = _nt(_unpack(bw1[c * chunk * gw:(c + 1) * chunk * gw, :]), xn)
            if c >= 1:
                t = proj[c - 1]
                for j in range(chunk):
                    g = (c - 1) * chunk + j
                    phi = _feature_map(t[2 * j * gw:(2 * j + 1) * gw])
                    kv_acc[g] += _nt(t[(2 * j + 1) * gw:(2 * j + 2) * gw], phi.astype(BF16))
                    z_acc[g] += functools.reduce(jnp.add, [phi[:, i:i + 128] for i in range(0, tb, 128)])
        return carry

    def out_copy(i):
        return pltpu.make_async_copy(out_stage.at[blk_rows(i)], out_hbm.at[blk_rows(i)], out_sem.at[i])

    def out_block(i, layer):
        rows = blk_rows(i)
        xn = xn_b[rows, :]
        sublane = _iota((8, tb), 0)
        proj, outs = {}, []

        def out_proj(y, lo, hi):
            o = jnp.concatenate(outs, axis=0)[lo:hi].astype(BF16).T
            return _nn(o, _unpack(bwo[lo // 2:hi // 2, :])) + y

        y = xres[rows, :]
        for c in range(n_chunk + 1):
            if c < n_chunk:
                proj[c] = _nt(_unpack(bwq[c * chunk * bdh:(c + 1) * chunk * bdh, :]), xn)
            else:
                y = out_proj(y, 0, 256)
            if c >= 1:
                for j in range(chunk):
                    g = (c - 1) * chunk + j
                    phi = _feature_map(proj[c - 1][j * gw:(j + 1) * gw])
                    z = jnp.concatenate([z_acc[g]] * (tb // 128), axis=1)
                    inv = _recip(_over_features(phi * z, jnp.add) + DEN_EPS)
                    swapped = pltpu.roll(inv, 1, 0)
                    inv_a = jnp.where(sublane % 2 == 0, inv, swapped)
                    inv_b = jnp.where(sublane % 2 == 0, swapped, inv)
                    inv_ab = jnp.where(sublane < bdh % 8, inv_a, inv_b)
                    outs.append(_nn(kv_acc[g], phi.astype(BF16))
                                * jnp.concatenate([inv_a, inv_a, inv_ab, inv_b, inv_b], axis=0))
        y = out_proj(out_proj(y, 256, 384), 384, dm)
        xres[rows, :] = y
        out_stage[rows, :] = y.astype(BF16)

        @pl.when(layer == n_layers - 1)
        def _():
            out_copy(i).start()

        return layer

    def hedgehog_layer(layer):
        kv_acc[...] = jnp.zeros(kv_acc.shape, F32)
        z_acc[...] = jnp.zeros(z_acc.shape, F32)
        lax.fori_loop(0, seq // tb, kv_block, 0)
        shape = kv_acc.shape[1:]
        same_head = _iota(shape, 0) // bdh == _iota(shape, 1) % 2
        for g in range(n_grp):
            kv_acc[g] = jnp.where(same_head, kv_acc[g], 0.0)
            z_acc[g] = jnp.broadcast_to(jnp.sum(z_acc[g], axis=1, keepdims=True), z_acc.shape[1:])
        lax.fori_loop(0, seq // tb, out_block, layer)

    def layer_pair(layer, carry):
        rmt_layer(layer)
        pl.when(layer == 0)(hedgehog_weights)
        hedgehog_layer(layer)
        return carry

    lax.fori_loop(0, n_layers, layer_pair, 0)
    for i in range(seq // tb):
        out_copy(i).wait()


@functools.partial(jax.jit, static_argnames=("A_seg_len",))
def pallas_interleave_layers__memory_aug_recurrent_mem_tr__linear_kernel_hedgehog__prompt_kernel(
    A_x: jax.Array,
    A_mem0: jax.Array,
    A_Wq: jax.Array,
    A_Wk: jax.Array,
    A_Wv: jax.Array,
    A_Wo: jax.Array,
    A_seg_len: int,
    B_x: jax.Array,
    B_wqkv: jax.Array,
    B_w_phi: jax.Array,
    B_wo: jax.Array,
):
    del B_x
    batch, seq, dm = A_x.shape
    _, heads, dh = A_Wq.shape
    n_mem = A_mem0.shape[1]
    bh, bdh, _ = B_w_phi.shape
    seg = int(A_seg_len)
    assert batch == 1 and bdh == 20 and bh * bdh == dm and heads % 2 == 0
    assert (2 * dh) % 128 == 0 and n_mem % 8 == 0 and seg % 16 == 0 and 2 * (n_mem + seg) <= 128
    n_pairs, pw, hd = heads // 2, 2 * dh, heads * dh
    tb, unroll = 512, 2
    early_rows = seq // seg * EARLY_ROWS
    early_cols = 128 * sum(hi - lo for lo, hi in EARLY_TILES)

    def feature_major(w):
        return jnp.transpose(w, (1, 2, 0)).reshape(hd, dm)

    hbm = pl.BlockSpec(memory_space=pl.ANY)
    out = pl.pallas_call(
        functools.partial(_kernel, seg=seg, dh=dh, n_layers=2, tb=tb, unroll=unroll),
        out_shape=jax.ShapeDtypeStruct((seq, dm), A_x.dtype),
        in_specs=[hbm] * 9,
        out_specs=hbm,
        scratch_shapes=[
            pltpu.VMEM((4, hd, dm), BF16),
            pltpu.VMEM((n_pairs, dm // 2, 3 * pw), U32),
            pltpu.VMEM((hd // 2, dm), U32),
            pltpu.VMEM((seq // seg, seg, dm), BF16),
            pltpu.VMEM((seq, dm), BF16),
            pltpu.VMEM((dm, 3 * dm), BF16),
            pltpu.VMEM((dm, dm), BF16),
            pltpu.VMEM((dm // 128, 8 * bdh, 128), BF16),
            pltpu.VMEM((dm, dm), U32),
            pltpu.VMEM((dm // 2, dm), U32),
            pltpu.VMEM((dm // 2, dm), U32),
            pltpu.VMEM((seq, dm), F32),
            pltpu.VMEM((seg, dm), F32),
            pltpu.VMEM((seq, dm), BF16),
            pltpu.VMEM((n_mem + seg, hd), F32),
            pltpu.VMEM((n_pairs, n_mem + 16, pw), F32),
            pltpu.VMEM((bh // 2, 2 * bdh, 4 * bdh), F32),
            pltpu.VMEM((bh // 2, 4 * bdh, 128), F32),
            pltpu.VMEM((seq // seg, EARLY_ROWS, dm), BF16),
            pltpu.VMEM((early_rows, dm), BF16),
            pltpu.VMEM((n_pairs, early_rows, early_cols), F32),
            pltpu.VMEM((n_mem, dm), BF16),
            pltpu.VMEM((bdh, bdh, bh), BF16),
            pltpu.SemaphoreType.DMA((5, n_pairs)),
            pltpu.SemaphoreType.DMA((5,)),
            pltpu.SemaphoreType.DMA((seq // tb,)),
        ],
        compiler_params=pltpu.CompilerParams(vmem_limit_bytes=120 * 1024 * 1024, disable_bounds_checks=True),
        name="rmt_hedgehog",
    )(
        A_x.reshape(seq // seg, seg, dm),
        A_mem0.reshape(n_mem, dm),
        feature_major(A_Wq),
        feature_major(A_Wk),
        feature_major(A_Wv),
        A_Wo.reshape(hd, dm),
        B_wqkv,
        jnp.transpose(B_w_phi, (1, 2, 0)),
        B_wo,
    )
    return out.reshape(batch, seq, dm)
```

```python
import functools
import math

import jax
import jax.numpy as jnp
from jax import lax
import jax.experimental.pallas as pl
import jax.experimental.pallas.tpu as pltpu

F32 = jnp.float32
BF16 = jnp.bfloat16
U32 = jnp.uint32
I32 = jnp.int32

LN_EPS = 1e-5
DEN_EPS = 1e-6
LOG2E = math.log2(math.e)
EARLY_ROWS = 8
EARLY_TILES = ((0, 3), (4, 6), (7, 9))
OUT_ROWS = 128
STEP_REGULAR = ("00000000000111111223", 1, "qosv", 256)
STEP_EARLY = ("00000001110111002221", 2, "qosv", 256)


def _nn(a, b):
    return lax.dot_general(a, b, (((1,), (0,)), ((), ())), preferred_element_type=F32)


def _nt(a, b):
    return lax.dot_general(a, b, (((1,), (1,)), ((), ())), preferred_element_type=F32)


def _unpack(x):
    return pltpu.bitcast(x, BF16)


def _pack(x):
    return pltpu.bitcast(x, U32)


def _iota(shape, dim):
    return lax.broadcasted_iota(I32, shape, dim)


def _recip(x):
    r = pltpu.reciprocal(x, approx=True)
    return r * (2.0 - x * r)


def _layernorm(x):
    inv_n = 1.0 / x.shape[-1]
    m = jnp.sum(x, axis=-1, keepdims=True) * inv_n
    d = x - m
    v = jnp.sum(d * d, axis=-1, keepdims=True) * inv_n
    return d * lax.rsqrt(v + LN_EPS)


def _pair_blockdiag(x, dh):
    rows, width = x.shape
    top, bot = [], []
    zero = jnp.zeros((rows, 128), F32)
    for c in range(0, width, 128):
        t = x[:, c:c + 128]
        if c + 128 <= dh:
            top.append(t)
            bot.append(zero)
        elif c >= dh:
            top.append(zero)
            bot.append(t)
        else:
            first = _iota((rows, 128), 1) < dh - c
            top.append(jnp.where(first, t, 0.0))
            bot.append(jnp.where(first, 0.0, t))
    return jnp.concatenate(
        [jnp.concatenate(top, axis=1), jnp.concatenate(bot, axis=1)], axis=0
    ).astype(BF16)


def _pair_softmax(s, n_mem, scale):
    rows = s.shape[0]
    row = _iota(s.shape, 0)
    col = _iota(s.shape, 1)
    is_a = col < rows
    key = jnp.where(is_a, col, col - rows)
    s = jnp.where((row < n_mem) | (row >= key), s * scale, -1000000000.0)
    ma = jnp.max(jnp.where(is_a, s, -jnp.inf), axis=1, keepdims=True)
    mb = jnp.max(jnp.where(is_a, -jnp.inf, s), axis=1, keepdims=True)
    e = jnp.exp(s - jnp.where(is_a, ma, mb))
    la = jnp.sum(jnp.where(is_a, e, 0.0), axis=1, keepdims=True)
    lb = jnp.sum(jnp.where(is_a, 0.0, e), axis=1, keepdims=True)
    return e / jnp.where(is_a, la, lb)


def _over_features(x, op):
    r = functools.reduce(op, [x[i:i + 8] for i in range(0, x.shape[0], 8)])
    r = op(r, pltpu.roll(r, 4, 0))
    return op(r, pltpu.roll(r, 2, 0))


def _feature_map(p):
    def tile(r):
        return jnp.concatenate([r] * (p.shape[0] // 8), axis=0)

    ep = jnp.exp2(p - tile(_over_features(p, jnp.maximum)))
    en = jnp.exp2(tile(_over_features(p, jnp.minimum)) - p)
    return jnp.concatenate([e * tile(_recip(_over_features(e, jnp.add))) for e in (ep, en)], axis=0)


def _kernel(x_hbm, mem0_hbm, wq_hbm, wk_hbm, wv_hbm, wo_hbm, bqkv_hbm, wphi_hbm, bwo_hbm,
            out_hbm,
            stage, wqkv, wo, x_stage, out_stage, bqkv_stage, bwo_stage, fold, bw1, bwq, bwo,
            xres, xn_a, xn_b, o_scr, v_scr, kv_acc, z_acc, early_x, early_xn, early_qkv,
            mem0_ref, wphi_ref,
            w_sem, b_sem, out_sem,
            *, seg, dh, n_layers, tb, unroll):
    n_pairs = wqkv.shape[0]
    pw = 2 * dh
    half = pw // 2
    seq, dm = xres.shape
    n_mem = mem0_ref.shape[0]
    n_seg = seq // seg
    scale = dh ** -0.5
    bdh, _, bh = wphi_ref.shape
    n_grp = bh // 2
    gw = 2 * bdh

    x_chunk = n_seg // n_pairs

    def pair_rows(p):
        return pl.ds(pl.multiple_of(p * pw, pw), pw)

    def weight_copy(i, p):
        src = (wq_hbm, wk_hbm, wv_hbm, wo_hbm)[i]
        return pltpu.make_async_copy(
            src.at[pair_rows(p)], stage.at[i, pair_rows(p)], w_sem.at[i, p % 4])

    def pair_copies(p):
        segs = pl.ds(p * x_chunk, x_chunk)
        return [weight_copy(i, p) for i in range(3)] + [
            pltpu.make_async_copy(x_hbm.at[segs], x_stage.at[segs], w_sem.at[4, p % 4])]

    def start_pair(p):
        for c in pair_copies(p) + [weight_copy(3, p - 1)]:
            c.start()

    def pack_wo(i, p):
        wo[pl.ds(pl.multiple_of(p * half, half), half), :] = _pack(stage[i, pair_rows(p), :])

    early_copy = pltpu.make_async_copy(
        x_hbm.at[:, pl.ds(seg - EARLY_ROWS, EARLY_ROWS)], early_x, b_sem.at[0])
    bqkv_copy = pltpu.make_async_copy(bqkv_hbm, bqkv_stage, b_sem.at[1])
    bwo_copy = pltpu.make_async_copy(bwo_hbm, bwo_stage, b_sem.at[2])
    mem0_copy = pltpu.make_async_copy(mem0_hbm, mem0_ref, b_sem.at[3])
    wphi_copy = pltpu.make_async_copy(wphi_hbm, wphi_ref, b_sem.at[4])
    for c in [wphi_copy, early_copy] + pair_copies(0) + [mem0_copy]:
        c.start()
    wphi_copy.wait()

    wphi = wphi_ref[...].astype(F32)
    wf = jnp.concatenate([wphi[d] for d in range(bdh)], axis=1)
    src = _iota((dm, 128), 0)
    natural = (src % bh) * bdh + src // bh
    first_grp = [c // gw for c in range(0, dm, 128)]
    r = _iota((4 * gw, 128), 0)
    lane = _iota((4 * gw, 128), 1)
    pick = ((r % gw) // 2 == lane).astype(BF16)
    head_start = ((r // gw) * 2 + r % 2) * bdh
    for j, g0 in enumerate(first_grp):
        wj = _nn(wf, (natural == _iota((dm, 128), 1) + j * 128).astype(BF16))
        wj = jnp.concatenate([wj, jnp.zeros((128 - bdh, 128), F32)], axis=0).astype(BF16)
        d = lane + (j * 128 - g0 * gw) - head_start
        fold[j] = jnp.where((d >= 0) & (d < bdh), _nn(pick, wj), 0.0).astype(BF16)

    early_copy.wait()
    early_xn[...] = _layernorm(
        early_x[...].astype(F32).reshape(early_xn.shape)).astype(BF16)

    start_pair(1)

    def load_pair(p, carry):
        for c in pair_copies(p):
            c.wait()
        pl.when(p > 0)(lambda: weight_copy(3, p - 1).wait())
        pl.when(p == n_pairs - 2)(lambda: weight_copy(3, n_pairs - 1).start())
        pl.when(p + 2 < n_pairs)(lambda: start_pair(p + 2))
        col = 0
        for i, (lo, hi) in enumerate(EARLY_TILES):
            w = stage[i, pair_rows(p), :]
            early_qkv[p, :, col:col + (hi - lo) * 128] = _nt(
                early_xn[...], w[lo * 128 - i * pw:hi * 128 - i * pw])
            col += (hi - lo) * 128
            wqkv[p, :, i * pw:(i + 1) * pw] = _pack(w.T)
        pack_wo(jnp.where(p > 0, 3, 0), jnp.maximum(p - 1, 0))
        wide = x_stage[pl.ds(p * x_chunk, x_chunk)].astype(F32).reshape(x_chunk * seg, dm)
        xres[pl.ds(pl.multiple_of(p * x_chunk * seg, x_chunk * seg), x_chunk * seg), :] = wide
        return carry

    lax.fori_loop(0, n_pairs, load_pair, 0)
    weight_copy(3, n_pairs - 1).wait()
    pack_wo(3, n_pairs - 1)
    mem0_copy.wait()
    bqkv_copy.start()
    bwo_copy.start()

    def fold_phi(base):
        groups = [None] * n_grp
        for j, g0 in enumerate(first_grp):
            t = _nt(fold[j], bqkv_stage[:, base + j * 128:base + (j + 1) * 128]) * LOG2E
            for i in range(4):
                part = t[i * gw:(i + 1) * gw]
                groups[g0 + i] = part if groups[g0 + i] is None else groups[g0 + i] + part
        return groups

    def hedgehog_weights():
        bqkv_copy.wait()
        bwo_copy.wait()
        wvt = bqkv_stage[:, 2 * dm:].astype(F32).T
        bwq[...] = _pack(jnp.concatenate(fold_phi(0), axis=0).astype(BF16))
        bw1[...] = _pack(jnp.concatenate(
            [t for g, wpk in enumerate(fold_phi(dm)) for t in (wpk, wvt[g * gw:(g + 1) * gw])],
            axis=0).astype(BF16))
        bwo[...] = _pack(bwo_stage[...])

    def seg_rows(s):
        return pl.ds(pl.multiple_of(s * seg, seg), seg)

    def rmt_step(s, mem, early):
        plan, norm_pair, order, ks = STEP_EARLY if early else STEP_REGULAR
        h = jnp.concatenate([mem, xn_a[...]], axis=0)
        h_short = h[:-EARLY_ROWS].astype(BF16)
        early_rows = pl.ds(pl.multiple_of(s * EARLY_ROWS, EARLY_ROWS), EARLY_ROWS)
        xn_next = _layernorm(xres[seg_rows(jnp.minimum(s + 1, n_seg - 1)), :])
        prev = seg_rows(jnp.maximum(s - 1, 0))
        xn_b[prev, :] = _layernorm(xres[prev, :]).astype(BF16)
        pending = {norm_pair: [xn_b[seg_rows(jnp.maximum(s, 1) - 1), :128].astype(F32)[:8]]}

        def project(p):
            spans, end = [], 0
            for lo, hi in EARLY_TILES if early else ():
                spans += [(h, end, lo)] * (end < lo) + [(h_short, lo, hi)]
                end = hi
            spans += [(h, end, 3 * pw // 128)] * (end < 3 * pw // 128)
            spans = [(x, slice(lo * 128, hi * 128)) for x, lo, hi in spans]
            if p > 0:
                parts = [_nn(x, _unpack(wqkv[p, :, cols])) for x, cols in spans]
            else:
                parts = [_nn(x[:, :ks], _unpack(wqkv[p, :ks // 2, cols])) for x, cols in spans]
                parts = [_nn(x[:, ks:], _unpack(wqkv[p, ks // 2:, cols])) + start
                         for start, (x, cols) in zip(parts, spans)]
            col = 0
            for i, t in enumerate(parts):
                if t.shape[0] < h.shape[0]:
                    known = early_qkv[p, early_rows, col:col + t.shape[1]]
                    parts[i] = jnp.concatenate([t, known], axis=0)
                    col += t.shape[1]
            return jnp.concatenate(parts, axis=1)

        def weighted_values(p, prob, v):
            head = prob[:n_mem]
            if p in pending:
                work = functools.reduce(jnp.add, pending[p])[:, :prob.shape[1]]
                head = jnp.where(s < 0, work, head)
            seen = n_mem + 8
            o = _nn(jnp.concatenate([head, prob[seen:]], axis=0), _pair_blockdiag(v, dh))
            v_scr[p, :seen, :] = v[:seen]
            v_scr[p, seen:seen + 1, :] = jnp.sum(v[seen:], axis=0, keepdims=True)
            first = jnp.concatenate(
                [prob[n_mem:seen], jnp.zeros((8, 128 - prob.shape[1]), F32)], axis=1)
            lane = _iota(first.shape, 1)
            tiles = [None] * (pw // 128)
            for k in range(seen + 1):
                wa, wb = (jnp.sum(jnp.where(lane == col, first, 0.0), axis=1, keepdims=True)
                          for col in (k, prob.shape[0] + k))
                for t, c in enumerate(range(0, pw, 128)):
                    w = wa if c + 128 <= dh else wb if c >= dh else jnp.where(lane < dh - c, wa, wb)
                    term = w * jnp.broadcast_to(v_scr[p, k:k + 1, c:c + 128], (8, 128))
                    tiles[t] = term if k == 0 else tiles[t] + term
            pending.setdefault(p + 1, []).extend(tiles)
            return jnp.concatenate([o[:n_mem], jnp.concatenate(tiles, axis=1), o[n_mem:]], axis=0)

        def out_proj(acc, lo, hi, cols=slice(None)):
            t = _nn(o_scr[:, lo * pw:hi * pw], _unpack(wo[lo * half:hi * half, cols]))
            return t if acc is None else t + acc[:, cols]

        qkv, prob = {}, {}
        acc, done = None, 0
        for p in range(len(plan)):
            r = p - (len(plan) - n_pairs)
            for what in order:
                if what == "q" and p < n_pairs:
                    qkv[p] = project(p)
                if what == "o" and plan[p] != "0":
                    acc = out_proj(acc, done, done + int(plan[p]))
                    done += int(plan[p])
                if what == "s" and 0 <= p - 1 < n_pairs:
                    t = qkv[p - 1]
                    scores = _nt(t[:, :pw], _pair_blockdiag(t[:, pw:2 * pw], dh))
                    prob[p - 1] = _pair_softmax(scores, n_mem, scale)
                if what == "v" and r >= 0:
                    o_scr[:, r * pw:(r + 1) * pw] = weighted_values(r, prob[r], qkv[r][:, 2 * pw:])
        acc = out_proj(acc, done, done + 1)
        acc = jnp.concatenate(
            [out_proj(acc, done + 1, n_pairs, cols) for cols in (slice(0, ks), slice(ks, dm))], axis=1)
        xn_a[...] = xn_next
        rows = seg_rows(s)
        xres[rows, :] = xres[rows, :] + acc[n_mem:]
        return acc[:n_mem]

    def rmt_steps(early):
        def body(i, mem):
            for u in range(unroll):
                mem = rmt_step(i * unroll + u, mem, early)
            return mem

        lax.fori_loop(0, n_seg // unroll, body, mem0_ref[...].astype(F32))

    def rmt_layer(layer):
        xn_a[...] = _layernorm(xres[0:seg, :])
        pl.when(layer == 0)(functools.partial(rmt_steps, True))
        pl.when(layer > 0)(functools.partial(rmt_steps, False))
        last = slice(seq - seg, seq)
        xn_b[last, :] = _layernorm(xres[last, :]).astype(BF16)

    chunk = 4
    n_chunk = n_grp // chunk

    def blk_rows(i):
        return pl.ds(pl.multiple_of(i * tb, tb), tb)

    def kv_block(i, carry):
        xn = xn_b[blk_rows(i), :]
        proj = {}
        for c in range(n_chunk + 1):
            if c < n_chunk:
                proj[c] = _nt(_unpack(bw1[c * chunk * gw:(c + 1) * chunk * gw, :]), xn)
            if c >= 1:
                t = proj[c - 1]
                for j in range(chunk):
                    g = (c - 1) * chunk + j
                    phi = _feature_map(t[2 * j * gw:(2 * j + 1) * gw])
                    kv_acc[g] += _nt(t[(2 * j + 1) * gw:(2 * j + 2) * gw], phi.astype(BF16))
                    z_acc[g] += functools.reduce(jnp.add, [phi[:, i:i + 128] for i in range(0, tb, 128)])
        return carry

    def out_rows(i):
        return pl.ds(pl.multiple_of(i * OUT_ROWS, OUT_ROWS), OUT_ROWS)

    def out_copy(i):
        return pltpu.make_async_copy(out_stage.at[out_rows(i)], out_hbm.at[out_rows(i)], out_sem.at[i])

    def out_block(i, layer):
        rows = blk_rows(i)
        xn = xn_b[rows, :]
        sublane = _iota((8, tb), 0)
        proj, outs = {}, []

        def out_proj(y, lo, hi):
            o = jnp.concatenate(outs, axis=0)[lo:hi].astype(BF16).T
            return _nn(o, _unpack(bwo[lo // 2:hi // 2, :])) + y

        y = xres[rows, :]
        for c in range(n_chunk + 1):
            if c < n_chunk:
                proj[c] = _nt(_unpack(bwq[c * chunk * bdh:(c + 1) * chunk * bdh, :]), xn)
            else:
                y = out_proj(y, 0, 256)
            if c >= 1:
                for j in range(chunk):
                    g = (c - 1) * chunk + j
                    phi = _feature_map(proj[c - 1][j * gw:(j + 1) * gw])
                    z = jnp.concatenate([z_acc[g]] * (tb // 128), axis=1)
                    inv = _recip(_over_features(phi * z, jnp.add) + DEN_EPS)
                    swapped = pltpu.roll(inv, 1, 0)
                    inv_a = jnp.where(sublane % 2 == 0, inv, swapped)
                    inv_b = jnp.where(sublane % 2 == 0, swapped, inv)
                    inv_ab = jnp.where(sublane < bdh % 8, inv_a, inv_b)
                    outs.append(_nn(kv_acc[g], phi.astype(BF16))
                                * jnp.concatenate([inv_a, inv_a, inv_ab, inv_b, inv_b], axis=0))
        y = out_proj(y, 256, 384)
        o = jnp.concatenate(outs, axis=0)[384:].astype(BF16).T
        for u in range(tb // OUT_ROWS):
            part = slice(u * OUT_ROWS, (u + 1) * OUT_ROWS)
            res = _nn(o[part], _unpack(bwo[384 // 2:, :])) + y[part]
            piece = i * (tb // OUT_ROWS) + u
            xres[out_rows(piece), :] = res
            out_stage[out_rows(piece), :] = res.astype(BF16)
            pl.when(layer == n_layers - 1)(lambda: out_copy(piece).start())
        return layer

    def hedgehog_layer(layer):
        kv_acc[...] = jnp.zeros(kv_acc.shape, F32)
        z_acc[...] = jnp.zeros(z_acc.shape, F32)
        lax.fori_loop(0, seq // tb, kv_block, 0)
        shape = kv_acc.shape[1:]
        same_head = _iota(shape, 0) // bdh == _iota(shape, 1) % 2
        for g in range(n_grp):
            kv_acc[g] = jnp.where(same_head, kv_acc[g], 0.0)
            z_acc[g] = jnp.broadcast_to(jnp.sum(z_acc[g], axis=1, keepdims=True), z_acc.shape[1:])
        lax.fori_loop(0, seq // tb, out_block, layer)

    def layer_pair(layer, carry):
        rmt_layer(layer)
        pl.when(layer == 0)(hedgehog_weights)
        hedgehog_layer(layer)
        return carry

    lax.fori_loop(0, n_layers, layer_pair, 0)
    for i in range(seq // OUT_ROWS):
        out_copy(i).wait()


@functools.partial(jax.jit, static_argnames=("A_seg_len",))
def pallas_interleave_layers__memory_aug_recurrent_mem_tr__linear_kernel_hedgehog__prompt_kernel(
    A_x: jax.Array,
    A_mem0: jax.Array,
    A_Wq: jax.Array,
    A_Wk: jax.Array,
    A_Wv: jax.Array,
    A_Wo: jax.Array,
    A_seg_len: int,
    B_x: jax.Array,
    B_wqkv: jax.Array,
    B_w_phi: jax.Array,
    B_wo: jax.Array,
):
    del B_x
    batch, seq, dm = A_x.shape
    _, heads, dh = A_Wq.shape
    n_mem = A_mem0.shape[1]
    bh, bdh, _ = B_w_phi.shape
    seg = int(A_seg_len)
    assert batch == 1 and bdh == 20 and bh * bdh == dm and heads % 2 == 0
    assert (2 * dh) % 128 == 0 and n_mem % 8 == 0 and seg % 16 == 0 and 2 * (n_mem + seg) <= 128
    n_pairs, pw, hd = heads // 2, 2 * dh, heads * dh
    tb, unroll = 512, 2
    early_rows = seq // seg * EARLY_ROWS
    early_cols = 128 * sum(hi - lo for lo, hi in EARLY_TILES)

    def feature_major(w):
        return jnp.transpose(w, (1, 2, 0)).reshape(hd, dm)

    hbm = pl.BlockSpec(memory_space=pl.ANY)
    out = pl.pallas_call(
        functools.partial(_kernel, seg=seg, dh=dh, n_layers=2, tb=tb, unroll=unroll),
        out_shape=jax.ShapeDtypeStruct((seq, dm), A_x.dtype),
        in_specs=[hbm] * 9,
        out_specs=hbm,
        scratch_shapes=[
            pltpu.VMEM((4, hd, dm), BF16),
            pltpu.VMEM((n_pairs, dm // 2, 3 * pw), U32),
            pltpu.VMEM((hd // 2, dm), U32),
            pltpu.VMEM((seq // seg, seg, dm), BF16),
            pltpu.VMEM((seq, dm), BF16),
            pltpu.VMEM((dm, 3 * dm), BF16),
            pltpu.VMEM((dm, dm), BF16),
            pltpu.VMEM((dm // 128, 8 * bdh, 128), BF16),
            pltpu.VMEM((dm, dm), U32),
            pltpu.VMEM((dm // 2, dm), U32),
            pltpu.VMEM((dm // 2, dm), U32),
            pltpu.VMEM((seq, dm), F32),
            pltpu.VMEM((seg, dm), F32),
            pltpu.VMEM((seq, dm), BF16),
            pltpu.VMEM((n_mem + seg, hd), F32),
            pltpu.VMEM((n_pairs, n_mem + 16, pw), F32),
            pltpu.VMEM((bh // 2, 2 * bdh, 4 * bdh), F32),
            pltpu.VMEM((bh // 2, 4 * bdh, 128), F32),
            pltpu.VMEM((seq // seg, EARLY_ROWS, dm), BF16),
            pltpu.VMEM((early_rows, dm), BF16),
            pltpu.VMEM((n_pairs, early_rows, early_cols), F32),
            pltpu.VMEM((n_mem, dm), BF16),
            pltpu.VMEM((bdh, bdh, bh), BF16),
            pltpu.SemaphoreType.DMA((5, 4)),
            pltpu.SemaphoreType.DMA((5,)),
            pltpu.SemaphoreType.DMA((seq // OUT_ROWS,)),
        ],
        compiler_params=pltpu.CompilerParams(vmem_limit_bytes=120 * 1024 * 1024, disable_bounds_checks=True),
        name="rmt_hedgehog",
    )(
        A_x.reshape(seq // seg, seg, dm),
        A_mem0.reshape(n_mem, dm),
        feature_major(A_Wq),
        feature_major(A_Wk),
        feature_major(A_Wv),
        A_Wo.reshape(hd, dm),
        B_wqkv,
        jnp.transpose(B_w_phi, (1, 2, 0)),
        B_wo,
    )
    return out.reshape(batch, seq, dm)
```
